```python
import jax
import jax.numpy as jnp

def _softmax(x, axis=-1):
    return jax.nn.softmax(x, axis=axis)
def _gelu(x):
    return jax.nn.gelu(x, approximate=True)
def _silu(x):
    return jax.nn.silu(x)
def _sigmoid(x):
    return jax.nn.sigmoid(x)
def _layernorm(x, axis=-1, eps=1e-5):
    m = jnp.mean(x, axis=axis, keepdims=True)
    v = jnp.var(x, axis=axis, keepdims=True)
    return (x - m) / jnp.sqrt(v + eps)
def _scatter_add(tgt, idx, src, axis=0):
    return tgt.at[idx].add(src)
def _segment_sum(src, seg, n):
    return jax.ops.segment_sum(src, seg, n)
class _Rng:
    def __init__(self, key):
        self._k = key
    def _next(self):
        self._k, sub = jax.random.split(self._k)
        return sub
    def normal(self, shape):
        return jax.random.normal(self._next(), shape, dtype=jnp.bfloat16)
    def randint(self, lo, hi, shape):
        return jax.random.randint(self._next(), shape, lo, hi, dtype=jnp.int32)
    def uniform(self, shape, lo=0.0, hi=1.0):
        return jax.random.uniform(self._next(), shape, jnp.bfloat16, lo, hi)
    def permutation(self, n):
        return jax.random.permutation(self._next(), n)


kernel_name = 'concat_heads__sliding_local_dilated__ssm_conv_s5__prompt'

def setup_inputs():
    _rng = _Rng(jax.random.key(int.from_bytes(__import__("os").urandom(4), "little")))
    _w = (lambda a: (lambda t: t.astype(jnp.bfloat16) if jnp.issubdtype(t.dtype, jnp.floating) else t)(jnp.asarray(a)))
    def _A_setup():
        B, S, D = 1, 2048, 448
        return {
            "x": _w((lambda *s: _rng.normal(s) * 0.05)(B, S, D)),
            "wqkv": _w((lambda *s: _rng.normal(s) * 0.05)(D, 3 * D)),
            "wo": _w((lambda *s: _rng.normal(s) * 0.05)(D, D)),
        }
    _A_in = _A_setup()

    def _B_setup():
        B, S, D = 1, 2048, 448
        P = D
        Lambda_re = -0.5 * jnp.exp((lambda *s: _rng.normal(s) * 0.05)(P))
        Lambda_im = (lambda *s: _rng.normal(s) * 0.05)(P) * 1.0
        B_re = (lambda *s: _rng.normal(s) * 0.05)(P, D) * (D ** -0.5)
        B_im = (lambda *s: _rng.normal(s) * 0.05)(P, D) * (D ** -0.5)
        C_re = (lambda *s: _rng.normal(s) * 0.05)(D, P) * (P ** -0.5)
        C_im = (lambda *s: _rng.normal(s) * 0.05)(D, P) * (P ** -0.5)
        log_dt = (lambda *s: _rng.normal(s) * 0.05)(P) * 0.3 - 2.0
        Dskip = (lambda *s: _rng.normal(s) * 0.05)(D)
        return {
            "x": _w((lambda *s: _rng.normal(s) * 0.05)(B, S, D)),
            "Lambda_re": _w(Lambda_re),
            "Lambda_im": _w(Lambda_im),
            "B_re": _w(B_re),
            "B_im": _w(B_im),
            "C_re": _w(C_re),
            "C_im": _w(C_im),
            "log_dt": _w(log_dt),
            "Dskip": _w(Dskip),
        }
    _B_in = _B_setup()

    return {
        "A_x": _A_in["x"],
        "A_wqkv": _A_in["wqkv"],
        "A_wo": _A_in["wo"],
        "B_x": _B_in["x"],
        "B_Lambda_re": _B_in["Lambda_re"],
        "B_Lambda_im": _B_in["Lambda_im"],
        "B_B_re": _B_in["B_re"],
        "B_B_im": _B_in["B_im"],
        "B_C_re": _B_in["C_re"],
        "B_C_im": _B_in["C_im"],
        "B_log_dt": _B_in["log_dt"],
        "B_Dskip": _B_in["Dskip"],
    }

def reference(A_x, A_wqkv, A_wo, B_x, B_Lambda_re, B_Lambda_im, B_B_re, B_B_im, B_C_re, B_C_im, B_log_dt, B_Dskip):
    def _A_ref(x, wqkv, wo):
        B, S, D = x.shape
        H = 16; Dh = D // H
        W, dil = 8, 2
        qkv = (lambda x, *d: x.transpose(*d))((x @ wqkv).reshape(B, S, 3, H, Dh), 2, 0, 3, 1, 4)
        q, k, v = qkv[0], qkv[1], qkv[2]
        scale = Dh ** -0.5
        pos = jnp.arange(S)
        off = jnp.arange(W) * dil
        idx = pos[:, None] - off[None, :]
        mask = idx >= 0
        idx_c = jnp.where(mask, idx, 0).reshape(-1)
        kg = k[:, :, idx_c, :].reshape(B, H, S, W, Dh)
        vg = v[:, :, idx_c, :].reshape(B, H, S, W, Dh)
        logits = jnp.einsum("bhsd,bhswd->bhsw", q, kg) * scale
        logits = jnp.where(mask[None, None, :, :], logits, -1e9)
        attn = _softmax(logits, axis=-1)
        o = jnp.einsum("bhsw,bhswd->bhsd", attn, vg)
        return (lambda x, *d: x.transpose(*d))(o, 0, 2, 1, 3).reshape(B, S, D) @ wo

    def _B_ref(x, Lambda_re, Lambda_im, B_re, B_im, C_re, C_im, log_dt, Dskip):
        Bsz, L, H = x.shape
        Lam = Lambda_re + 1j * Lambda_im
        Bmat = B_re + 1j * B_im
        Cmat = C_re + 1j * C_im
        dt = jnp.exp(log_dt)
        Lam_bar = jnp.exp(dt * Lam)
        B_bar = ((Lam_bar - 1.0) / Lam)[:, None] * Bmat
        Bu = jnp.einsum("bld,pd->blp", x + 0j, B_bar)
        h = jnp.zeros_like(Bu[:, 0, :])
        hs = []
        for t in range(L):
            h = Lam_bar[None, :] * h + Bu[:, t, :]
            hs.append(h)
        hseq = jnp.stack(hs, 1)
        y = 2.0 * jnp.einsum("blp,dp->bld", hseq, Cmat).real + x * Dskip[None, None, :]
        return y

    a = _A_ref(A_x, A_wqkv, A_wo)
    b = _B_ref(B_x, B_Lambda_re, B_Lambda_im, B_B_re, B_B_im, B_C_re, B_C_im, B_log_dt, B_Dskip)
    return jnp.concatenate([a, b], axis=-1)
```

```python
import jax
import jax.numpy as jnp
from jax import lax
import jax.experimental.pallas as pl
import jax.experimental.pallas.tpu as pltpu

S = 2048
D = 448
H = 16
DH = 28
W = 8
R = 16
G = 4
TG = S // G
JG = TG // R

F32 = jnp.float32
BF16 = jnp.bfloat16
U32 = jnp.uint32
NT = (((1,), (1,)), ((), ()))


def _unpack(w):
    lo = pltpu.bitcast(w << 16, F32)
    hi = pltpu.bitcast(w & jnp.uint32(0xFFFF0000), F32)
    return lo, hi


def _pack(even, odd):
    return pltpu.pack_elementwise([even, odd], packed_dtype=BF16)


def _transpose_x(xt_ref, xn_ref, t0, nt):
    for c in range(4):
        rows = min(128, D - c * 128)
        v = xt_ref[c * 128:c * 128 + rows, pl.ds(t0, nt)]
        if rows < 128:
            v = jnp.concatenate([v, jnp.zeros((128 - rows, nt), v.dtype)], axis=0)
        xn_ref[pl.ds(c * S + t0, nt), :] = v.T


def _gather_rows(xn_ref, row0, rhos, nj):
    xu = xn_ref.bitcast(U32)
    cols = []
    for c in range(4):
        parts = []
        for rho in rhos:
            lo, hi = _unpack(xu[pl.ds(c * (S // 2) + row0 + rho, nj, stride=R // 2), :])
            parts += [lo, hi]
        cols.append(jnp.concatenate(parts, axis=0).astype(BF16))
    return jnp.concatenate(cols, axis=1)


def _step(lam, h, b):
    if len(h) == 2:
        lr, li = lam
        return (lr * h[0] - li * h[1] + b[0], lr * h[1] + li * h[0] + b[1])
    la, lb = lam
    return (la * h[0] + lb * pltpu.roll(h[0], 64, 1) + b[0],)


def _lam_tiles(re, im, lane):
    out = []
    for c in range(3):
        out.append((re[:, c * 128:(c + 1) * 128], im[:, c * 128:(c + 1) * 128]))
    z = jnp.zeros((1, 64), F32)
    r3 = jnp.concatenate([re[:, 384:], z], axis=1)
    i3 = jnp.concatenate([im[:, 384:], z], axis=1)
    out.append((jnp.where(lane < 64, r3, pltpu.roll(r3, 64, 1)),
                jnp.where(lane < 64, -i3, pltpu.roll(i3, 64, 1))))
    return out


def _kernel(xa_hbm, wqkv_hbm, wo_hbm, xb_hbm, lre_ref, lim_ref, bre_hbm, bim_hbm,
            cre_hbm, cim_hbm, ldt_ref, dsk_ref, out_hbm,
            xat, xbt, xan, xbn, bst, bu, wraw, wtn, wt, q_s, k_s, v_s, h_s, o_s,
            cre, cim, cst, woraw, won, wop, ob, sem_xb, sem_b, sem_in, sem_out):
    xb_cp = [pltpu.make_async_copy(xb_hbm.at[0, :, pl.ds(g * TG, TG)],
                                   xbt.at[:, pl.ds(g * TG, TG)], sem_xb.at[g])
             for g in range(G)]
    b_cp = []
    for c in range(3):
        b_cp.append(pltpu.make_async_copy(bre_hbm.at[pl.ds(c * 128, 128)],
                                          bst.at[pl.ds(c * 256, 128)], sem_b.at[0]))
        b_cp.append(pltpu.make_async_copy(bim_hbm.at[pl.ds(c * 128, 128)],
                                          bst.at[pl.ds(c * 256 + 128, 128)], sem_b.at[0]))
    b_cp.append(pltpu.make_async_copy(bre_hbm.at[pl.ds(384, 64)], bst.at[pl.ds(768, 64)], sem_b.at[0]))
    b_cp.append(pltpu.make_async_copy(bim_hbm.at[pl.ds(384, 64)], bst.at[pl.ds(832, 64)], sem_b.at[0]))
    w_cp = pltpu.make_async_copy(wqkv_hbm, wraw, sem_in.at[0])
    xa_cp = pltpu.make_async_copy(xa_hbm.at[0], xat, sem_in.at[1])
    cre_cp = pltpu.make_async_copy(cre_hbm, cre, sem_in.at[2])
    cim_cp = pltpu.make_async_copy(cim_hbm, cim, sem_in.at[3])
    wo_cp = pltpu.make_async_copy(wo_hbm, woraw, sem_in.at[4])

    xb_cp[0].start()
    for cp in b_cp:
        cp.start()
    for cp in xb_cp[1:]:
        cp.start()

    lane = lax.broadcasted_iota(jnp.int32, (1, 128), 1)
    a_re = lre_ref[...].astype(F32).reshape(1, D)
    a_im = lim_ref[...].astype(F32).reshape(1, D)
    dt = jnp.exp(ldt_ref[...].astype(F32).reshape(1, D)).astype(BF16).astype(F32)
    mag = jnp.exp(dt * a_re)
    l_re = mag * jnp.cos(dt * a_im)
    l_im = mag * jnp.sin(dt * a_im)
    den = a_re * a_re + a_im * a_im
    n_re = l_re - 1.0
    co_re = 2.0 * (n_re * a_re + l_im * a_im) / den
    co_im = 2.0 * (l_im * a_re - n_re * a_im) / den
    lam1 = _lam_tiles(l_re, l_im, lane)
    p_re, p_im = l_re, l_im
    for _ in range(4):
        p_re, p_im = p_re * p_re - p_im * p_im, 2.0 * p_re * p_im
    lam_pows = []
    for _ in range(5):
        lam_pows.append(_lam_tiles(p_re, p_im, lane))
        p_re, p_im = p_re * p_re - p_im * p_im, 2.0 * p_re * p_im

    xb_cp[0].wait()
    for cp in b_cp:
        cp.wait()
    for cp in (w_cp, xa_cp, cre_cp, cim_cp, wo_cp):
        cp.start()

    def prep_w():
        for c in range(4):
            rows = min(128, D - c * 128)
            for n in range(11):
                cols = min(128, 3 * D - n * 128)
                v = wraw[c * 128:c * 128 + rows, n * 128:n * 128 + cols]
                if rows < 128:
                    v = jnp.concatenate([v, jnp.zeros((128 - rows, cols), BF16)], axis=0)
                if cols < 128:
                    v = jnp.concatenate([v, jnp.zeros((128, 128 - cols), BF16)], axis=1)
                wtn[pl.ds(c * 1408 + n * 128, 128), :] = v.T
        wu = wtn.bitcast(U32)
        for c in range(4):
            for part in range(3):
                for dp in range(DH // 2):
                    lo, hi = _unpack(wu[pl.ds(c * 704 + part * (D // 2) + dp, H, stride=DH // 2), :])
                    base = part * D + dp * 2 * H
                    wt[base:base + 2 * H, c * 128:(c + 1) * 128] = (
                        jnp.concatenate([lo, hi], axis=0).astype(BF16))

    def prep_wo():
        for c in range(4):
            cols = min(128, D - c * 128)
            v = woraw[:, c * 128:c * 128 + cols]
            if cols < 128:
                v = jnp.concatenate([v, jnp.zeros((D, 128 - cols), BF16)], axis=1)
            won[pl.ds(c * D, D), :] = v
        wu = won.bitcast(U32)
        for c in range(4):
            for dp in range(DH // 2):
                lo, hi = _unpack(wu[pl.ds(c * (D // 2) + dp, H, stride=DH // 2), :])
                wop[dp * 2 * H:(dp + 1) * 2 * H, c * 128:(c + 1) * 128] = (
                    jnp.concatenate([lo, hi], axis=0).astype(BF16))
        wop[D:512, :] = jnp.zeros((512 - D, 512), BF16)

    def prep_c():
        cst[0:64, :] = jnp.zeros((64, 2 * D), BF16)
        for c in range(3):
            sl = slice(c * 128, (c + 1) * 128)
            xr = cre[:, sl].astype(F32)
            xi = cim[:, sl].astype(F32)
            cr, ci = co_re[:, sl], co_im[:, sl]
            cst[64:512, c * 256:c * 256 + 128] = (xr * cr - xi * ci).astype(BF16)
            cst[64:512, c * 256 + 128:c * 256 + 256] = (-(xr * ci + xi * cr)).astype(BF16)
        xr = cre[:, 384:D].astype(F32)
        xi = cim[:, 384:D].astype(F32)
        cr, ci = co_re[:, 384:], co_im[:, 384:]
        cst[64:512, 768:896] = jnp.concatenate(
            [xr * cr - xi * ci, -(xr * ci + xi * cr)], axis=1).astype(BF16)

    for g in range(G):
        if g > 0:
            xb_cp[g].wait()
        _transpose_x(xbt, xbn, g * TG, TG)
        xp = _gather_rows(xbn, g * (TG // 2), range(R // 2), JG)
        bu[g * TG:(g + 1) * TG, :] = lax.dot_general(
            xp[:, :D], bst[...], NT, preferred_element_type=F32)
        if g == 1:
            w_cp.wait()
            prep_w()
        if g == 2:
            xa_cp.wait()
            _transpose_x(xat, xan, 0, S)
        if g == 3:
            cre_cp.wait()
            cim_cp.wait()
            wo_cp.wait()
            prep_c()
            prep_wo()

    row = lax.broadcasted_iota(jnp.int32, (JG, 128), 0)
    hu = h_s.bitcast(U32)

    def scan_chunk(g, prev):
        last = []
        for c in range(4):
            nparts = 2 if c < 3 else 1

            def load(r):
                return tuple(
                    bu[pl.ds(g * TG + r * JG, JG),
                       c * 256 + k * 128:c * 256 + (k + 1) * 128]
                    for k in range(nparts))

            f = load(0)
            for r in range(1, R):
                f = _step(lam1[c], f, load(r))
            s = tuple(pltpu.roll(jnp.where(row == JG - 1, p, x), 1, 0)
                      for p, x in zip(prev[c], f))
            for m in range(5):
                sh = tuple(jnp.where(row >= 2 ** m, pltpu.roll(x, 2 ** m, 0), 0.0) for x in s)
                s = _step(lam_pows[m][c], sh, s)
            for rho in range(R // 2):
                e = _step(lam1[c], s, load(2 * rho))
                s = _step(lam1[c], e, load(2 * rho + 1))
                for k in range(nparts):
                    hu[pl.ds((2 * c + k) * (S // 2) + g * (TG // 2) + rho, JG,
                             stride=R // 2), :] = pltpu.bitcast(_pack(e[k], s[k]), U32)
            last.append(s)
        return tuple(last)

    def phase2(g, prev):
        last = scan_chunk(g, prev)
        xp = _gather_rows(xan, 2 * g, range(2), 128)
        res = lax.dot_general(wt[:, :D], xp[:, :D], NT, preferred_element_type=F32)
        for i in range(4):
            sl = slice(i * 128, (i + 1) * 128)
            q_s[4 * g + i] = res[0:D, sl]
            kk = res[D:2 * D, sl]
            vv = res[2 * D:3 * D, sl]
            k_s[R + 4 * g + i] = kk
            v_s[R + 4 * g + i] = vv
            if 4 * g + i >= 2:
                k_s[4 * g + i] = pltpu.roll(kk, 1, 1)
                v_s[4 * g + i] = pltpu.roll(vv, 1, 1)
        return last

    zero = jnp.zeros((JG, 128), F32)
    prev = ((zero, zero),) * 3 + ((zero,),)
    for g in range(G):
        prev = phase2(g, prev)

    lane_h = lax.broadcasted_iota(jnp.int32, (H, 128), 1)
    scale = DH ** -0.5
    ou = o_s.bitcast(U32)
    z64 = jnp.zeros((1, 64), F32)
    dsk = jnp.concatenate([z64, dsk_ref[...].astype(F32).reshape(1, D)], axis=1)

    def attend(r):
        acc = [None] * W
        for d in range(DH):
            rows = slice(d * H, (d + 1) * H)
            qd = q_s[r, rows, :]
            for w in range(W):
                t = qd * k_s[R + r - 2 * w, rows, :]
                acc[w] = t if d == 0 else acc[w] + t
        lg = []
        for w in range(W):
            x = acc[w] * scale
            lg.append(jnp.where(lane_h < 1, -1e9, x) if r < 2 * w else x)
        m = lg[0]
        for w in range(1, W):
            m = jnp.maximum(m, lg[w])
        e = [jnp.exp(x - m) for x in lg]
        tot = e[0]
        for w in range(1, W):
            tot = tot + e[w]
        inv = 1.0 / tot
        p = [x * inv for x in e]
        outs = []
        for d in range(DH):
            rows = slice(d * H, (d + 1) * H)
            o = p[0] * v_s[R + r, rows, :]
            for w in range(1, W):
                o = o + p[w] * v_s[R + r - 2 * w, rows, :]
            outs.append(o)
        return jnp.concatenate(outs, axis=0)

    def y_copy(g):
        rows = pl.ds(g * TG, TG)
        return pltpu.make_async_copy(ob.at[rows, pl.ds(512, 384)],
                                     out_hbm.at[0, rows, pl.ds(512, 384)], sem_out.at[g])

    def phase3(g, carry):
        for i in range(2):
            rho = 2 * g + i
            wds = pltpu.bitcast(_pack(attend(2 * rho), attend(2 * rho + 1)), U32)
            wds = jnp.concatenate([wds, jnp.zeros((512 - D, 128), U32)], axis=0)
            for c in range(4):
                ou[pl.ds(c * (S // 2) + rho, 128, stride=R // 2), :] = wds[c * 128:(c + 1) * 128].T
        t0 = g * TG
        hh = jnp.concatenate([h_s[pl.ds(k * S + t0, TG), :] for k in range(7)], axis=1)
        y = lax.dot_general(hh, cst[...], NT, preferred_element_type=F32)
        xr = [pltpu.roll(xbn[pl.ds(c * S + t0, TG), :].astype(F32), 64, 1) for c in range(4)]
        xs = jnp.concatenate([jnp.where(lane < 64, xr[c - 1], xr[c]) for c in range(4)], axis=1)
        ob[pl.ds(t0, TG), 384:896] = y + xs * dsk
        y_copy(g).start()
        return carry

    for g in range(G):
        phase3(g, 0)

    TA = 256

    def a_copy(i):
        rows = pl.ds(pl.multiple_of(i * TA, TA), TA)
        return pltpu.make_async_copy(ob.at[rows, pl.ds(0, 512)],
                                     out_hbm.at[0, rows, pl.ds(0, 512)], sem_out.at[G + i])

    def phase4(i, carry):
        t0 = pl.multiple_of(i * TA, TA)
        oo = jnp.concatenate([o_s[pl.ds(c * S + t0, TA), :] for c in range(4)], axis=1)
        a = jnp.dot(oo, wop[...], preferred_element_type=F32)
        ob[pl.ds(t0, TA), 0:384] = a[:, 0:384]
        ob[pl.ds(t0, TA), 384:512] = ob[pl.ds(t0, TA), 384:512] + a[:, 384:512]
        a_copy(i).start()
        return carry

    lax.fori_loop(0, S // TA, phase4, 0)
    for g in range(G):
        y_copy(g).wait()
    for i in range(S // TA):
        a_copy(i).wait()


@jax.jit
def pallas_concat_heads__sliding_local_dilated__ssm_conv_s5__prompt_kernel(
    A_x, A_wqkv, A_wo, B_x, B_Lambda_re, B_Lambda_im, B_B_re, B_B_im, B_C_re, B_C_im,
    B_log_dt, B_Dskip,
):
    hbm = pl.BlockSpec(memory_space=pl.ANY)
    vec = pl.BlockSpec(memory_space=pltpu.VMEM)
    vm = pltpu.VMEM
    scratch = [
        vm((D, S), BF16), vm((D, S), BF16),
        vm((4 * S, 128), BF16), vm((4 * S, 128), BF16),
        vm((2 * D, D), BF16),
        vm((S, 2 * D), F32),
        vm((D, 3 * D), BF16),
        vm((4 * 1408, 128), BF16),
        vm((3 * D, 512), BF16),
        vm((R, D, 128), F32),
        vm((2 * R, D, 128), F32), vm((2 * R, D, 128), F32),
        vm((7 * S, 128), BF16),
        vm((4 * S, 128), BF16),
        vm((D, D), BF16), vm((D, D), BF16),
        vm((512, 2 * D), BF16),
        vm((D, D), BF16), vm((4 * D, 128), BF16), vm((512, 512), BF16),
        vm((S, 2 * D), F32),
        pltpu.SemaphoreType.DMA((G,)), pltpu.SemaphoreType.DMA((1,)),
        pltpu.SemaphoreType.DMA((5,)), pltpu.SemaphoreType.DMA((G + 8,)),
    ]
    return pl.pallas_call(
        _kernel,
        out_shape=jax.ShapeDtypeStruct((1, S, 2 * D), F32),
        in_specs=[hbm, hbm, hbm, hbm, vec, vec, hbm, hbm, hbm, hbm, vec, vec],
        out_specs=hbm,
        scratch_shapes=scratch,
        compiler_params=pltpu.CompilerParams(vmem_limit_bytes=100 * 1024 * 1024),
    )(jnp.swapaxes(A_x, 1, 2), A_wqkv, A_wo, jnp.swapaxes(B_x, 1, 2), B_Lambda_re, B_Lambda_im,
      B_B_re, B_B_im, B_C_re, B_C_im, B_log_dt, B_Dskip)
```

```python
import jax
import jax.numpy as jnp
from functools import partial
from jax import lax
import jax.experimental.pallas as pl
import jax.experimental.pallas.tpu as pltpu

S = 2048
D = 448
H = 16
DH = 28
W = 8
R = 16
G = 4
TG = S // G
JG = TG // R

F32 = jnp.float32
BF16 = jnp.bfloat16
U32 = jnp.uint32
NT = (((1,), (1,)), ((), ()))


def _unpack(w):
    lo = pltpu.bitcast(w << 16, F32)
    hi = pltpu.bitcast(w & jnp.uint32(0xFFFF0000), F32)
    return lo, hi


def _pack(even, odd):
    return pltpu.pack_elementwise([even, odd], packed_dtype=BF16)


def _transpose_x(xt_ref, xn_ref, c, t0, nt):
    xn_ref[pl.ds(c * S + t0, nt), :] = xt_ref[c * 128:(c + 1) * 128, pl.ds(t0, nt)].T


def _gather_rows(xn_ref, xp_ref, c, row0, rho, nj, dst):
    xu = xn_ref.bitcast(U32)
    lo, hi = _unpack(xu[pl.ds(c * (S // 2) + row0 + rho, nj, stride=R // 2), :])
    xp_ref[dst:dst + nj, c * 128:(c + 1) * 128] = lo.astype(BF16)
    xp_ref[dst + nj:dst + 2 * nj, c * 128:(c + 1) * 128] = hi.astype(BF16)


def _interleave(main, side):
    side = list(side)
    done = 0
    for i, task in enumerate(main):
        task()
        upto = (len(side) * (i + 1)) // len(main)
        for t in side[done:upto]:
            t()
        done = upto


def _step(lam, h, b):
    lr, li = lam
    return (lr * h[0] - li * h[1] + b[0], lr * h[1] + li * h[0] + b[1])


def _lam_tiles(re, im, lane):
    out = []
    for c in range(3):
        out.append((re[:, c * 128:(c + 1) * 128], im[:, c * 128:(c + 1) * 128]))
    z = jnp.zeros((1, 64), F32)
    r3 = jnp.concatenate([re[:, 384:], z], axis=1)
    i3 = jnp.concatenate([im[:, 384:], z], axis=1)
    out.append((jnp.where(lane < 64, r3, pltpu.roll(r3, 64, 1)),
                jnp.where(lane < 64, i3, -pltpu.roll(i3, 64, 1))))
    return out


def _kernel(xa_hbm, wqkv_hbm, wo_hbm, xb_hbm, lre_ref, lim_ref, bre_hbm, bim_hbm,
            cre_hbm, cim_hbm, ldt_ref, dsk_ref, out_hbm,
            xat, xbt, xan, xbn, xap, xbp, bst, bu, wraw, wtn, wt, q_s, k_s, v_s, h_s, o_s,
            cre, cim, cst, woraw, won, wop, ow, ob, sem_xb, sem_b, sem_in, sem_out):
    xb_cp = [pltpu.make_async_copy(xb_hbm.at[0, :, pl.ds(g * TG, TG)],
                                   xbt.at[pl.ds(0, D), pl.ds(g * TG, TG)], sem_xb.at[g])
             for g in range(G)]
    b_cp = []
    for c in range(3):
        b_cp.append(pltpu.make_async_copy(bre_hbm.at[pl.ds(c * 128, 128)],
                                          bst.at[pl.ds(c * 256, 128)], sem_b.at[c]))
        b_cp.append(pltpu.make_async_copy(bim_hbm.at[pl.ds(c * 128, 128)],
                                          bst.at[pl.ds(c * 256 + 128, 128)], sem_b.at[c]))
    b_cp.append(pltpu.make_async_copy(bre_hbm.at[pl.ds(384, 64)], bst.at[pl.ds(768, 64)], sem_b.at[3]))
    b_cp.append(pltpu.make_async_copy(bim_hbm.at[pl.ds(384, 64)], bst.at[pl.ds(832, 64)], sem_b.at[3]))
    w_cp = pltpu.make_async_copy(wqkv_hbm, wraw, sem_in.at[0])
    xa_cp = pltpu.make_async_copy(xa_hbm.at[0], xat.at[pl.ds(0, D)], sem_in.at[1])
    cre_cp = pltpu.make_async_copy(cre_hbm, cre, sem_in.at[2])
    cim_cp = pltpu.make_async_copy(cim_hbm, cim, sem_in.at[3])
    wo_cp = pltpu.make_async_copy(wo_hbm, woraw, sem_in.at[4])

    xb_cp[0].start()
    for cp in b_cp:
        cp.start()
    for cp in xb_cp[1:]:
        cp.start()

    lane = lax.broadcasted_iota(jnp.int32, (1, 128), 1)
    a_re = lre_ref[...].astype(F32).reshape(1, D)
    a_im = lim_ref[...].astype(F32).reshape(1, D)
    dt = jnp.exp(ldt_ref[...].astype(F32).reshape(1, D)).astype(BF16).astype(F32)
    mag = jnp.exp(dt * a_re)
    l_re = mag * jnp.cos(dt * a_im)
    l_im = mag * jnp.sin(dt * a_im)
    den = a_re * a_re + a_im * a_im
    n_re = l_re - 1.0
    co_re = 2.0 * (n_re * a_re + l_im * a_im) / den
    co_im = 2.0 * (l_im * a_re - n_re * a_im) / den
    lam1 = _lam_tiles(l_re, l_im, lane)
    p_re, p_im = l_re, l_im
    for _ in range(4):
        p_re, p_im = p_re * p_re - p_im * p_im, 2.0 * p_re * p_im
    lam_pows = []
    for _ in range(5):
        lam_pows.append(_lam_tiles(p_re, p_im, lane))
        p_re, p_im = p_re * p_re - p_im * p_im, 2.0 * p_re * p_im

    xat[D:512, :] = jnp.zeros((512 - D, S), BF16)
    xbt[D:512, :] = jnp.zeros((512 - D, S), BF16)
    wop[D:512, :] = jnp.zeros((512 - D, 512), BF16)
    cst[0:64, :] = jnp.zeros((64, 2 * D), BF16)

    zbits = lax.broadcasted_iota(U32, (8, 128), 1) >> 16
    cur = [None]

    queue = []
    pos = [0, 1]

    def pace(tasks, steps):
        queue[:] = tasks
        pos[:] = [0, steps]

    def gate(xs):
        i, n = pos
        if i % n == 0:
            queue.pop(0)()
        pos[0] = i + 1
        res = cur[0]
        k = (res.shape[0] // 8 * (i % n)) // n * 8
        tok = mark(res[k:k + 8])
        return tuple(after(x, tok) for x in xs)

    def mark(res):
        return pltpu.bitcast(res[0:8, 0:128], U32) & zbits

    def after(x, tok, rest=None):
        u = pltpu.bitcast(x, U32)
        x = pltpu.bitcast(u | jnp.tile(tok, (u.shape[0] // 8, u.shape[1] // 128)), x.dtype)
        return x if rest is None else jnp.concatenate([x, rest], axis=1)

    def w_transpose(n):
        cols = min(128, 3 * D - n * 128)
        for c in range(4):
            rows = min(128, D - c * 128)
            v = wraw[c * 128:c * 128 + rows, n * 128:n * 128 + cols]
            if rows < 128:
                v = jnp.concatenate([v, jnp.zeros((128 - rows, cols), BF16)], axis=0)
            if cols < 128:
                v = jnp.concatenate([v, jnp.zeros((128, 128 - cols), BF16)], axis=1)
            wtn[pl.ds(c * 1408 + n * 128, 128), :] = v.T

    def w_gather(part, c):
        wu = wtn.bitcast(U32)
        for dp in range(DH // 2):
            lo, hi = _unpack(wu[pl.ds(c * 704 + part * (D // 2) + dp, H, stride=DH // 2), :])
            base = part * D + dp * 2 * H
            wt[base:base + H, c * 128:(c + 1) * 128] = lo.astype(BF16)
            wt[base + H:base + 2 * H, c * 128:(c + 1) * 128] = hi.astype(BF16)

    def prep_wo(c):
        cols = min(128, D - c * 128)
        v = woraw[:, c * 128:c * 128 + cols]
        if cols < 128:
            v = jnp.concatenate([v, jnp.zeros((D, 128 - cols), BF16)], axis=1)
        won[pl.ds(c * D, D), :] = v
        wu = won.bitcast(U32)
        for dp in range(DH // 2):
            lo, hi = _unpack(wu[pl.ds(c * (D // 2) + dp, H, stride=DH // 2), :])
            base = dp * 2 * H
            wop[base:base + H, c * 128:(c + 1) * 128] = lo.astype(BF16)
            wop[base + H:base + 2 * H, c * 128:(c + 1) * 128] = hi.astype(BF16)

    def prep_c(c, r0):
        src = pl.ds(pl.multiple_of(r0, 16), D // G)
        dst = pl.ds(pl.multiple_of(r0 + 64, 16), D // G)
        sl = slice(c * 128, min(D, (c + 1) * 128))
        xr = cre[src, sl].astype(F32)
        xi = cim[src, sl].astype(F32)
        cr, ci = co_re[:, sl], co_im[:, sl]
        yr, yi = xr * cr - xi * ci, -(xr * ci + xi * cr)
        if c < 3:
            cst[dst, c * 256:c * 256 + 128] = yr.astype(BF16)
            cst[dst, c * 256 + 128:c * 256 + 256] = yi.astype(BF16)
        else:
            cst[dst, 768:896] = jnp.concatenate([yr, yi], axis=1).astype(BF16)

    def xb_tasks(g):
        ts = [xb_cp[g].wait]
        for c in range(4):
            ts.append(partial(_transpose_x, xbt, xbn, c, g * TG, TG))
            for rho in range(R // 2):
                ts.append(partial(_gather_rows, xbn, xbp, c, g * (TG // 2), rho, JG,
                                  g * TG + rho * 2 * JG))
        return ts

    def bu_piece(g, n):
        if g == 0 and n % 2 == 0:
            b_cp[n].wait()
            b_cp[n + 1].wait()
        bu[g * TG:(g + 1) * TG, n * 128:(n + 1) * 128] = lax.dot_general(
            xbp[g * TG:(g + 1) * TG, 0:D], bst[n * 128:(n + 1) * 128, :], NT,
            preferred_element_type=F32)

    first = xb_tasks(0)
    first[0]()
    for cp in (w_cp, xa_cp, cre_cp, cim_cp, wo_cp):
        cp.start()
    for t in first[1:]:
        t()
    w_tasks = [w_cp.wait] + [partial(w_transpose, n) for n in range(11)]
    w_tasks += [partial(w_gather, part, c) for part in range(3) for c in range(4)]
    xa_tasks = [xa_cp.wait]
    for c in range(4):
        xa_tasks += [partial(_transpose_x, xat, xan, c, g * TG, TG) for g in range(G)]
        xa_tasks += [partial(_gather_rows, xan, xap, c, 0, rho, 128, rho * 256)
                     for rho in range(R // 2)]
    side = [xb_tasks(1), xb_tasks(2) + w_tasks[:12], w_tasks[12:] + xb_tasks(3) + xa_tasks[:13],
            xa_tasks[13:] + [wo_cp.wait] + [partial(prep_wo, c) for c in range(4)]]
    for g in range(G):
        _interleave([partial(bu_piece, g, n) for n in range(7)], side[g])

    row = lax.broadcasted_iota(jnp.int32, (JG, 128), 0)
    hu = h_s.bitcast(U32)

    zero = jnp.zeros((JG, 128), F32)

    def scan_chunk(g, c, prev):
        if True:
            nparts = 2 if c < 3 else 1

            def load(r):
                v = tuple(
                    bu[pl.ds(pl.multiple_of(g * TG + r * JG, JG), JG),
                       c * 256 + k * 128:c * 256 + (k + 1) * 128]
                    for k in range(nparts))
                return v if c < 3 else (v[0], pltpu.roll(v[0], 64, 1))

            f = gate(load(0))
            for r in range(1, R):
                f = _step(lam1[c], f, gate(load(r)))
            s = tuple(pltpu.roll(jnp.where(row == JG - 1, p, x), 1, 0)
                      for p, x in zip(prev, f))
            for m in range(5):
                sh = tuple(jnp.where(row >= 2 ** m, pltpu.roll(x, 2 ** m, 0), 0.0) for x in s)
                s = _step(lam_pows[m][c], sh, s)
            for rho in range(R // 2):
                e = _step(lam1[c], s, gate(load(2 * rho)))
                s = _step(lam1[c], e, load(2 * rho + 1))
                for k in range(nparts):
                    hu[(2 * c + k) * G + g, pl.ds(rho, JG, stride=R // 2), :] = pltpu.bitcast(_pack(e[k], s[k]), U32)
            return s

    def qkv_part(r, part):
        dst, i = ((q_s, r), (k_s, R + r), (v_s, R + r))[part]
        xr = xap[pl.ds(pl.multiple_of(r * 128, 128), 128), :]
        res = lax.dot_general(wt[part * D:(part + 1) * D, 0:D], xr[:, 0:D],
                                 NT, preferred_element_type=F32)
        dst[i] = res
        cur[0] = res

    def shift_kv(r):
        k_s[r] = pltpu.roll(k_s[R + r], 1, 1)
        v_s[r] = pltpu.roll(v_s[R + r], 1, 1)

    def phase2a(g, prev):
        last = []
        for i in range(2):
            r = 4 * g + 2 * i
            pace([partial(qkv_part, r, k) for k in (1, 2, 0)], 16)
            last.append(scan_chunk(g, 2 * i, prev[2 * i]))
            last.append(scan_chunk(g, 2 * i + 1, prev[2 * i + 1]))
            shift_kv(r)
        return tuple(last)

    lax.fori_loop(0, G, phase2a, ((zero, zero),) * 4)

    lane_h = lax.broadcasted_iota(jnp.int32, (H, 128), 1)
    scale = DH ** -0.5
    z64 = jnp.zeros((1, 64), F32)
    dsk = jnp.concatenate([z64, dsk_ref[...].astype(F32).reshape(1, D)], axis=1)

    def attend(r, odd):
        acc = [None] * W
        for d in range(DH):
            rows = slice(d * H, (d + 1) * H)
            qd = gate((q_s[r, rows, :],))[0]
            for w in range(W):
                t = qd * k_s[R + r - 2 * w, rows, :]
                acc[w] = t if d == 0 else acc[w] + t
        lg = []
        for w in range(W):
            first = jnp.where(r < 2 * w, 1, 0)
            lg.append(jnp.where(lane_h < first, -1e9, acc[w] * scale))
        m = lg[0]
        for w in range(1, W):
            m = jnp.maximum(m, lg[w])
        e = [jnp.exp(x - m) for x in lg]
        tot = e[0]
        for w in range(1, W):
            tot = tot + e[w]
        inv = 1.0 / tot
        p = [x * inv for x in e]
        for d in range(DH):
            rows = slice(d * H, (d + 1) * H)
            o = p[0] * v_s[R + r, rows, :]
            if odd or d < 26:
                o = gate((o,))[0]
            for w in range(1, W):
                o = o + p[w] * v_s[R + r - 2 * w, rows, :]
            if not odd:
                q_s[r, rows, :] = o
            else:
                ow[rows, :] = pltpu.bitcast(_pack(q_s[r - 1, rows, :], o), U32)

    def y_copy(g):
        rows = pl.ds(pl.multiple_of(g * TG, TG), TG)
        return pltpu.make_async_copy(ob.at[rows, pl.ds(512, 384)],
                                     out_hbm.at[0, rows, pl.ds(512, 384)], sem_out.at[g])

    TY = TG // 2

    def y_piece(g, n, i):
        t0 = pl.multiple_of(g * TG + i * TY, TY)
        hh = jnp.concatenate([h_s[k * G + g, i * TY:(i + 1) * TY, :] for k in range(7)], axis=1)
        y = lax.dot_general(hh, cst[n * 128:(n + 1) * 128, :], NT, preferred_element_type=F32)
        cur[0] = y
        xcur = pltpu.roll(xbn[pl.ds(n * S + t0, TY), :].astype(F32), 64, 1)
        if n > 0:
            xcur = jnp.where(lane < 64,
                             pltpu.roll(xbn[pl.ds((n - 1) * S + t0, TY), :].astype(F32), 64, 1), xcur)
        ob[pl.ds(t0, TY), 384 + n * 128:512 + n * 128] = y + xcur * dsk[:, n * 128:(n + 1) * 128]
        if n == 3 and i == 1:
            y_copy(g).start()

    ow[D:512, :] = jnp.zeros((512 - D, 128), U32)
    cre_cp.wait()
    cim_cp.wait()

    def phase2b(g, carry):
        for i in range(2):
            r = 4 * g + 2 * i

            pace([partial(qkv_part, r + 1, k) for k in (1, 2, 0)], 18)
            attend(r, False)
            shift_kv(r + 1)
            prep_c(2 * i, g * (D // G))
            prep_c(2 * i + 1, g * (D // G))
        return carry

    lax.fori_loop(0, G, phase2b, 0)

    def phase3(g, carry):
        for i in range(2):
            pace([partial(y_piece, g, 2 * i + k // 2, k % 2) for k in range(4)], 14)
            attend(4 * g + 2 * i + 1, True)
            for c in range(4):
                dst = pl.ds(pl.multiple_of(c * (S // 2) + (2 * g + i) * 128, 128), 128)
                o_s[dst, :] = ow[c * 128:(c + 1) * 128, :].T
        return carry

    lax.fori_loop(0, G, phase3, 0)

    TA = 256
    wo_b = wop[...]

    def a_copy(i):
        rows = pl.ds(i * TA, TA)
        return pltpu.make_async_copy(ob.at[rows, pl.ds(0, 512)],
                                     out_hbm.at[0, rows, pl.ds(0, 512)], sem_out.at[G + i])

    for i in range(S // TA):
        rows = slice(i * TA, (i + 1) * TA)
        oo = jnp.concatenate([
            pltpu.bitcast(jnp.concatenate(
                [o_s[pl.ds(c * (S // 2) + i * (TA // R) + j, R // 2, stride=128), :]
                 for j in range(TA // R)], axis=0), BF16)
            for c in range(4)], axis=1)
        a = jnp.dot(oo, wo_b, preferred_element_type=F32)
        ob[rows, 0:384] = a[:, 0:384]
        ob[rows, 384:512] = ob[rows, 384:512] + a[:, 384:512]
        a_copy(i).start()

    for g in range(G):
        y_copy(g).wait()
    for i in range(S // TA):
        a_copy(i).wait()


@jax.jit
def pallas_concat_heads__sliding_local_dilated__ssm_conv_s5__prompt_kernel(
    A_x, A_wqkv, A_wo, B_x, B_Lambda_re, B_Lambda_im, B_B_re, B_B_im, B_C_re, B_C_im,
    B_log_dt, B_Dskip,
):
    hbm = pl.BlockSpec(memory_space=pl.ANY)
    vec = pl.BlockSpec(memory_space=pltpu.VMEM)
    vm = pltpu.VMEM
    scratch = [
        vm((512, S), BF16), vm((512, S), BF16),
        vm((4 * S, 128), BF16), vm((4 * S, 128), BF16),
        vm((S, 512), BF16), vm((S, 512), BF16),
        vm((2 * D, D), BF16),
        vm((S, 2 * D), F32),
        vm((D, 3 * D), BF16),
        vm((4 * 1408, 128), BF16),
        vm((3 * D, 512), BF16),
        vm((R, D, 128), F32),
        vm((2 * R, D, 128), F32), vm((2 * R, D, 128), F32),
        vm((7 * G, TG, 128), BF16),
        vm((4 * (S // 2), 128), U32),
        vm((D, D), BF16), vm((D, D), BF16),
        vm((512, 2 * D), BF16),
        vm((D, D), BF16), vm((4 * D, 128), BF16), vm((512, 512), BF16),
        vm((512, 128), U32),
        vm((S, 2 * D), F32),
        pltpu.SemaphoreType.DMA((G,)), pltpu.SemaphoreType.DMA((4,)),
        pltpu.SemaphoreType.DMA((5,)), pltpu.SemaphoreType.DMA((G + 8,)),
    ]
    return pl.pallas_call(
        _kernel,
        out_shape=jax.ShapeDtypeStruct((1, S, 2 * D), F32),
        in_specs=[hbm, hbm, hbm, hbm, vec, vec, hbm, hbm, hbm, hbm, vec, vec],
        out_specs=hbm,
        scratch_shapes=scratch,
        compiler_params=pltpu.CompilerParams(vmem_limit_bytes=100 * 1024 * 1024),
    )(jnp.swapaxes(A_x, 1, 2), A_wqkv, A_wo, jnp.swapaxes(B_x, 1, 2), B_Lambda_re, B_Lambda_im,
      B_B_re, B_B_im, B_C_re, B_C_im, B_log_dt, B_Dskip)
```

```python
from functools import partial

import jax
import jax.numpy as jnp
from jax import lax
import jax.experimental.pallas as pl
import jax.experimental.pallas.tpu as pltpu

S = 2048
D = 448
H = 16
DH = 28
W = 8
R = 16
G = 4
TG = S // G
JG = TG // R
TP = 128
NP = S // TP

F32 = jnp.float32
BF16 = jnp.bfloat16
U32 = jnp.uint32
NT = (((1,), (1,)), ((), ()))


def _unpack(w):
    lo = pltpu.bitcast(w.astype(jnp.uint16), U32)
    hi = pltpu.bitcast((w >> 16).astype(jnp.uint16), U32)
    return lo, hi


def _pack(even, odd):
    return pltpu.bitcast(pltpu.pack_elementwise([even, odd], packed_dtype=BF16), U32)


def _words(x):
    return pltpu.bitcast(x.astype(BF16), U32)


def _bf16(w, cols=None):
    x = pltpu.bitcast(w, BF16)
    return x if cols is None else x[:, :cols]


def _ds(start, size, align=None):
    return pl.ds(pl.multiple_of(start, align or size), size)


def _step(lam, h, b):
    lr, li = lam
    return (lr * h[0] - li * h[1] + b[0], lr * h[1] + li * h[0] + b[1])


def _lam_tiles(re, im, lane):
    out = [(re[:, c * 128:(c + 1) * 128], im[:, c * 128:(c + 1) * 128]) for c in range(3)]
    z = jnp.zeros((1, 64), F32)
    r3 = jnp.concatenate([re[:, 384:], z], axis=1)
    i3 = jnp.concatenate([im[:, 384:], z], axis=1)
    out.append((jnp.where(lane < 64, r3, pltpu.roll(r3, 64, 1)),
                jnp.where(lane < 64, i3, -pltpu.roll(i3, 64, 1))))
    return out


class _Pacer:
    def __init__(self):
        self.zero = lax.broadcasted_iota(U32, (8, 128), 1) >> 16

    def pace(self, matmuls, steps):
        self.queue = list(matmuls)
        self.per = -(-steps // len(matmuls))
        self.pos = 0

    def gate(self, *xs):
        i = self.pos % self.per
        if i == 0:
            self.res = self.queue.pop(0)()
        self.pos += 1
        k = (self.res.shape[0] // 8 * i) // self.per * 8
        tok = pltpu.bitcast(self.res[k:k + 8, 0:128], U32) & self.zero
        out = []
        for x in xs:
            u = pltpu.bitcast(x, U32)
            u = u | jnp.tile(tok, (u.shape[0] // 8, u.shape[1] // 128))
            out.append(pltpu.bitcast(u, x.dtype))
        return out if len(out) > 1 else out[0]

    def finish(self):
        while self.queue:
            self.queue.pop(0)()


def _kernel(xa_hbm, wqkv_hbm, wo_hbm, xb_hbm, lre_hbm, lim_hbm, bre_hbm, bim_hbm,
            cre_hbm, cim_hbm, ldt_hbm, dsk_hbm, out_hbm,
            lre, lim, ldt, dsk, xat, xbt, xan, xbn, xap, xbp, bst, bu, wraw, wtn, wt,
            q_s, k_s, v_s, h_s, o_s, cre, cim, cst, woraw, won, wop, wot, ow, dcol, ylow, ob,
            sem_xb, sem_b, sem_in, sem_out):
    copy = pltpu.make_async_copy
    xb_cp = [copy(xb_hbm.at[0, :, pl.ds(g * TG, TG)], xbt.at[pl.ds(0, D), pl.ds(g * TG, TG)],
                  sem_xb.at[g]) for g in range(G)]
    b_cp = []
    for c in range(3):
        b_cp.append([copy(bre_hbm.at[pl.ds(c * 128, 128)], bst.at[pl.ds(c * 256, 128)], sem_b.at[2 * c])])
        b_cp.append([copy(bim_hbm.at[pl.ds(c * 128, 128)], bst.at[pl.ds(c * 256 + 128, 128)],
                          sem_b.at[2 * c + 1])])
    b_cp.append([copy(bre_hbm.at[pl.ds(384, 64)], bst.at[pl.ds(768, 64)], sem_b.at[6]),
                 copy(bim_hbm.at[pl.ds(384, 64)], bst.at[pl.ds(832, 64)], sem_b.at[6])])
    p_cp = [copy(src, dst, sem_in.at[5]) for src, dst in
            ((lre_hbm, lre), (lim_hbm, lim), (ldt_hbm, ldt), (dsk_hbm, dsk))]
    w_cp = copy(wqkv_hbm, wraw, sem_in.at[0])
    xa_cp = copy(xa_hbm.at[0], xat.at[pl.ds(0, D)], sem_in.at[1])
    c_cp = [copy(cre_hbm, cre, sem_in.at[2]), copy(cim_hbm, cim, sem_in.at[3])]
    wo_cp = [copy(wo_hbm.at[:, pl.ds(c * 128, 128)], won.at[c], sem_in.at[4]) for c in range(3)]
    wo_cp.append(copy(wo_hbm, woraw, sem_in.at[4]))

    for cp in [xb_cp[0]] + b_cp[0] + p_cp + b_cp[1]:
        cp.start()

    xat[D:512, :] = jnp.zeros((512 - D, S), BF16)
    xbt[D:512, :] = jnp.zeros((512 - D, S), BF16)
    ow[D:512, :] = jnp.zeros((512 - D, 128), U32)
    pacer = _Pacer()
    gate = pacer.gate

    def transpose_x(xt_ref, xn_ref, c, g):
        xn_ref[pl.ds(c * S + g * TG, TG), :] = gate(xt_ref[c * 128:(c + 1) * 128, g * TG:(g + 1) * TG]).T

    def gather_x(xn_ref, xp_ref, c, row0, rhos, nj):
        xu = xn_ref.bitcast(U32)
        for rho in rhos:
            lo, hi = _unpack(xu[pl.ds(c * (S // 2) + row0 + rho, nj, stride=R // 2), :])
            dst = row0 + rho * nj
            xp_ref[dst:dst + nj // 2, c * 128:(c + 1) * 128] = lo
            xp_ref[dst + nj // 2:dst + nj, c * 128:(c + 1) * 128] = hi

    def w_transpose(n):
        cols = min(128, 3 * D - n * 128)
        for c in range(4):
            rows = min(128, D - c * 128)
            v = wraw[c * 128:c * 128 + rows, n * 128:n * 128 + cols]
            if rows < 128:
                v = jnp.concatenate([v, jnp.zeros((128 - rows, cols), BF16)], axis=0)
            if cols < 128:
                v = jnp.concatenate([v, jnp.zeros((128, 128 - cols), BF16)], axis=1)
            wtn[pl.ds(c * 1408 + n * 128, 128), :] = (gate(v) if c == 0 else v).T

    def w_gather(part, c):
        wu = wtn.bitcast(U32)
        for dp in range(DH // 2):
            lo, hi = _unpack(wu[pl.ds(c * 704 + part * (D // 2) + dp, H, stride=DH // 2), :])
            base = part * (D // 2) + dp * H
            wt[base:base + H // 2, c * 128:(c + 1) * 128] = lo
            wt[base + H // 2:base + H, c * 128:(c + 1) * 128] = hi

    def bu_piece(g, n):
        if g == 0:
            for cp in b_cp[n]:
                cp.wait()
        res = lax.dot_general(_bf16(xbp[g * TG // 2:(g + 1) * TG // 2, :], D),
                              bst[n * 128:(n + 1) * 128, :], NT, preferred_element_type=F32)
        bu[g * TG:(g + 1) * TG, n * 128:(n + 1) * 128] = res
        return res

    def prep_xb(g):
        xb_cp[g].wait()
        for c in range(4):
            transpose_x(xbt, xbn, c, g)
            gather_x(xbn, xbp, c, g * (TG // 2), range(R // 2), JG)

    def prep_xa(cs):
        for c in cs:
            for g in range(G):
                transpose_x(xat, xan, c, g)
            gather_x(xan, xap, c, 0, range(R // 2), 128)

    xb_cp[0].wait()
    for cp in sum(b_cp[2:], []) + [xb_cp[1], w_cp, xb_cp[2]]:
        cp.start()
    for c in range(4):
        xbn[pl.ds(c * S, TG), :] = xbt[c * 128:(c + 1) * 128, 0:TG].T
        gather_x(xbn, xbp, c, 0, range(R // 2), JG)

    for cp in p_cp:
        cp.wait()
    lane = lax.broadcasted_iota(jnp.int32, (1, 128), 1)
    a_re = lre[...].astype(F32).reshape(1, D)
    a_im = lim[...].astype(F32).reshape(1, D)
    dt = jnp.exp(ldt[...].astype(F32).reshape(1, D)).astype(BF16).astype(F32)
    mag = jnp.exp(dt * a_re)
    l_re = mag * jnp.cos(dt * a_im)
    l_im = mag * jnp.sin(dt * a_im)
    den = a_re * a_re + a_im * a_im
    n_re = l_re - 1.0
    co_re = 2.0 * (n_re * a_re + l_im * a_im) / den
    co_im = 2.0 * (l_im * a_re - n_re * a_im) / den
    lam1 = _lam_tiles(l_re, l_im, lane)
    p_re, p_im = l_re, l_im
    for _ in range(4):
        p_re, p_im = p_re * p_re - p_im * p_im, 2.0 * p_re * p_im
    lam_pows = []
    for _ in range(5):
        lam_pows.append(_lam_tiles(p_re, p_im, lane))
        p_re, p_im = p_re * p_re - p_im * p_im, 2.0 * p_re * p_im
    drow = jnp.concatenate([dsk[...].astype(F32).reshape(1, D), jnp.zeros((1, 64), F32)], axis=1)
    dcol[...] = jnp.broadcast_to(drow, (128, 512)).T

    def bu_chunk(g, steps):
        pacer.pace([partial(bu_piece, g, n) for n in range(7)], steps)

    bu_chunk(0, 7)
    for _ in range(3):
        gate(pacer.zero)
    prep_xb(1)
    pacer.finish()

    for cp in (xa_cp, xb_cp[3]):
        cp.start()
    bu_chunk(1, 14)
    w_cp.wait()
    for n in range(7):
        w_transpose(n)
    prep_xb(2)
    for n in range(7, 10):
        w_transpose(n)
    for part in range(2):
        for c in range(4):
            w_gather(part, c)
    pacer.finish()

    for cp in wo_cp + c_cp:
        cp.start()
    bu_chunk(2, 13)
    xa_cp.wait()
    w_transpose(10)
    prep_xb(3)
    for c in range(4):
        w_gather(2, c)
    prep_xa([0, 1])
    pacer.finish()

    bu_chunk(3, 10)
    for cp in wo_cp:
        cp.wait()
    won[3] = jnp.concatenate([woraw[:, 384:D], jnp.zeros((D, 64), BF16)], axis=1)
    prep_xa([2, 3])
    pacer.finish()

    row = lax.broadcasted_iota(jnp.int32, (JG, 128), 0)
    hu = h_s.bitcast(U32)

    def scan_chunk(g, c, prev):
        nparts = 2 if c < 3 else 1

        def load(r):
            v = [bu[_ds(g * TG + r * JG, JG), c * 256 + k * 128:c * 256 + (k + 1) * 128]
                 for k in range(nparts)]
            return v if c < 3 else (v[0], pltpu.roll(v[0], 64, 1))

        f = gate(*load(0))
        for r in range(1, R):
            f = _step(lam1[c], f, gate(*load(r)))
        s = tuple(pltpu.roll(jnp.where(row == JG - 1, p, x), 1, 0) for p, x in zip(prev, f))
        for m in range(5):
            sh = tuple(jnp.where(row >= 2 ** m, pltpu.roll(x, 2 ** m, 0), 0.0) for x in s)
            s = _step(lam_pows[m][c], sh, s)
        for rho in range(R // 2):
            e = _step(lam1[c], s, gate(*load(2 * rho)))
            s = _step(lam1[c], e, load(2 * rho + 1))
            for k in range(nparts):
                hu[(2 * c + k) * G + g, pl.ds(rho, JG, stride=R // 2), :] = _pack(e[k], s[k])
        return s

    def qkv_part(r, part):
        dst, i = ((q_s, r), (k_s, R + r), (v_s, R + r))[part]
        res = lax.dot_general(_bf16(wt[part * D // 2:(part + 1) * D // 2, :], D),
                              _bf16(xap[_ds(r * 64, 64), :], D), NT, preferred_element_type=F32)
        dst[i] = res
        return res

    def shift_kv(r):
        k_s[r] = pltpu.roll(k_s[R + r], 1, 1)
        v_s[r] = pltpu.roll(v_s[R + r], 1, 1)

    def prep_wo(c):
        wu = won.bitcast(U32)
        for dp in range(DH // 2):
            lo, hi = _unpack(wu[c, pl.ds(dp, H, stride=DH // 2), :])
            wop[dp * H:dp * H + H // 2, :] = lo
            wop[dp * H + H // 2:(dp + 1) * H, :] = hi
        wop[D // 2:256, :] = jnp.zeros((256 - D // 2, 128), U32)
        wot[_ds(c * 64, 64), :] = pltpu.bitcast(_bf16(wop[...]).T, U32)

    def phase2a(g, prev):
        last = []
        for i in range(2):
            r = 4 * g + 2 * i
            pacer.pace([partial(qkv_part, r, k) for k in (1, 2, 0)], 48)
            last.append(scan_chunk(g, 2 * i, prev[2 * i]))
            last.append(scan_chunk(g, 2 * i + 1, prev[2 * i + 1]))
            shift_kv(r)
        prep_wo(g)
        return tuple(last)

    zero = jnp.zeros((JG, 128), F32)
    lax.fori_loop(0, G, phase2a, ((zero, zero),) * 4)

    lane_h = lax.broadcasted_iota(jnp.int32, (H, 128), 1)
    scale = DH ** -0.5

    def attend(r, odd):
        acc = [None] * W
        for d in range(DH):
            rows = slice(d * H, (d + 1) * H)
            qd = gate(q_s[r, rows, :])
            for w in range(W):
                t = qd * k_s[R + r - 2 * w, rows, :]
                acc[w] = t if d == 0 else acc[w] + t
        lg = []
        for w in range(W):
            first = jnp.where(r < 2 * w, 1, 0)
            lg.append(jnp.where(lane_h < first, -1e9, acc[w] * scale))
        m = lg[0]
        for w in range(1, W):
            m = jnp.maximum(m, lg[w])
        e = [jnp.exp(x - m) for x in lg]
        tot = e[0]
        for w in range(1, W):
            tot = tot + e[w]
        inv = 1.0 / tot
        p = [x * inv for x in e]
        for d in range(DH):
            rows = slice(d * H, (d + 1) * H)
            o = gate(p[0] * v_s[R + r, rows, :])
            for w in range(1, W):
                o = o + p[w] * v_s[R + r - 2 * w, rows, :]
            if odd:
                ow[rows, :] = _pack(q_s[r - 1, rows, :], o)
            else:
                q_s[r, rows, :] = o

    def prep_c(r0):
        src, dst = _ds(r0, D // G, 16), _ds(r0 // 2, D // G // 2, 8)
        for c in range(4):
            sl = slice(c * 128, min(D, (c + 1) * 128))
            xr, xi = cre[src, sl].astype(F32), cim[src, sl].astype(F32)
            cr, ci = co_re[:, sl], co_im[:, sl]
            yr, yi = xr * cr - xi * ci, -(xr * ci + xi * cr)
            if c < 3:
                cst[dst, c * 256:c * 256 + 128] = _words(yr)
                cst[dst, c * 256 + 128:c * 256 + 256] = _words(yi)
            else:
                cst[dst, 768:896] = _words(jnp.concatenate([yr, yi], axis=1))

    for cp in c_cp:
        cp.wait()

    def phase2b(g, carry):
        for i in range(2):
            r = 4 * g + 2 * i
            pacer.pace([partial(qkv_part, r + 1, k) for k in (1, 2, 0)], 2 * DH + 1)
            attend(r, False)
            shift_kv(r + 1)
        prep_c(g * (D // G))
        return carry

    lax.fori_loop(0, G, phase2b, 0)

    def y_copy(i):
        rows = _ds(i * TP, TP)
        return copy(ob.at[rows, pl.ds(512, 384)], out_hbm.at[0, rows, pl.ds(512, 384)], sem_out.at[i])

    def a_copy(i):
        rows = _ds(i * TP, TP)
        return copy(ob.at[rows, pl.ds(0, 512)], out_hbm.at[0, rows, pl.ds(0, 512)], sem_out.at[NP + i])

    def y_piece(i):
        rows = _ds(i * TP, TP)
        sub = _ds((i % (TG // TP)) * TP, TP)
        hh = jnp.concatenate([h_s[k * G + i // (TG // TP), sub, :] for k in range(7)], axis=1)
        res = lax.dot_general(_bf16(cst[...]), hh, NT, preferred_element_type=F32)
        y = res + xbt[0:D, rows] * dcol[0:D, :]
        ylow[i] = y[0:64]
        for n in range(3):
            ob[rows, 512 + n * 128:640 + n * 128] = y[64 + n * 128:192 + n * 128].T
        y_copy(i).start()
        return res

    def phase3(g, carry):
        pacer.pace([partial(y_piece, 3 * g + k) for k in range(3)], 4 * DH + 8)
        for i in range(2):
            attend(4 * g + 2 * i + 1, True)
            for c in range(4):
                o_s[c * NP:(c + 1) * NP, _ds((2 * g + i) * 8, 8), :] = (
                    ow[c * 128:(c + 1) * 128, :].T.reshape(NP, 8, 128))
        pacer.finish()
        return carry

    lax.fori_loop(0, G, phase3, 0)

    def a_piece(i):
        rows = _ds(i * TP, TP)
        oo = jnp.concatenate([
            _bf16(jnp.concatenate(
                [o_s[c * NP + i, pl.ds(j, R // 2, stride=8), :]
                 for j in range(TP // R)], axis=0))
            for c in range(4)], axis=1)
        a = lax.dot_general(_bf16(wot[0:D // 2, :]), oo, NT, preferred_element_type=F32)
        for n in range(3):
            ob[rows, n * 128:(n + 1) * 128] = a[n * 128:(n + 1) * 128].T
        ob[rows, 384:512] = jnp.concatenate([a[384:D], ylow[i]], axis=0).T
        a_copy(i).start()

    def phase4(g, carry):
        y_piece(3 * G + g)
        for k in range(NP // G):
            a_piece(g * (NP // G) + k)
        return carry

    lax.fori_loop(0, G, phase4, 0)
    for i in range(NP):
        y_copy(i).wait()
        a_copy(i).wait()


@jax.jit
def pallas_concat_heads__sliding_local_dilated__ssm_conv_s5__prompt_kernel(
    A_x, A_wqkv, A_wo, B_x, B_Lambda_re, B_Lambda_im, B_B_re, B_B_im, B_C_re, B_C_im,
    B_log_dt, B_Dskip,
):
    hbm = pl.BlockSpec(memory_space=pl.ANY)
    vm = pltpu.VMEM
    dma = pltpu.SemaphoreType.DMA
    scratch = [vm((D,), BF16)] * 4 + [
        vm((512, S), BF16), vm((512, S), BF16),
        vm((4 * S, 128), BF16), vm((4 * S, 128), BF16),
        vm((S // 2, 512), U32), vm((S // 2, 512), U32),
        vm((2 * D, D), BF16),
        vm((S, 2 * D), F32),
        vm((D, 3 * D), BF16),
        vm((4 * 1408, 128), BF16),
        vm((3 * D // 2, 512), U32),
        vm((R, D, 128), F32),
        vm((2 * R, D, 128), F32), vm((2 * R, D, 128), F32),
        vm((7 * G, TG, 128), BF16),
        vm((4 * NP, TP // 2, 128), U32),
        vm((D, D), BF16), vm((D, D), BF16),
        vm((D // 2, 2 * D), U32),
        vm((D, D), BF16), vm((4, D, 128), BF16),
        vm((256, 128), U32), vm((256, 512), U32),
        vm((512, 128), U32),
        vm((512, 128), F32),
        vm((NP, 64, 128), F32),
        vm((S, 2 * D), F32),
        dma((G,)), dma((7,)), dma((6,)), dma((2 * NP,)),
    ]
    return pl.pallas_call(
        _kernel,
        out_shape=jax.ShapeDtypeStruct((1, S, 2 * D), F32),
        in_specs=[hbm] * 12,
        out_specs=hbm,
        scratch_shapes=scratch,
        compiler_params=pltpu.CompilerParams(vmem_limit_bytes=100 * 1024 * 1024),
    )(jnp.swapaxes(A_x, 1, 2), A_wqkv, A_wo, jnp.swapaxes(B_x, 1, 2), B_Lambda_re, B_Lambda_im,
      B_B_re, B_B_im, B_C_re, B_C_im, B_log_dt, B_Dskip)
```

```python
from functools import partial

import jax
import jax.numpy as jnp
from jax import lax
import jax.experimental.pallas as pl
import jax.experimental.pallas.tpu as pltpu

S = 2048
D = 448
H = 16
DH = 28
W = 8
R = 16
G = 4
TG = S // G
JG = TG // R
TP = 128
NP = S // TP

F32 = jnp.float32
BF16 = jnp.bfloat16
U32 = jnp.uint32
NT = (((1,), (1,)), ((), ()))


def _unpack(w):
    lo = pltpu.bitcast(w.astype(jnp.uint16), U32)
    hi = pltpu.bitcast((w >> 16).astype(jnp.uint16), U32)
    return lo, hi


def _pack(even, odd):
    return pltpu.bitcast(pltpu.pack_elementwise([even, odd], packed_dtype=BF16), U32)


def _words(x):
    return pltpu.bitcast(x.astype(BF16), U32)


def _bf16(w, cols=None):
    x = pltpu.bitcast(w, BF16)
    return x if cols is None else x[:, :cols]


def _ds(start, size, align=None):
    return pl.ds(pl.multiple_of(start, align or size), size)


def _step(lam, h, b):
    lr, li = lam
    return (lr * h[0] - li * h[1] + b[0], lr * h[1] + li * h[0] + b[1])


def _lam_tiles(re, im, lane):
    out = [(re[:, c * 128:(c + 1) * 128], im[:, c * 128:(c + 1) * 128]) for c in range(3)]
    z = jnp.zeros((1, 64), F32)
    r3 = jnp.concatenate([re[:, 384:], z], axis=1)
    i3 = jnp.concatenate([im[:, 384:], z], axis=1)
    out.append((jnp.where(lane < 64, r3, pltpu.roll(r3, 64, 1)),
                jnp.where(lane < 64, i3, -pltpu.roll(i3, 64, 1))))
    return out


class _Pacer:
    def __init__(self):
        self.zero = lax.broadcasted_iota(U32, (8, 128), 1) >> 16

    def pace(self, matmuls, steps):
        self.queue = list(matmuls)
        self.per = -(-steps // len(matmuls))
        self.pos = 0

    def gate(self, *xs):
        i = self.pos % self.per
        if i == 0:
            self.res = self.queue.pop(0)()
        self.pos += 1
        k = (self.res.shape[0] // 8 * i) // self.per * 8
        tok = pltpu.bitcast(self.res[k:k + 8, 0:128], U32) & self.zero
        out = []
        for x in xs:
            u = pltpu.bitcast(x, U32)
            u = u | jnp.tile(tok, (u.shape[0] // 8, u.shape[1] // 128))
            out.append(pltpu.bitcast(u, x.dtype))
        return out if len(out) > 1 else out[0]

    def finish(self):
        while self.queue:
            self.queue.pop(0)()


def _loop(body, init, unroll=2):
    def outer(t, carry):
        for u in range(unroll):
            carry = body(t * unroll + u, carry)
        return carry
    return lax.fori_loop(0, G // unroll, outer, init)


def _kernel(xa_hbm, wqkv_hbm, wo_hbm, xb_hbm, lre_hbm, lim_hbm, bre_hbm, bim_hbm,
            cre_hbm, cim_hbm, ldt_hbm, dsk_hbm, out_hbm,
            lre, lim, ldt, dsk, xat, xbt, xan, xbn, xap, xbp, bst, bu, wraw, wtn, wt,
            q_s, k_s, v_s, h_s, o_s, cre, cim, cst, woraw, won, wop, wot, ow, dcol, ylow, ob,
            sem_xb, sem_b, sem_in, sem_out):
    copy = pltpu.make_async_copy
    xb_cp = [copy(xb_hbm.at[0, :, pl.ds(g * TG, TG)], xbt.at[pl.ds(0, D), pl.ds(g * TG, TG)],
                  sem_xb.at[g]) for g in range(G)]
    b_cp = []
    for c in range(3):
        b_cp.append([copy(bre_hbm.at[pl.ds(c * 128, 128)], bst.at[pl.ds(c * 256, 128)], sem_b.at[2 * c])])
        b_cp.append([copy(bim_hbm.at[pl.ds(c * 128, 128)], bst.at[pl.ds(c * 256 + 128, 128)],
                          sem_b.at[2 * c + 1])])
    b_cp.append([copy(bre_hbm.at[pl.ds(384, 64)], bst.at[pl.ds(768, 64)], sem_b.at[6]),
                 copy(bim_hbm.at[pl.ds(384, 64)], bst.at[pl.ds(832, 64)], sem_b.at[6])])
    p_cp = [copy(src, dst, sem_in.at[5]) for src, dst in
            ((lre_hbm, lre), (lim_hbm, lim), (ldt_hbm, ldt), (dsk_hbm, dsk))]
    w_cp = copy(wqkv_hbm, wraw, sem_in.at[0])
    xa_cp = copy(xa_hbm.at[0], xat.at[pl.ds(0, D)], sem_in.at[1])
    c_cp = [copy(cre_hbm, cre, sem_in.at[2]), copy(cim_hbm, cim, sem_in.at[3])]
    wo_cp = [copy(wo_hbm.at[:, pl.ds(c * 128, 128)], won.at[c], sem_in.at[4]) for c in range(3)]
    wo_cp.append(copy(wo_hbm, woraw, sem_in.at[4]))

    for cp in [xb_cp[0]] + sum(b_cp, []) + p_cp:
        cp.start()

    xat[D:512, :] = jnp.zeros((512 - D, S), BF16)
    xbt[D:512, :] = jnp.zeros((512 - D, S), BF16)
    ow[D:512, :] = jnp.zeros((512 - D, 128), U32)
    pacer = _Pacer()
    gate = pacer.gate

    def transpose_x(xt_ref, xn_ref, c, g):
        for t in range(g * TG, (g + 1) * TG, 128):
            xn_ref[pl.ds(c * S + t, 128), :] = gate(xt_ref[c * 128:(c + 1) * 128, t:t + 128]).T

    def gather_x(xn_ref, xp_ref, c, row0, rhos, nj, g8=gate):
        xu = xn_ref.bitcast(U32)
        for rho in rhos:
            lo, hi = _unpack(g8(xu[pl.ds(c * (S // 2) + row0 + rho, nj, stride=R // 2), :]))
            dst = row0 + rho * nj
            xp_ref[dst:dst + nj // 2, c * 128:(c + 1) * 128] = lo
            xp_ref[dst + nj // 2:dst + nj, c * 128:(c + 1) * 128] = hi

    def w_transpose(n):
        cols = min(128, 3 * D - n * 128)
        for c in range(4):
            rows = min(128, D - c * 128)
            v = wraw[c * 128:c * 128 + rows, n * 128:n * 128 + cols]
            if rows < 128:
                v = jnp.concatenate([v, jnp.zeros((128 - rows, cols), BF16)], axis=0)
            if cols < 128:
                v = jnp.concatenate([v, jnp.zeros((128, 128 - cols), BF16)], axis=1)
            wtn[pl.ds(c * 1408 + n * 128, 128), :] = gate(v).T

    def w_gather(part, c):
        wu = wtn.bitcast(U32)
        for dp in range(DH // 2):
            lo, hi = _unpack(gate(wu[pl.ds(c * 704 + part * (D // 2) + dp, H, stride=DH // 2), :]))
            base = part * (D // 2) + dp * H
            wt[base:base + H // 2, c * 128:(c + 1) * 128] = lo
            wt[base + H // 2:base + H, c * 128:(c + 1) * 128] = hi

    def bu_piece(g, n):
        res = lax.dot_general(_bf16(xbp[g * TG // 2:(g + 1) * TG // 2, :], D),
                              bst[n * 128:(n + 1) * 128, :], NT, preferred_element_type=F32)
        bu[g * TG:(g + 1) * TG, n * 128:(n + 1) * 128] = res
        return res

    def prep_xb(g):
        xb_cp[g].wait()
        for c in range(4):
            transpose_x(xbt, xbn, c, g)
            gather_x(xbn, xbp, c, g * (TG // 2), range(R // 2), JG)

    def prep_xa(cs):
        for c in cs:
            for g in range(G):
                transpose_x(xat, xan, c, g)
            gather_x(xan, xap, c, 0, range(R // 2), 128)

    xb_cp[0].wait()
    for cp in [xb_cp[1], w_cp, xb_cp[2]]:
        cp.start()
    for c in range(4):
        xbn[pl.ds(c * S, TG), :] = xbt[c * 128:(c + 1) * 128, 0:TG].T
        gather_x(xbn, xbp, c, 0, range(R // 2), JG, lambda v: v)

    def bu_chunk(g, steps):
        pacer.pace([partial(bu_piece, g, n) for n in range(7)], steps)

    for cp in b_cp[0] + b_cp[1]:
        cp.wait()
    bu_chunk(0, 70)
    for _ in range(20):
        gate(pacer.zero)
    for cp in sum(b_cp[2:], []):
        cp.wait()
    prep_xb(1)
    for cp in p_cp:
        cp.wait()
    lane = lax.broadcasted_iota(jnp.int32, (1, 128), 1)
    a_re = lre[...].astype(F32).reshape(1, D)
    a_im = lim[...].astype(F32).reshape(1, D)
    dt = jnp.exp(ldt[...].astype(F32).reshape(1, D)).astype(BF16).astype(F32)
    mag = jnp.exp(dt * a_re)
    l_re = mag * jnp.cos(dt * a_im)
    l_im = mag * jnp.sin(dt * a_im)
    den = a_re * a_re + a_im * a_im
    n_re = l_re - 1.0
    co_re = 2.0 * (n_re * a_re + l_im * a_im) / den
    co_im = 2.0 * (l_im * a_re - n_re * a_im) / den
    lam1 = _lam_tiles(l_re, l_im, lane)
    p_re, p_im = l_re, l_im
    for _ in range(4):
        p_re, p_im = p_re * p_re - p_im * p_im, 2.0 * p_re * p_im
    lam_pows = []
    for _ in range(5):
        lam_pows.append(_lam_tiles(p_re, p_im, lane))
        p_re, p_im = p_re * p_re - p_im * p_im, 2.0 * p_re * p_im
    drow = jnp.concatenate([dsk[...].astype(F32).reshape(1, D), jnp.zeros((1, 64), F32)], axis=1)
    dcol[...] = jnp.broadcast_to(drow, (128, 512)).T

    pacer.finish()

    for cp in (xa_cp, xb_cp[3]):
        cp.start()
    bu_chunk(1, 28 + 48 + 12 + 56)
    w_cp.wait()
    for n in range(7):
        w_transpose(n)
    prep_xb(2)
    for n in range(7, 10):
        w_transpose(n)
    for part in range(1):
        for c in range(4):
            w_gather(part, c)
    pacer.finish()

    for cp in wo_cp + c_cp:
        cp.start()
    bu_chunk(2, 4 + 48 + 112 + 24)
    xa_cp.wait()
    w_transpose(10)
    prep_xb(3)
    for c in range(4):
        w_gather(1, c)
        w_gather(2, c)
    prep_xa([0])
    pacer.finish()

    bu_chunk(3, 78)
    for cp in wo_cp:
        cp.wait()
    won[3] = jnp.concatenate([woraw[:, 384:D], jnp.zeros((D, 64), BF16)], axis=1)
    prep_xa([1, 2, 3])
    pacer.finish()

    row = lax.broadcasted_iota(jnp.int32, (JG, 128), 0)
    hu = h_s.bitcast(U32)

    def scan_chunk(g, c, prev):
        nparts = 2 if c < 3 else 1

        def load(r):
            v = [bu[_ds(g * TG + r * JG, JG), c * 256 + k * 128:c * 256 + (k + 1) * 128]
                 for k in range(nparts)]
            return v if c < 3 else (v[0], pltpu.roll(v[0], 64, 1))

        f = gate(*load(0))
        for r in range(1, R):
            f = _step(lam1[c], f, gate(*load(r)))
        s = tuple(pltpu.roll(jnp.where(row == JG - 1, p, x), 1, 0) for p, x in zip(prev, f))
        for m in range(5):
            sh = tuple(jnp.where(row >= 2 ** m, pltpu.roll(x, 2 ** m, 0), 0.0) for x in s)
            s = _step(lam_pows[m][c], sh, s)
        for rho in range(R // 2):
            e = _step(lam1[c], s, gate(*load(2 * rho)))
            s = _step(lam1[c], e, load(2 * rho + 1))
            for k in range(nparts):
                hu[(2 * c + k) * G + g, pl.ds(rho, JG, stride=R // 2), :] = _pack(e[k], s[k])
        return s

    def qkv_part(r, part):
        dst, i = ((q_s, r), (k_s, R + r), (v_s, R + r))[part]
        res = lax.dot_general(_bf16(wt[part * D // 2:(part + 1) * D // 2, :], D),
                              _bf16(xap[_ds(r * 64, 64), :], D), NT, preferred_element_type=F32)
        dst[i] = res
        return res

    def shift_kv(r):
        k_s[r] = pltpu.roll(k_s[R + r], 1, 1)
        v_s[r] = pltpu.roll(v_s[R + r], 1, 1)

    def prep_wo(c):
        wu = won.bitcast(U32)
        for dp in range(DH // 2):
            lo, hi = _unpack(wu[c, pl.ds(dp, H, stride=DH // 2), :])
            wop[dp * H:dp * H + H // 2, :] = lo
            wop[dp * H + H // 2:(dp + 1) * H, :] = hi
        wop[D // 2:256, :] = jnp.zeros((256 - D // 2, 128), U32)
        wot[_ds(c * 64, 64), :] = pltpu.bitcast(_bf16(wop[...]).T, U32)

    def phase2a(g, prev):
        last = []
        for i in range(2):
            r = 4 * g + 2 * i
            pacer.pace([partial(qkv_part, r, k) for k in (1, 2, 0)], 48)
            last.append(scan_chunk(g, 2 * i, prev[2 * i]))
            last.append(scan_chunk(g, 2 * i + 1, prev[2 * i + 1]))
            shift_kv(r)
        prep_wo(g)
        return tuple(last)

    zero = jnp.zeros((JG, 128), F32)
    _loop(phase2a, ((zero, zero),) * 4)

    lane_h = lax.broadcasted_iota(jnp.int32, (H, 128), 1)
    scale = DH ** -0.5

    def attend(r, odd):
        acc = [None] * W
        for d in range(DH):
            rows = slice(d * H, (d + 1) * H)
            qd = gate(q_s[r, rows, :])
            for w in range(W):
                t = qd * k_s[R + r - 2 * w, rows, :]
                acc[w] = t if d == 0 else acc[w] + t
        lg = []
        for w in range(W):
            first = jnp.where(r < 2 * w, 1, 0)
            lg.append(jnp.where(lane_h < first, -1e9, acc[w] * scale))
        m = lg[0]
        for w in range(1, W):
            m = jnp.maximum(m, lg[w])
        e = [jnp.exp(x - m) for x in lg]
        tot = e[0]
        for w in range(1, W):
            tot = tot + e[w]
        inv = 1.0 / tot
        p = [x * inv for x in e]
        for d in range(DH):
            rows = slice(d * H, (d + 1) * H)
            o = gate(p[0] * v_s[R + r, rows, :])
            for w in range(1, W):
                o = o + p[w] * v_s[R + r - 2 * w, rows, :]
            if odd:
                ow[rows, :] = _pack(q_s[r - 1, rows, :], o)
            else:
                q_s[r, rows, :] = o

    def prep_c(r0):
        src, dst = _ds(r0, D // G, 16), _ds(r0 // 2, D // G // 2, 8)
        for c in range(4):
            sl = slice(c * 128, min(D, (c + 1) * 128))
            xr, xi = cre[src, sl].astype(F32), cim[src, sl].astype(F32)
            cr, ci = co_re[:, sl], co_im[:, sl]
            yr, yi = xr * cr - xi * ci, -(xr * ci + xi * cr)
            if c < 3:
                cst[dst, c * 256:c * 256 + 128] = _words(yr)
                cst[dst, c * 256 + 128:c * 256 + 256] = _words(yi)
            else:
                cst[dst, 768:896] = _words(jnp.concatenate([yr, yi], axis=1))

    for cp in c_cp:
        cp.wait()

    def phase2b(g, carry):
        for i in range(2):
            r = 4 * g + 2 * i
            pacer.pace([partial(qkv_part, r + 1, k) for k in (1, 2, 0)], 2 * DH + 1)
            attend(r, False)
            shift_kv(r + 1)
        prep_c(g * (D // G))
        return carry

    for g in range(G):
        phase2b(g, 0)

    def y_copy(i):
        rows = _ds(i * TP, TP)
        return copy(ob.at[rows, pl.ds(512, 384)], out_hbm.at[0, rows, pl.ds(512, 384)], sem_out.at[i])

    def a_copy(i):
        rows = _ds(i * TP, TP)
        return copy(ob.at[rows, pl.ds(0, 512)], out_hbm.at[0, rows, pl.ds(0, 512)], sem_out.at[NP + i])

    def y_piece(i):
        rows = _ds(i * TP, TP)
        sub = _ds((i % (TG // TP)) * TP, TP)
        hh = jnp.concatenate([h_s[k * G + i // (TG // TP), sub, :] for k in range(7)], axis=1)
        res = lax.dot_general(_bf16(cst[...]), hh, NT, preferred_element_type=F32)
        y = res + xbt[0:D, rows] * dcol[0:D, :]
        ylow[i] = y[0:64]
        for n in range(3):
            ob[rows, 512 + n * 128:640 + n * 128] = y[64 + n * 128:192 + n * 128].T
        y_copy(i).start()
        return res

    def phase3(g, carry):
        pacer.pace([partial(y_piece, 3 * g + k) for k in range(3)], 4 * DH + 8)
        for i in range(2):
            attend(4 * g + 2 * i + 1, True)
            for c in range(4):
                o_s[c * NP:(c + 1) * NP, _ds((2 * g + i) * 8, 8), :] = (
                    ow[c * 128:(c + 1) * 128, :].T.reshape(NP, 8, 128))
        pacer.finish()
        return carry

    for g in range(G):
        phase3(g, 0)

    def a_piece(i):
        rows = _ds(i * TP, TP)
        oo = jnp.concatenate([
            _bf16(jnp.concatenate(
                [o_s[c * NP + i, pl.ds(j, R // 2, stride=8), :]
                 for j in range(TP // R)], axis=0))
            for c in range(4)], axis=1)
        a = lax.dot_general(_bf16(wot[0:D // 2, :]), oo, NT, preferred_element_type=F32)
        for n in range(3):
            ob[rows, n * 128:(n + 1) * 128] = a[n * 128:(n + 1) * 128].T
        ob[rows, 384:512] = jnp.concatenate([a[384:D], ylow[i]], axis=0).T
        a_copy(i).start()

    def phase4(g, carry):
        y_piece(3 * G + g)
        for k in range(NP // G):
            a_piece(g * (NP // G) + k)
        return carry

    _loop(phase4, 0, unroll=1)
    for i in range(NP):
        y_copy(i).wait()
        a_copy(i).wait()


@jax.jit
def pallas_concat_heads__sliding_local_dilated__ssm_conv_s5__prompt_kernel(
    A_x, A_wqkv, A_wo, B_x, B_Lambda_re, B_Lambda_im, B_B_re, B_B_im, B_C_re, B_C_im,
    B_log_dt, B_Dskip,
):
    hbm = pl.BlockSpec(memory_space=pl.ANY)
    vm = pltpu.VMEM
    dma = pltpu.SemaphoreType.DMA
    scratch = [vm((D,), BF16)] * 4 + [
        vm((512, S), BF16), vm((512, S), BF16),
        vm((4 * S, 128), BF16), vm((4 * S, 128), BF16),
        vm((S // 2, 512), U32), vm((S // 2, 512), U32),
        vm((2 * D, D), BF16),
        vm((S, 2 * D), F32),
        vm((D, 3 * D), BF16),
        vm((4 * 1408, 128), BF16),
        vm((3 * D // 2, 512), U32),
        vm((R, D, 128), F32),
        vm((2 * R, D, 128), F32), vm((2 * R, D, 128), F32),
        vm((7 * G, TG, 128), BF16),
        vm((4 * NP, TP // 2, 128), U32),
        vm((D, D), BF16), vm((D, D), BF16),
        vm((D // 2, 2 * D), U32),
        vm((D, D), BF16), vm((4, D, 128), BF16),
        vm((256, 128), U32), vm((256, 512), U32),
        vm((512, 128), U32),
        vm((512, 128), F32),
        vm((NP, 64, 128), F32),
        vm((S, 2 * D), F32),
        dma((G,)), dma((7,)), dma((6,)), dma((2 * NP,)),
    ]
    return pl.pallas_call(
        _kernel,
        out_shape=jax.ShapeDtypeStruct((1, S, 2 * D), F32),
        in_specs=[hbm] * 12,
        out_specs=hbm,
        scratch_shapes=scratch,
        compiler_params=pltpu.CompilerParams(vmem_limit_bytes=100 * 1024 * 1024),
    )(jnp.swapaxes(A_x, 1, 2), A_wqkv, A_wo, jnp.swapaxes(B_x, 1, 2), B_Lambda_re, B_Lambda_im,
      B_B_re, B_B_im, B_C_re, B_C_im, B_log_dt, B_Dskip)
```

```python
from functools import partial

import jax
import jax.numpy as jnp
from jax import lax
import jax.experimental.pallas as pl
import jax.experimental.pallas.tpu as pltpu

S = 2048
D = 448
H = 16
DH = 28
W = 8
R = 16
G = 4
TG = S // G
JG = TG // R
TP = 128
NP = S // TP
NY = 12

F32 = jnp.float32
BF16 = jnp.bfloat16
U32 = jnp.uint32
NT = (((1,), (1,)), ((), ()))


def _unpack(w):
    lo = pltpu.bitcast(w.astype(jnp.uint16), U32)
    hi = pltpu.bitcast((w >> 16).astype(jnp.uint16), U32)
    return lo, hi


def _pack(even, odd):
    return pltpu.bitcast(pltpu.pack_elementwise([even, odd], packed_dtype=BF16), U32)


def _words(x):
    return pltpu.bitcast(x.astype(BF16), U32)


def _bf16(w, cols=None):
    x = pltpu.bitcast(w, BF16)
    return x if cols is None else x[:, :cols]


def _ds(start, size, align=None):
    return pl.ds(pl.multiple_of(start, align or size), size)


def _step(lam, h, b):
    lr, li = lam
    return (lr * h[0] - li * h[1] + b[0], lr * h[1] + li * h[0] + b[1])


def _lam_tiles(re, im, lane):
    out = [(re[:, c * 128:(c + 1) * 128], im[:, c * 128:(c + 1) * 128]) for c in range(3)]
    z = jnp.zeros((1, 64), F32)
    r3 = jnp.concatenate([re[:, 384:], z], axis=1)
    i3 = jnp.concatenate([im[:, 384:], z], axis=1)
    out.append((jnp.where(lane < 64, r3, pltpu.roll(r3, 64, 1)),
                jnp.where(lane < 64, i3, -pltpu.roll(i3, 64, 1))))
    return out


class _Pacer:
    def __init__(self):
        self.zero = lax.broadcasted_iota(U32, (8, 128), 1) >> 16

    def pace(self, matmuls, steps):
        self.queue = list(matmuls)
        self.per = -(-steps // len(matmuls))
        self.pos = 0

    def gate(self, *xs):
        i = self.pos % self.per
        if i == 0:
            self.res = self.queue.pop(0)()
        self.pos += 1
        k = (self.res.shape[0] // 8 * i) // self.per * 8
        tok = pltpu.bitcast(self.res[k:k + 8, 0:128], U32) & self.zero
        out = []
        for x in xs:
            u = pltpu.bitcast(x, U32)
            u = u | jnp.tile(tok, (u.shape[0] // 8, u.shape[1] // 128))
            out.append(pltpu.bitcast(u, x.dtype))
        return out if len(out) > 1 else out[0]

    def finish(self):
        while self.queue:
            self.queue.pop(0)()


def _loop(body, init, unroll=2):
    def outer(t, carry):
        for u in range(unroll):
            carry = body(t * unroll + u, carry)
        return carry
    return lax.fori_loop(0, G // unroll, outer, init)


def _kernel(xa_hbm, wqkv_hbm, wo_hbm, xb_hbm, lre_hbm, lim_hbm, bre_hbm, bim_hbm,
            cre_hbm, cim_hbm, ldt_hbm, dsk_hbm, out_hbm,
            lre, lim, ldt, dsk, xat, xbt, xan, xbn, xap, xbp, bst, bu, wraw, wtn, wt,
            q_s, k_s, v_s, h_s, o_s, cre, cim, cst, woraw, won, wop, wot, ow, dcol, ylow, ob,
            sem_xb, sem_b, sem_in, sem_out):
    copy = pltpu.make_async_copy
    xb_cp = [copy(xb_hbm.at[0, :, pl.ds(g * TG, TG)], xbt.at[pl.ds(0, D), pl.ds(g * TG, TG)],
                  sem_xb.at[g]) for g in range(G)]
    b_cp = []
    for c in range(3):
        b_cp.append([copy(bre_hbm.at[pl.ds(c * 128, 128)], bst.at[pl.ds(c * 256, 128)], sem_b.at[2 * c])])
        b_cp.append([copy(bim_hbm.at[pl.ds(c * 128, 128)], bst.at[pl.ds(c * 256 + 128, 128)],
                          sem_b.at[2 * c + 1])])
    b_cp.append([copy(bre_hbm.at[pl.ds(384, 64)], bst.at[pl.ds(768, 64)], sem_b.at[6]),
                 copy(bim_hbm.at[pl.ds(384, 64)], bst.at[pl.ds(832, 64)], sem_b.at[6])])
    p_cp = [copy(src, dst, sem_in.at[5]) for src, dst in
            ((lre_hbm, lre), (lim_hbm, lim), (ldt_hbm, ldt), (dsk_hbm, dsk))]
    w_cp = copy(wqkv_hbm, wraw, sem_in.at[0])
    xa_cp = copy(xa_hbm.at[0], xat.at[pl.ds(0, D)], sem_in.at[1])
    c_cp = [copy(cre_hbm, cre, sem_in.at[2]), copy(cim_hbm, cim, sem_in.at[3])]
    wo_cp = [copy(wo_hbm.at[:, pl.ds(c * 128, 128)], won.at[c], sem_in.at[4]) for c in range(3)]
    wo_cp.append(copy(wo_hbm, woraw, sem_in.at[4]))

    for cp in [xb_cp[0]] + sum(b_cp, []) + p_cp:
        cp.start()

    xat[D:512, :] = jnp.zeros((512 - D, S), BF16)
    xbt[D:512, :] = jnp.zeros((512 - D, S), BF16)
    ow[D:512, :] = jnp.zeros((512 - D, 128), U32)
    pacer = _Pacer()
    gate = pacer.gate

    def transpose_x(xt_ref, xn_ref, c, g):
        for t in range(g * TG, (g + 1) * TG, 128):
            xn_ref[pl.ds(c * S + t, 128), :] = gate(xt_ref[c * 128:(c + 1) * 128, t:t + 128]).T

    def gather_x(xn_ref, xp_ref, c, row0, rhos, nj, g8=gate):
        xu = xn_ref.bitcast(U32)
        for rho in rhos:
            lo, hi = _unpack(g8(xu[pl.ds(c * (S // 2) + row0 + rho, nj, stride=R // 2), :]))
            dst = row0 + rho * nj
            xp_ref[dst:dst + nj // 2, c * 128:(c + 1) * 128] = lo
            xp_ref[dst + nj // 2:dst + nj, c * 128:(c + 1) * 128] = hi

    def w_transpose(n):
        cols = min(128, 3 * D - n * 128)
        for c in range(4):
            rows = min(128, D - c * 128)
            v = wraw[c * 128:c * 128 + rows, n * 128:n * 128 + cols]
            if rows < 128:
                v = jnp.concatenate([v, jnp.zeros((128 - rows, cols), BF16)], axis=0)
            if cols < 128:
                v = jnp.concatenate([v, jnp.zeros((128, 128 - cols), BF16)], axis=1)
            wtn[pl.ds(c * 1408 + n * 128, 128), :] = gate(v).T

    def w_gather(part, c):
        wu = wtn.bitcast(U32)
        for dp in range(DH // 2):
            lo, hi = _unpack(gate(wu[pl.ds(c * 704 + part * (D // 2) + dp, H, stride=DH // 2), :]))
            base = part * (D // 2) + dp * H
            wt[base:base + H // 2, c * 128:(c + 1) * 128] = lo
            wt[base + H // 2:base + H, c * 128:(c + 1) * 128] = hi

    def bu_piece(g, n):
        res = lax.dot_general(_bf16(xbp[g * TG // 2:(g + 1) * TG // 2, :], D),
                              bst[n * 128:(n + 1) * 128, :], NT, preferred_element_type=F32)
        bu[g * TG:(g + 1) * TG, n * 128:(n + 1) * 128] = res
        return res

    def prep_xb(g):
        xb_cp[g].wait()
        for c in range(4):
            transpose_x(xbt, xbn, c, g)
            gather_x(xbn, xbp, c, g * (TG // 2), range(R // 2), JG)

    def prep_xa(cs):
        for c in cs:
            for g in range(G):
                transpose_x(xat, xan, c, g)
            gather_x(xan, xap, c, 0, range(R // 2), 128)

    xb_cp[0].wait()
    for cp in [xb_cp[1], w_cp, xb_cp[2]]:
        cp.start()
    for c in range(4):
        xbn[pl.ds(c * S, TG), :] = xbt[c * 128:(c + 1) * 128, 0:TG].T
        gather_x(xbn, xbp, c, 0, range(R // 2), JG, lambda v: v)

    def bu_chunk(g, steps):
        pacer.pace([partial(bu_piece, g, n) for n in range(7)], steps)

    for cp in b_cp[0] + b_cp[1]:
        cp.wait()
    bu_chunk(0, 70)
    for _ in range(20):
        gate(pacer.zero)
    for cp in sum(b_cp[2:], []):
        cp.wait()
    prep_xb(1)
    for cp in p_cp:
        cp.wait()
    lane = lax.broadcasted_iota(jnp.int32, (1, 128), 1)
    a_re = lre[...].astype(F32).reshape(1, D)
    a_im = lim[...].astype(F32).reshape(1, D)
    dt = jnp.exp(ldt[...].astype(F32).reshape(1, D)).astype(BF16).astype(F32)
    mag = jnp.exp(dt * a_re)
    l_re = mag * jnp.cos(dt * a_im)
    l_im = mag * jnp.sin(dt * a_im)
    den = a_re * a_re + a_im * a_im
    n_re = l_re - 1.0
    co_re = 2.0 * (n_re * a_re + l_im * a_im) / den
    co_im = 2.0 * (l_im * a_re - n_re * a_im) / den
    lam1 = _lam_tiles(l_re, l_im, lane)
    p_re, p_im = l_re, l_im
    for _ in range(4):
        p_re, p_im = p_re * p_re - p_im * p_im, 2.0 * p_re * p_im
    lam_pows = []
    for _ in range(5):
        lam_pows.append(_lam_tiles(p_re, p_im, lane))
        p_re, p_im = p_re * p_re - p_im * p_im, 2.0 * p_re * p_im
    drow = jnp.concatenate([dsk[...].astype(F32).reshape(1, D), jnp.zeros((1, 64), F32)], axis=1)
    dcol[...] = jnp.broadcast_to(drow, (128, 512)).T

    pacer.finish()

    for cp in (xa_cp, xb_cp[3]):
        cp.start()
    bu_chunk(1, 28 + 48 + 12 + 56)
    w_cp.wait()
    for n in range(7):
        w_transpose(n)
    prep_xb(2)
    for n in range(7, 10):
        w_transpose(n)
    for part in range(1):
        for c in range(4):
            w_gather(part, c)
    pacer.finish()

    for cp in wo_cp + c_cp:
        cp.start()
    bu_chunk(2, 4 + 48 + 112 + 24)
    xa_cp.wait()
    w_transpose(10)
    prep_xb(3)
    for c in range(4):
        w_gather(1, c)
        w_gather(2, c)
    prep_xa([0])
    pacer.finish()

    bu_chunk(3, 78)
    for cp in wo_cp:
        cp.wait()
    won[3] = jnp.concatenate([woraw[:, 384:D], jnp.zeros((D, 64), BF16)], axis=1)
    prep_xa([1, 2, 3])
    pacer.finish()

    row = lax.broadcasted_iota(jnp.int32, (JG, 128), 0)
    hu = h_s.bitcast(U32)

    def scan_chunk(g, c, prev):
        nparts = 2 if c < 3 else 1

        def load(r):
            v = [bu[_ds(g * TG + r * JG, JG), c * 256 + k * 128:c * 256 + (k + 1) * 128]
                 for k in range(nparts)]
            return v if c < 3 else (v[0], pltpu.roll(v[0], 64, 1))

        f = gate(*load(0))
        for r in range(1, R):
            f = _step(lam1[c], f, gate(*load(r)))
        s = tuple(pltpu.roll(jnp.where(row == JG - 1, p, x), 1, 0) for p, x in zip(prev, f))
        for m in range(5):
            sh = tuple(jnp.where(row >= 2 ** m, pltpu.roll(x, 2 ** m, 0), 0.0) for x in s)
            s = _step(lam_pows[m][c], sh, s)
        for rho in range(R // 2):
            e = _step(lam1[c], s, gate(*load(2 * rho)))
            s = _step(lam1[c], e, load(2 * rho + 1))
            for k in range(nparts):
                hu[(2 * c + k) * G + g, pl.ds(rho, JG, stride=R // 2), :] = _pack(e[k], s[k])
        return s

    def qkv_part(r, part):
        dst, i = ((q_s, r), (k_s, R + r), (v_s, R + r))[part]
        res = lax.dot_general(_bf16(wt[part * D // 2:(part + 1) * D // 2, :], D),
                              _bf16(xap[_ds(r * 64, 64), :], D), NT, preferred_element_type=F32)
        dst[i] = res
        return res

    def shift_kv(r):
        k_s[r] = pltpu.roll(k_s[R + r], 1, 1)
        v_s[r] = pltpu.roll(v_s[R + r], 1, 1)

    def prep_wo(c):
        wu = won.bitcast(U32)
        for dp in range(DH // 2):
            lo, hi = _unpack(wu[c, pl.ds(dp, H, stride=DH // 2), :])
            wop[dp * H:dp * H + H // 2, :] = lo
            wop[dp * H + H // 2:(dp + 1) * H, :] = hi
        wop[D // 2:256, :] = jnp.zeros((256 - D // 2, 128), U32)
        wot[_ds(c * 64, 64), :] = pltpu.bitcast(_bf16(wop[...]).T, U32)

    def phase2a(g, prev):
        last = []
        for i in range(2):
            r = 4 * g + 2 * i
            pacer.pace([partial(qkv_part, r, k) for k in (1, 2, 0)], 48)
            last.append(scan_chunk(g, 2 * i, prev[2 * i]))
            last.append(scan_chunk(g, 2 * i + 1, prev[2 * i + 1]))
            shift_kv(r)
        prep_wo(g)
        return tuple(last)

    zero = jnp.zeros((JG, 128), F32)
    _loop(phase2a, ((zero, zero),) * 4)

    lane_h = lax.broadcasted_iota(jnp.int32, (H, 128), 1)
    scale = DH ** -0.5

    def attend(r, odd):
        acc = [None] * W
        for d in range(DH):
            rows = slice(d * H, (d + 1) * H)
            qd = gate(q_s[r, rows, :])
            for w in range(W):
                t = qd * k_s[R + r - 2 * w, rows, :]
                acc[w] = t if d == 0 else acc[w] + t
        lg = []
        for w in range(W):
            first = jnp.where(r < 2 * w, 1, 0)
            lg.append(jnp.where(lane_h < first, -1e9, acc[w] * scale))
        m = lg[0]
        for w in range(1, W):
            m = jnp.maximum(m, lg[w])
        e = [jnp.exp(x - m) for x in lg]
        tot = e[0]
        for w in range(1, W):
            tot = tot + e[w]
        inv = 1.0 / tot
        p = [x * inv for x in e]
        for d in range(DH):
            rows = slice(d * H, (d + 1) * H)
            o = gate(p[0] * v_s[R + r, rows, :])
            for w in range(1, W):
                o = o + p[w] * v_s[R + r - 2 * w, rows, :]
            if odd:
                ow[rows, :] = _pack(q_s[r - 1, rows, :], o)
            else:
                q_s[r, rows, :] = o

    def prep_c(r0):
        src, dst = _ds(r0, D // G, 16), _ds(r0 // 2, D // G // 2, 8)
        for c in range(4):
            sl = slice(c * 128, min(D, (c + 1) * 128))
            xr, xi = cre[src, sl].astype(F32), cim[src, sl].astype(F32)
            cr, ci = co_re[:, sl], co_im[:, sl]
            yr, yi = xr * cr - xi * ci, -(xr * ci + xi * cr)
            if c < 3:
                cst[dst, c * 256:c * 256 + 128] = _words(yr)
                cst[dst, c * 256 + 128:c * 256 + 256] = _words(yi)
            else:
                cst[dst, 768:896] = _words(jnp.concatenate([yr, yi], axis=1))

    for cp in c_cp:
        cp.wait()

    for r in range(0, R, 2):
        pacer.pace([partial(qkv_part, r + 1, k) for k in (1, 2)], 2 * DH + 1)
        attend(r, False)
        shift_kv(r + 1)
        if r % 4 == 2:
            prep_c(r // 4 * (D // G))

    def y_copy(i):
        rows = _ds(i * TP, TP)
        return copy(ob.at[rows, pl.ds(512, 384)], out_hbm.at[0, rows, pl.ds(512, 384)], sem_out.at[i])

    def a_copy(i):
        rows = _ds(i * TP, TP)
        return copy(ob.at[rows, pl.ds(0, 512)], out_hbm.at[0, rows, pl.ds(0, 512)], sem_out.at[NP + i])

    def y_piece(i):
        rows = _ds(i * TP, TP)
        sub = _ds((i % (TG // TP)) * TP, TP)
        hh = jnp.concatenate([h_s[k * G + i // (TG // TP), sub, :] for k in range(7)], axis=1)
        res = lax.dot_general(_bf16(cst[...]), hh, NT, preferred_element_type=F32)
        y = res + xbt[0:D, rows] * dcol[0:D, :]
        ylow[i] = y[0:64]
        for n in range(3):
            ob[rows, 512 + n * 128:640 + n * 128] = y[64 + n * 128:192 + n * 128].T
        y_copy(i).start()
        return res

    qkv_part(1, 0)
    for i in range(R // 2):
        nxt = [partial(qkv_part, 2 * i + 3, 0)] if i < R // 2 - 1 else []
        ys = [partial(y_piece, k) for k in range(NY * i // 8, NY * (i + 1) // 8)]
        pacer.pace(nxt + ys, 2 * DH + 4)
        attend(2 * i + 1, True)
        for c in range(4):
            o_s[c * NP:(c + 1) * NP, i * 8:(i + 1) * 8, :] = (
                ow[c * 128:(c + 1) * 128, :].T.reshape(NP, 8, 128))
        pacer.finish()

    def a_piece(i):
        rows = _ds(i * TP, TP)
        oo = jnp.concatenate([
            _bf16(jnp.concatenate(
                [o_s[c * NP + i, pl.ds(j, R // 2, stride=8), :]
                 for j in range(TP // R)], axis=0))
            for c in range(4)], axis=1)
        a = lax.dot_general(_bf16(wot[0:D // 2, :]), oo, NT, preferred_element_type=F32)
        for n in range(3):
            ob[rows, n * 128:(n + 1) * 128] = a[n * 128:(n + 1) * 128].T
        ob[rows, 384:512] = jnp.concatenate([a[384:D], ylow[i]], axis=0).T
        a_copy(i).start()

    def phase4(g, carry):
        for k in range(1):
            y_piece(NY + g * 1 + k)
        for k in range(4):
            a_piece(g * 4 + k)
        return carry

    lax.fori_loop(0, 4, phase4, 0)
    for i in range(NP):
        y_copy(i).wait()
        a_copy(i).wait()


@jax.jit
def pallas_concat_heads__sliding_local_dilated__ssm_conv_s5__prompt_kernel(
    A_x, A_wqkv, A_wo, B_x, B_Lambda_re, B_Lambda_im, B_B_re, B_B_im, B_C_re, B_C_im,
    B_log_dt, B_Dskip,
):
    hbm = pl.BlockSpec(memory_space=pl.ANY)
    vm = pltpu.VMEM
    dma = pltpu.SemaphoreType.DMA
    scratch = [vm((D,), BF16)] * 4 + [
        vm((512, S), BF16), vm((512, S), BF16),
        vm((4 * S, 128), BF16), vm((4 * S, 128), BF16),
        vm((S // 2, 512), U32), vm((S // 2, 512), U32),
        vm((2 * D, D), BF16),
        vm((S, 2 * D), F32),
        vm((D, 3 * D), BF16),
        vm((4 * 1408, 128), BF16),
        vm((3 * D // 2, 512), U32),
        vm((R, D, 128), F32),
        vm((2 * R, D, 128), F32), vm((2 * R, D, 128), F32),
        vm((7 * G, TG, 128), BF16),
        vm((4 * NP, TP // 2, 128), U32),
        vm((D, D), BF16), vm((D, D), BF16),
        vm((D // 2, 2 * D), U32),
        vm((D, D), BF16), vm((4, D, 128), BF16),
        vm((256, 128), U32), vm((256, 512), U32),
        vm((512, 128), U32),
        vm((512, 128), F32),
        vm((NP, 64, 128), F32),
        vm((S, 2 * D), F32),
        dma((G,)), dma((7,)), dma((6,)), dma((2 * NP,)),
    ]
    return pl.pallas_call(
        _kernel,
        out_shape=jax.ShapeDtypeStruct((1, S, 2 * D), F32),
        in_specs=[hbm] * 12,
        out_specs=hbm,
        scratch_shapes=scratch,
        compiler_params=pltpu.CompilerParams(vmem_limit_bytes=100 * 1024 * 1024),
    )(jnp.swapaxes(A_x, 1, 2), A_wqkv, A_wo, jnp.swapaxes(B_x, 1, 2), B_Lambda_re, B_Lambda_im,
      B_B_re, B_B_im, B_C_re, B_C_im, B_log_dt, B_Dskip)
```

```python
from functools import partial

import jax
import jax.numpy as jnp
from jax import lax
import jax.experimental.pallas as pl
import jax.experimental.pallas.tpu as pltpu

S = 2048
D = 448
H = 16
DH = 28
W = 8
R = 16
G = 4
TG = S // G
JG = TG // R
TP = 128
NP = S // TP
NY = 12

F32 = jnp.float32
BF16 = jnp.bfloat16
U32 = jnp.uint32
NT = (((1,), (1,)), ((), ()))


def _unpack(w):
    lo = pltpu.bitcast(w.astype(jnp.uint16), U32)
    hi = pltpu.bitcast((w >> 16).astype(jnp.uint16), U32)
    return lo, hi


def _pack(even, odd):
    return pltpu.bitcast(pltpu.pack_elementwise([even, odd], packed_dtype=BF16), U32)


def _words(x):
    return pltpu.bitcast(x.astype(BF16), U32)


def _bf16(w, cols=None):
    x = pltpu.bitcast(w, BF16)
    return x if cols is None else x[:, :cols]


def _ds(start, size, align=None):
    return pl.ds(pl.multiple_of(start, align or size), size)


def _step(lam, h, b):
    lr, li = lam
    return (lr * h[0] - li * h[1] + b[0], lr * h[1] + li * h[0] + b[1])


def _lam_tiles(re, im, lane):
    out = [(re[:, c * 128:(c + 1) * 128], im[:, c * 128:(c + 1) * 128]) for c in range(3)]
    z = jnp.zeros((1, 64), F32)
    r3 = jnp.concatenate([re[:, 384:], z], axis=1)
    i3 = jnp.concatenate([im[:, 384:], z], axis=1)
    out.append((jnp.where(lane < 64, r3, pltpu.roll(r3, 64, 1)),
                jnp.where(lane < 64, i3, -pltpu.roll(i3, 64, 1))))
    return out


class _Pacer:
    def __init__(self):
        self.zero = lax.broadcasted_iota(U32, (8, 128), 1) >> 16

    def pace(self, matmuls, steps):
        self.queue = list(matmuls)
        self.per = -(-steps // len(matmuls))
        self.pos = 0

    def gate(self, *xs):
        i = self.pos % self.per
        if i == 0 and not self.queue:
            return xs if len(xs) > 1 else xs[0]
        if i == 0:
            self.res = self.queue.pop(0)()
        self.pos += 1
        k = (self.res.shape[0] // 8 * i) // self.per * 8
        tok = pltpu.bitcast(self.res[k:k + 8, 0:128], U32) & self.zero
        out = []
        for x in xs:
            u = pltpu.bitcast(x, U32)
            u = u | jnp.tile(tok, (u.shape[0] // 8, u.shape[1] // 128))
            out.append(pltpu.bitcast(u, x.dtype))
        return out if len(out) > 1 else out[0]

    def finish(self):
        while self.queue:
            self.queue.pop(0)()
        self.pos = 0


def _loop(body, init, unroll=2):
    def outer(t, carry):
        for u in range(unroll):
            carry = body(t * unroll + u, carry)
        return carry
    return lax.fori_loop(0, G // unroll, outer, init)


def _kernel(xa_hbm, wqkv_hbm, wo_hbm, xb_hbm, lre_hbm, lim_hbm, bre_hbm, bim_hbm,
            cre_hbm, cim_hbm, ldt_hbm, dsk_hbm, out_hbm,
            lre, lim, ldt, dsk, xat, xbt, xan, xbn, xap, xbp, bst, bu, wraw, wtn, wt,
            q_s, k_s, v_s, h_s, o_s, cre, cim, cst, woraw, won, wop, wot, ow, dcol, ylow, fin, ob,
            sem_xb, sem_b, sem_in, sem_out):
    copy = pltpu.make_async_copy
    xb_cp = [copy(xb_hbm.at[0, :, pl.ds(g * TG, TG)], xbt.at[pl.ds(0, D), pl.ds(g * TG, TG)],
                  sem_xb.at[g]) for g in range(G)]
    b_cp = []
    for c in range(3):
        b_cp.append([copy(bre_hbm.at[pl.ds(c * 128, 128)], bst.at[pl.ds(c * 256, 128)], sem_b.at[2 * c])])
        b_cp.append([copy(bim_hbm.at[pl.ds(c * 128, 128)], bst.at[pl.ds(c * 256 + 128, 128)],
                          sem_b.at[2 * c + 1])])
    b_cp.append([copy(bre_hbm.at[pl.ds(384, 64)], bst.at[pl.ds(768, 64)], sem_b.at[6]),
                 copy(bim_hbm.at[pl.ds(384, 64)], bst.at[pl.ds(832, 64)], sem_b.at[6])])
    p_cp = [copy(src, dst, sem_in.at[5]) for src, dst in
            ((lre_hbm, lre), (lim_hbm, lim), (ldt_hbm, ldt), (dsk_hbm, dsk))]
    w_cp = copy(wqkv_hbm, wraw, sem_in.at[0])
    xa_cp = copy(xa_hbm.at[0], xat.at[pl.ds(0, D)], sem_in.at[1])
    c_cp = [copy(cre_hbm, cre, sem_in.at[2]), copy(cim_hbm, cim, sem_in.at[3])]
    wo_cp = [copy(wo_hbm.at[:, pl.ds(c * 128, 128)], won.at[c], sem_in.at[4]) for c in range(3)]
    wo_cp.append(copy(wo_hbm, woraw, sem_in.at[4]))

    for cp in [xb_cp[0]] + sum(b_cp, []) + p_cp:
        cp.start()

    xat[D:512, :] = jnp.zeros((512 - D, S), BF16)
    xbt[D:512, :] = jnp.zeros((512 - D, S), BF16)
    ow[D:512, :] = jnp.zeros((512 - D, 128), U32)
    pacer = _Pacer()
    gate = pacer.gate

    def transpose_x(xt_ref, xn_ref, c, g):
        for t in range(g * TG, (g + 1) * TG, 128):
            xn_ref[pl.ds(c * S + t, 128), :] = gate(xt_ref[c * 128:(c + 1) * 128, t:t + 128]).T

    def gather_x(xn_ref, xp_ref, c, row0, rhos, nj, g8=gate):
        xu = xn_ref.bitcast(U32)
        for rho in rhos:
            lo, hi = _unpack(g8(xu[pl.ds(c * (S // 2) + row0 + rho, nj, stride=R // 2), :]))
            dst = row0 + rho * nj
            xp_ref[dst:dst + nj // 2, c * 128:(c + 1) * 128] = lo
            xp_ref[dst + nj // 2:dst + nj, c * 128:(c + 1) * 128] = hi

    def w_transpose(n):
        cols = min(128, 3 * D - n * 128)
        for c in range(4):
            rows = min(128, D - c * 128)
            v = wraw[c * 128:c * 128 + rows, n * 128:n * 128 + cols]
            if rows < 128:
                v = jnp.concatenate([v, jnp.zeros((128 - rows, cols), BF16)], axis=0)
            if cols < 128:
                v = jnp.concatenate([v, jnp.zeros((128, 128 - cols), BF16)], axis=1)
            wtn[pl.ds(c * 1408 + n * 128, 128), :] = gate(v).T

    def w_gather(part, c):
        wu = wtn.bitcast(U32)
        for dp in range(DH // 2):
            lo, hi = _unpack(gate(wu[pl.ds(c * 704 + part * (D // 2) + dp, H, stride=DH // 2), :]))
            base = part * (D // 2) + dp * H
            wt[base:base + H // 2, c * 128:(c + 1) * 128] = lo
            wt[base + H // 2:base + H, c * 128:(c + 1) * 128] = hi

    def bu_piece(g, n):
        res = lax.dot_general(_bf16(xbp[g * TG // 2:(g + 1) * TG // 2, :], D),
                              bst[n * 128:(n + 1) * 128, :], NT, preferred_element_type=F32)
        bu[g * TG:(g + 1) * TG, n * 128:(n + 1) * 128] = res
        return res

    def prep_xb(g):
        xb_cp[g].wait()
        for c in range(4):
            transpose_x(xbt, xbn, c, g)
            gather_x(xbn, xbp, c, g * (TG // 2), range(R // 2), JG)

    def prep_xa(cs):
        for c in cs:
            for g in range(G):
                transpose_x(xat, xan, c, g)
            gather_x(xan, xap, c, 0, range(R // 2), 128)

    xb_cp[0].wait()
    for cp in [xb_cp[1], w_cp, xb_cp[2]]:
        cp.start()
    for c in range(4):
        xbn[pl.ds(c * S, TG), :] = xbt[c * 128:(c + 1) * 128, 0:TG].T
        gather_x(xbn, xbp, c, 0, range(R // 2), JG, lambda v: v)

    def load_bu(g, c, r):
        v = [bu[_ds(g * TG + r * JG, JG), c * 256 + k * 128:c * 256 + (k + 1) * 128]
             for k in range(2 if c < 3 else 1)]
        return v if c < 3 else (v[0], pltpu.roll(v[0], 64, 1))

    def local_scan(g):
        for c in range(4):
            f = gate(*load_bu(g, c, 0))
            for r in range(1, R):
                f = _step(lam1[c], f, gate(*load_bu(g, c, r)))
            for k in range(2):
                fin[g * JG:(g + 1) * JG, (2 * c + k) * 128:(2 * c + k + 1) * 128] = f[k]

    def bu_chunk(g, steps):
        pacer.pace([partial(bu_piece, g, n) for n in range(7)], steps)

    for cp in b_cp[0] + b_cp[1]:
        cp.wait()
    bu_chunk(0, 70)
    for _ in range(20):
        gate(pacer.zero)
    for cp in sum(b_cp[2:], []):
        cp.wait()
    prep_xb(1)
    for cp in p_cp:
        cp.wait()
    lane = lax.broadcasted_iota(jnp.int32, (1, 128), 1)
    a_re = lre[...].astype(F32).reshape(1, D)
    a_im = lim[...].astype(F32).reshape(1, D)
    dt = jnp.exp(ldt[...].astype(F32).reshape(1, D)).astype(BF16).astype(F32)
    mag = jnp.exp(dt * a_re)
    l_re = mag * jnp.cos(dt * a_im)
    l_im = mag * jnp.sin(dt * a_im)
    den = a_re * a_re + a_im * a_im
    n_re = l_re - 1.0
    co_re = 2.0 * (n_re * a_re + l_im * a_im) / den
    co_im = 2.0 * (l_im * a_re - n_re * a_im) / den
    lam1 = _lam_tiles(l_re, l_im, lane)
    p_re, p_im = l_re, l_im
    for _ in range(4):
        p_re, p_im = p_re * p_re - p_im * p_im, 2.0 * p_re * p_im
    lam_pows = []
    for _ in range(5):
        lam_pows.append(_lam_tiles(p_re, p_im, lane))
        p_re, p_im = p_re * p_re - p_im * p_im, 2.0 * p_re * p_im
    drow = jnp.concatenate([dsk[...].astype(F32).reshape(1, D), jnp.zeros((1, 64), F32)], axis=1)
    dcol[...] = jnp.broadcast_to(drow, (128, 512)).T

    pacer.finish()

    for cp in (xa_cp, xb_cp[3]):
        cp.start()
    bu_chunk(1, 28 + 48 + 12 + 56 + 64)
    local_scan(0)
    w_cp.wait()
    for n in range(7):
        w_transpose(n)
    prep_xb(2)
    for n in range(7, 10):
        w_transpose(n)
    for part in range(1):
        for c in range(4):
            w_gather(part, c)
    pacer.finish()

    for cp in wo_cp + c_cp:
        cp.start()
    bu_chunk(2, 4 + 48 + 112 + 24 + 64)
    local_scan(1)
    xa_cp.wait()
    w_transpose(10)
    prep_xb(3)
    for c in range(4):
        w_gather(1, c)
        w_gather(2, c)
    prep_xa([0])
    pacer.finish()

    bu_chunk(3, 78 + 64)
    local_scan(2)
    for cp in wo_cp:
        cp.wait()
    won[3] = jnp.concatenate([woraw[:, 384:D], jnp.zeros((D, 64), BF16)], axis=1)
    prep_xa([1, 2, 3])
    pacer.finish()
    local_scan(3)

    row = lax.broadcasted_iota(jnp.int32, (JG, 128), 0)
    hu = h_s.bitcast(U32)

    def scan_chunk(g, c, prev):
        nparts = 2 if c < 3 else 1
        load = partial(load_bu, g, c)
        f = [fin[_ds(g * JG, JG), (2 * c + k) * 128:(2 * c + k + 1) * 128] for k in range(2)]
        s = tuple(pltpu.roll(jnp.where(row == JG - 1, p, x), 1, 0) for p, x in zip(prev, f))
        for m in range(5):
            sh = tuple(jnp.where(row >= 2 ** m, pltpu.roll(x, 2 ** m, 0), 0.0) for x in s)
            s = _step(lam_pows[m][c], sh, s)
        for rho in range(R // 2):
            e = _step(lam1[c], s, gate(*load(2 * rho)))
            s = _step(lam1[c], e, load(2 * rho + 1))
            for k in range(nparts):
                hu[(2 * c + k) * G + g, pl.ds(rho, JG, stride=R // 2), :] = _pack(e[k], s[k])
        return s

    def qkv_part(r, part):
        dst, i = ((q_s, r), (k_s, R + r), (v_s, R + r))[part]
        res = lax.dot_general(_bf16(wt[part * D // 2:(part + 1) * D // 2, :], D),
                              _bf16(xap[_ds(r * 64, 64), :], D), NT, preferred_element_type=F32)
        dst[i] = res
        return res

    def shift_kv(r):
        k_s[r] = pltpu.roll(k_s[R + r], 1, 1)
        v_s[r] = pltpu.roll(v_s[R + r], 1, 1)

    def prep_wo(c):
        wu = won.bitcast(U32)
        for dp in range(DH // 2):
            lo, hi = _unpack(wu[c, pl.ds(dp, H, stride=DH // 2), :])
            wop[dp * H:dp * H + H // 2, :] = lo
            wop[dp * H + H // 2:(dp + 1) * H, :] = hi
        wop[D // 2:256, :] = jnp.zeros((256 - D // 2, 128), U32)
        wot[_ds(c * 64, 64), :] = pltpu.bitcast(_bf16(wop[...]).T, U32)

    def phase2a(g, prev):
        last = []
        for i in range(2):
            r = 4 * g + 2 * i
            pacer.pace([partial(qkv_part, r, k) for k in (1, 2, 0)], 18)
            last.append(scan_chunk(g, 2 * i, prev[2 * i]))
            last.append(scan_chunk(g, 2 * i + 1, prev[2 * i + 1]))
            pacer.finish()
            shift_kv(r)
        prep_wo(g)
        return tuple(last)

    zero = jnp.zeros((JG, 128), F32)
    _loop(phase2a, ((zero, zero),) * 4)

    lane_h = lax.broadcasted_iota(jnp.int32, (H, 128), 1)
    scale = DH ** -0.5

    def attend(r, odd):
        acc = [None] * W
        for d in range(DH):
            rows = slice(d * H, (d + 1) * H)
            qd = gate(q_s[r, rows, :])
            for w in range(W):
                t = qd * k_s[R + r - 2 * w, rows, :]
                acc[w] = t if d == 0 else acc[w] + t
        lg = []
        for w in range(W):
            first = jnp.where(r < 2 * w, 1, 0)
            lg.append(jnp.where(lane_h < first, -1e9, acc[w] * scale))
        m = lg[0]
        for w in range(1, W):
            m = jnp.maximum(m, lg[w])
        e = [jnp.exp(x - m) for x in lg]
        tot = e[0]
        for w in range(1, W):
            tot = tot + e[w]
        inv = 1.0 / tot
        p = [x * inv for x in e]
        for d in range(DH):
            rows = slice(d * H, (d + 1) * H)
            o = gate(p[0] * v_s[R + r, rows, :])
            for w in range(1, W):
                o = o + p[w] * v_s[R + r - 2 * w, rows, :]
            if odd:
                ow[rows, :] = _pack(q_s[r - 1, rows, :], o)
            else:
                q_s[r, rows, :] = o

    def prep_c(r0):
        src, dst = _ds(r0, D // G, 16), _ds(r0 // 2, D // G // 2, 8)
        for c in range(4):
            sl = slice(c * 128, min(D, (c + 1) * 128))
            xr, xi = cre[src, sl].astype(F32), cim[src, sl].astype(F32)
            cr, ci = co_re[:, sl], co_im[:, sl]
            yr, yi = xr * cr - xi * ci, -(xr * ci + xi * cr)
            if c < 3:
                cst[dst, c * 256:c * 256 + 128] = _words(yr)
                cst[dst, c * 256 + 128:c * 256 + 256] = _words(yi)
            else:
                cst[dst, 768:896] = _words(jnp.concatenate([yr, yi], axis=1))

    for cp in c_cp:
        cp.wait()

    for r in range(0, R, 2):
        pacer.pace([partial(qkv_part, r + 1, k) for k in (1, 2)], 2 * DH + 1)
        attend(r, False)
        shift_kv(r + 1)
        if r % 4 == 2:
            prep_c(r // 4 * (D // G))

    def y_copy(i):
        rows = _ds(i * TP, TP)
        return copy(ob.at[rows, pl.ds(512, 384)], out_hbm.at[0, rows, pl.ds(512, 384)], sem_out.at[i])

    def a_copy(i):
        rows = _ds(i * TP, TP)
        return copy(ob.at[rows, pl.ds(0, 512)], out_hbm.at[0, rows, pl.ds(0, 512)], sem_out.at[NP + i])

    def y_piece(i):
        rows = _ds(i * TP, TP)
        sub = _ds((i % (TG // TP)) * TP, TP)
        hh = jnp.concatenate([h_s[k * G + i // (TG // TP), sub, :] for k in range(7)], axis=1)
        res = lax.dot_general(_bf16(cst[...]), hh, NT, preferred_element_type=F32)
        y = res + xbt[0:D, rows] * dcol[0:D, :]
        ylow[i] = y[0:64]
        for n in range(3):
            ob[rows, 512 + n * 128:640 + n * 128] = y[64 + n * 128:192 + n * 128].T
        y_copy(i).start()
        return res

    qkv_part(1, 0)
    for i in range(R // 2):
        nxt = [partial(qkv_part, 2 * i + 3, 0)] if i < R // 2 - 1 else []
        ys = [partial(y_piece, k) for k in range(NY * i // 8, NY * (i + 1) // 8)]
        pacer.pace(nxt + ys, 2 * DH + 4)
        attend(2 * i + 1, True)
        for c in range(4):
            o_s[c * NP:(c + 1) * NP, i * 8:(i + 1) * 8, :] = (
                ow[c * 128:(c + 1) * 128, :].T.reshape(NP, 8, 128))
        pacer.finish()

    def a_piece(i):
        rows = _ds(i * TP, TP)
        oo = jnp.concatenate([
            _bf16(jnp.concatenate(
                [o_s[c * NP + i, pl.ds(j, R // 2, stride=8), :]
                 for j in range(TP // R)], axis=0))
            for c in range(4)], axis=1)
        a = lax.dot_general(_bf16(wot[0:D // 2, :]), oo, NT, preferred_element_type=F32)
        for n in range(3):
            ob[rows, n * 128:(n + 1) * 128] = a[n * 128:(n + 1) * 128].T
        ob[rows, 384:512] = jnp.concatenate([a[384:D], ylow[i]], axis=0).T
        a_copy(i).start()

    def phase4(g, carry):
        for k in range(1):
            y_piece(NY + g * 1 + k)
        for k in range(4):
            a_piece(g * 4 + k)
        return carry

    lax.fori_loop(0, 4, phase4, 0)
    for i in range(NP):
        y_copy(i).wait()
        a_copy(i).wait()


@jax.jit
def pallas_concat_heads__sliding_local_dilated__ssm_conv_s5__prompt_kernel(
    A_x, A_wqkv, A_wo, B_x, B_Lambda_re, B_Lambda_im, B_B_re, B_B_im, B_C_re, B_C_im,
    B_log_dt, B_Dskip,
):
    hbm = pl.BlockSpec(memory_space=pl.ANY)
    vm = pltpu.VMEM
    dma = pltpu.SemaphoreType.DMA
    scratch = [vm((D,), BF16)] * 4 + [
        vm((512, S), BF16), vm((512, S), BF16),
        vm((4 * S, 128), BF16), vm((4 * S, 128), BF16),
        vm((S // 2, 512), U32), vm((S // 2, 512), U32),
        vm((2 * D, D), BF16),
        vm((S, 2 * D), F32),
        vm((D, 3 * D), BF16),
        vm((4 * 1408, 128), BF16),
        vm((3 * D // 2, 512), U32),
        vm((R, D, 128), F32),
        vm((2 * R, D, 128), F32), vm((2 * R, D, 128), F32),
        vm((7 * G, TG, 128), BF16),
        vm((4 * NP, TP // 2, 128), U32),
        vm((D, D), BF16), vm((D, D), BF16),
        vm((D // 2, 2 * D), U32),
        vm((D, D), BF16), vm((4, D, 128), BF16),
        vm((256, 128), U32), vm((256, 512), U32),
        vm((512, 128), U32),
        vm((512, 128), F32),
        vm((NP, 64, 128), F32),
        vm((G * JG, 1024), F32),
        vm((S, 2 * D), F32),
        dma((G,)), dma((7,)), dma((6,)), dma((2 * NP,)),
    ]
    return pl.pallas_call(
        _kernel,
        out_shape=jax.ShapeDtypeStruct((1, S, 2 * D), F32),
        in_specs=[hbm] * 12,
        out_specs=hbm,
        scratch_shapes=scratch,
        compiler_params=pltpu.CompilerParams(
            vmem_limit_bytes=100 * 1024 * 1024,
            flags={"XLA_TPU_EVENLY_DISTRIBUTE_CRITICAL_NODES": True}),
    )(jnp.swapaxes(A_x, 1, 2), A_wqkv, A_wo, jnp.swapaxes(B_x, 1, 2), B_Lambda_re, B_Lambda_im,
      B_B_re, B_B_im, B_C_re, B_C_im, B_log_dt, B_Dskip)
```

```python
from functools import partial

import jax
import jax.numpy as jnp
from jax import lax
import jax.experimental.pallas as pl
import jax.experimental.pallas.tpu as pltpu

S = 2048
D = 448
H = 16
DH = 28
W = 8
R = 16
G = 4
TG = S // G
JG = TG // R
TP = 128
NP = S // TP
NY = 12

F32 = jnp.float32
BF16 = jnp.bfloat16
U32 = jnp.uint32
NT = (((1,), (1,)), ((), ()))


def _unpack(w):
    lo = pltpu.bitcast(w.astype(jnp.uint16), U32)
    hi = pltpu.bitcast((w >> 16).astype(jnp.uint16), U32)
    return lo, hi


def _pack(even, odd):
    return pltpu.bitcast(pltpu.pack_elementwise([even, odd], packed_dtype=BF16), U32)


def _words(x):
    return pltpu.bitcast(x.astype(BF16), U32)


def _bf16(w, cols=None):
    x = pltpu.bitcast(w, BF16)
    return x if cols is None else x[:, :cols]


def _ds(start, size, align=None):
    return pl.ds(pl.multiple_of(start, align or size), size)


def _step(lam, h, b):
    lr, li = lam
    return (lr * h[0] - li * h[1] + b[0], lr * h[1] + li * h[0] + b[1])


def _lam_tiles(re, im, lane):
    out = [(re[:, c * 128:(c + 1) * 128], im[:, c * 128:(c + 1) * 128]) for c in range(3)]
    z = jnp.zeros((1, 64), F32)
    r3 = jnp.concatenate([re[:, 384:], z], axis=1)
    i3 = jnp.concatenate([im[:, 384:], z], axis=1)
    out.append((jnp.where(lane < 64, r3, pltpu.roll(r3, 64, 1)),
                jnp.where(lane < 64, i3, -pltpu.roll(i3, 64, 1))))
    return out


class _Pacer:
    def __init__(self):
        self.zero = lax.broadcasted_iota(U32, (8, 128), 1) >> 16

    def pace(self, matmuls, steps):
        self.queue = list(matmuls)
        self.per = -(-steps // len(matmuls))
        self.pos = 0

    def gate(self, *xs):
        i = self.pos % self.per
        if i == 0 and not self.queue:
            return xs if len(xs) > 1 else xs[0]
        if i == 0:
            self.res = self.queue.pop(0)()
        self.pos += 1
        k = (self.res.shape[0] // 8 * i) // self.per * 8
        tok = pltpu.bitcast(self.res[k:k + 8, 0:128], U32) & self.zero
        out = []
        for x in xs:
            u = pltpu.bitcast(x, U32)
            u = u | jnp.tile(tok, (u.shape[0] // 8, u.shape[1] // 128))
            out.append(pltpu.bitcast(u, x.dtype))
        return out if len(out) > 1 else out[0]

    def finish(self):
        while self.queue:
            self.queue.pop(0)()
        self.pos = 0


def _loop(body, init, unroll=2):
    def outer(t, carry):
        for u in range(unroll):
            carry = body(t * unroll + u, carry)
        return carry
    return lax.fori_loop(0, G // unroll, outer, init)


def _kernel(xa_hbm, wqkv_hbm, wo_hbm, xb_hbm, lre_hbm, lim_hbm, bre_hbm, bim_hbm,
            cre_hbm, cim_hbm, ldt_hbm, dsk_hbm, out_hbm,
            lre, lim, ldt, dsk, xat, xbt, xan, xbn, xap, xbp, bst, bu, wraw, wtn, wt,
            q_s, k_s, v_s, h_s, o_s, cre, cim, cst, woraw, won, wop, wot, ow, dcol, ylow, fin, ob,
            sem_xb, sem_b, sem_in, sem_out):
    copy = pltpu.make_async_copy
    xb_cp = [copy(xb_hbm.at[0, :, pl.ds(g * TG, TG)], xbt.at[pl.ds(0, D), pl.ds(g * TG, TG)],
                  sem_xb.at[g]) for g in range(G)]
    b_cp = []
    for c in range(3):
        b_cp.append([copy(bre_hbm.at[pl.ds(c * 128, 128)], bst.at[pl.ds(c * 256, 128)], sem_b.at[2 * c])])
        b_cp.append([copy(bim_hbm.at[pl.ds(c * 128, 128)], bst.at[pl.ds(c * 256 + 128, 128)],
                          sem_b.at[2 * c + 1])])
    b_cp.append([copy(bre_hbm.at[pl.ds(384, 64)], bst.at[pl.ds(768, 64)], sem_b.at[6]),
                 copy(bim_hbm.at[pl.ds(384, 64)], bst.at[pl.ds(832, 64)], sem_b.at[6])])
    p_cp = [copy(src, dst, sem_in.at[5]) for src, dst in
            ((lre_hbm, lre), (lim_hbm, lim), (ldt_hbm, ldt), (dsk_hbm, dsk))]
    w_cp = copy(wqkv_hbm, wraw, sem_in.at[0])
    xa_cp = copy(xa_hbm.at[0], xat.at[pl.ds(0, D)], sem_in.at[1])
    c_cp = [copy(cre_hbm, cre, sem_in.at[2]), copy(cim_hbm, cim, sem_in.at[3])]
    wo_cp = [copy(wo_hbm.at[:, pl.ds(c * 128, 128)], won.at[c, pl.ds(0, D)], sem_in.at[4]) for c in range(3)]
    wo_cp.append(copy(wo_hbm, woraw, sem_in.at[4]))

    for cp in [xb_cp[0]] + sum(b_cp, []) + p_cp:
        cp.start()

    xat[D:512, :] = jnp.zeros((512 - D, S), BF16)
    xbt[D:512, :] = jnp.zeros((512 - D, S), BF16)
    ow[D:512, :] = jnp.zeros((512 - D, 128), U32)
    xan[4 * S:, :] = jnp.zeros((16, 128), BF16)
    xbn[4 * S:, :] = jnp.zeros((16, 128), BF16)
    won[:, D:, :] = jnp.zeros((4, 32, 128), BF16)
    o_s[:, TP // 2:, :] = jnp.zeros((4 * NP, 8, 128), U32)
    pacer = _Pacer()
    gate = pacer.gate

    def transpose_x(xt_ref, xn_ref, c, g):
        for t in range(g * TG, (g + 1) * TG, 128):
            xn_ref[pl.ds(c * S + t, 128), :] = gate(xt_ref[c * 128:(c + 1) * 128, t:t + 128]).T

    def gather_x(xn_ref, xp_ref, c, row0, rhos, nj, g8=gate):
        xu = xn_ref.bitcast(U32)
        for rho in rhos:
            lo, hi = _unpack(g8(xu[pl.ds(c * (S // 2) + row0 + rho, nj, stride=R // 2), :]))
            dst = row0 + rho * nj
            xp_ref[dst:dst + nj // 2, c * 128:(c + 1) * 128] = lo
            xp_ref[dst + nj // 2:dst + nj, c * 128:(c + 1) * 128] = hi

    def w_transpose(n):
        cols = min(128, 3 * D - n * 128)
        for c in range(4):
            rows = min(128, D - c * 128)
            v = wraw[c * 128:c * 128 + rows, n * 128:n * 128 + cols]
            if rows < 128:
                v = jnp.concatenate([v, jnp.zeros((128 - rows, cols), BF16)], axis=0)
            if cols < 128:
                v = jnp.concatenate([v, jnp.zeros((128, 128 - cols), BF16)], axis=1)
            wtn[pl.ds(c * 1408 + n * 128, 128), :] = gate(v).T

    def w_gather(part, c):
        wu = wtn.bitcast(U32)
        for dp in range(DH // 2):
            lo, hi = _unpack(gate(wu[pl.ds(c * 704 + part * (D // 2) + dp, H, stride=DH // 2), :]))
            base = part * (D // 2) + dp * H
            wt[base:base + H // 2, c * 128:(c + 1) * 128] = lo
            wt[base + H // 2:base + H, c * 128:(c + 1) * 128] = hi

    def bu_piece(g, n):
        res = lax.dot_general(_bf16(xbp[g * TG // 2:(g + 1) * TG // 2, :], D),
                              bst[n * 128:(n + 1) * 128, :], NT, preferred_element_type=F32)
        bu[g * TG:(g + 1) * TG, n * 128:(n + 1) * 128] = res
        return res

    def prep_xb(g):
        xb_cp[g].wait()
        for c in range(4):
            transpose_x(xbt, xbn, c, g)
            gather_x(xbn, xbp, c, g * (TG // 2), range(R // 2), JG)

    def prep_xa(cs):
        for c in cs:
            for g in range(G):
                transpose_x(xat, xan, c, g)
            gather_x(xan, xap, c, 0, range(R // 2), 128)

    xb_cp[0].wait()
    for cp in [xb_cp[1], w_cp, xb_cp[2]]:
        cp.start()
    for c in range(4):
        xbn[pl.ds(c * S, TG), :] = xbt[c * 128:(c + 1) * 128, 0:TG].T
        gather_x(xbn, xbp, c, 0, range(R // 2), JG, lambda v: v)

    def load_bu(g, c, r):
        v = [bu[_ds(g * TG + r * JG, JG), c * 256 + k * 128:c * 256 + (k + 1) * 128]
             for k in range(2 if c < 3 else 1)]
        return v if c < 3 else (v[0], pltpu.roll(v[0], 64, 1))

    def local_scan(g):
        for c in range(4):
            f = gate(*load_bu(g, c, 0))
            for r in range(1, R):
                f = _step(lam1[c], f, gate(*load_bu(g, c, r)))
            for k in range(2):
                fin[g * JG:(g + 1) * JG, (2 * c + k) * 128:(2 * c + k + 1) * 128] = f[k]

    def bu_chunk(g, steps):
        pacer.pace([partial(bu_piece, g, n) for n in range(7)], steps)

    for cp in b_cp[0] + b_cp[1]:
        cp.wait()
    bu_chunk(0, 70)
    for _ in range(20):
        gate(pacer.zero)
    for cp in sum(b_cp[2:], []):
        cp.wait()
    prep_xb(1)
    for cp in p_cp:
        cp.wait()
    lane = lax.broadcasted_iota(jnp.int32, (1, 128), 1)
    a_re = lre[...].astype(F32).reshape(1, D)
    a_im = lim[...].astype(F32).reshape(1, D)
    dt = jnp.exp(ldt[...].astype(F32).reshape(1, D)).astype(BF16).astype(F32)
    mag = jnp.exp(dt * a_re)
    l_re = mag * jnp.cos(dt * a_im)
    l_im = mag * jnp.sin(dt * a_im)
    den = a_re * a_re + a_im * a_im
    n_re = l_re - 1.0
    co_re = 2.0 * (n_re * a_re + l_im * a_im) / den
    co_im = 2.0 * (l_im * a_re - n_re * a_im) / den
    lam1 = _lam_tiles(l_re, l_im, lane)
    p_re, p_im = l_re, l_im
    for _ in range(4):
        p_re, p_im = p_re * p_re - p_im * p_im, 2.0 * p_re * p_im
    lam_pows = []
    for _ in range(5):
        lam_pows.append(_lam_tiles(p_re, p_im, lane))
        p_re, p_im = p_re * p_re - p_im * p_im, 2.0 * p_re * p_im
    drow = jnp.concatenate([dsk[...].astype(F32).reshape(1, D), jnp.zeros((1, 64), F32)], axis=1)
    dcol[...] = jnp.broadcast_to(drow, (128, 512)).T

    pacer.finish()

    for cp in (xa_cp, xb_cp[3]):
        cp.start()
    bu_chunk(1, 28 + 48 + 12 + 56 + 64)
    local_scan(0)
    w_cp.wait()
    for n in range(7):
        w_transpose(n)
    prep_xb(2)
    for n in range(7, 10):
        w_transpose(n)
    for part in range(1):
        for c in range(4):
            w_gather(part, c)
    pacer.finish()

    for cp in wo_cp + c_cp:
        cp.start()
    bu_chunk(2, 4 + 48 + 112 + 24 + 64)
    local_scan(1)
    xa_cp.wait()
    w_transpose(10)
    prep_xb(3)
    for c in range(4):
        w_gather(1, c)
        w_gather(2, c)
    prep_xa([0])
    pacer.finish()

    bu_chunk(3, 78 + 64)
    local_scan(2)
    for cp in wo_cp:
        cp.wait()
    won[3, 0:D, :] = jnp.concatenate([woraw[:, 384:D], jnp.zeros((D, 64), BF16)], axis=1)
    prep_xa([1, 2, 3])
    pacer.finish()
    local_scan(3)

    row = lax.broadcasted_iota(jnp.int32, (JG, 128), 0)
    hu = h_s.bitcast(U32)

    def scan_chunk(g, c, prev):
        nparts = 2 if c < 3 else 1
        load = partial(load_bu, g, c)
        f = [fin[_ds(g * JG, JG), (2 * c + k) * 128:(2 * c + k + 1) * 128] for k in range(2)]
        s = tuple(pltpu.roll(jnp.where(row == JG - 1, p, x), 1, 0) for p, x in zip(prev, f))
        for m in range(5):
            sh = tuple(jnp.where(row >= 2 ** m, pltpu.roll(x, 2 ** m, 0), 0.0) for x in s)
            s = _step(lam_pows[m][c], sh, s)
        for rho in range(R // 2):
            e = _step(lam1[c], s, gate(*load(2 * rho)))
            s = _step(lam1[c], e, load(2 * rho + 1))
            for k in range(nparts):
                hu[(2 * c + k) * G + g, pl.ds(rho, JG, stride=R // 2), :] = _pack(e[k], s[k])
        return s

    def qkv_part(r, part):
        dst, i = ((q_s, r), (k_s, R + r), (v_s, R + r))[part]
        res = lax.dot_general(_bf16(wt[part * D // 2:(part + 1) * D // 2, :], D),
                              _bf16(xap[_ds(r * 64, 64), :], D), NT, preferred_element_type=F32)
        dst[i] = res
        return res

    def shift_kv(r):
        k_s[r] = pltpu.roll(k_s[R + r], 1, 1)
        v_s[r] = pltpu.roll(v_s[R + r], 1, 1)

    def prep_wo(c):
        wu = won.bitcast(U32)
        for dp in range(DH // 2):
            lo, hi = _unpack(wu[c, pl.ds(dp, H, stride=DH // 2), :])
            wop[dp * H:dp * H + H // 2, :] = lo
            wop[dp * H + H // 2:(dp + 1) * H, :] = hi
        wop[D // 2:256, :] = jnp.zeros((256 - D // 2, 128), U32)
        wot[_ds(c * 64, 64), :] = pltpu.bitcast(_bf16(wop[...]).T, U32)

    def phase2a(g, prev):
        last = []
        for i in range(2):
            r = 4 * g + 2 * i
            pacer.pace([partial(qkv_part, r, k) for k in (1, 2, 0)], 18)
            last.append(scan_chunk(g, 2 * i, prev[2 * i]))
            last.append(scan_chunk(g, 2 * i + 1, prev[2 * i + 1]))
            pacer.finish()
            shift_kv(r)
        prep_wo(g)
        return tuple(last)

    zero = jnp.zeros((JG, 128), F32)
    _loop(phase2a, ((zero, zero),) * 4)

    lane_h = lax.broadcasted_iota(jnp.int32, (H, 128), 1)
    scale = DH ** -0.5

    def attend(r, odd):
        acc = [None] * W
        for d in range(DH):
            rows = slice(d * H, (d + 1) * H)
            qd = gate(q_s[r, rows, :])
            for w in range(W):
                t = qd * k_s[R + r - 2 * w, rows, :]
                acc[w] = t if d == 0 else acc[w] + t
        lg = []
        for w in range(W):
            first = jnp.where(r < 2 * w, 1, 0)
            lg.append(jnp.where(lane_h < first, -1e9, acc[w] * scale))
        m = lg[0]
        for w in range(1, W):
            m = jnp.maximum(m, lg[w])
        e = [jnp.exp(x - m) for x in lg]
        tot = e[0]
        for w in range(1, W):
            tot = tot + e[w]
        inv = 1.0 / tot
        p = [x * inv for x in e]
        for d in range(DH):
            rows = slice(d * H, (d + 1) * H)
            o = gate(p[0] * v_s[R + r, rows, :])
            for w in range(1, W):
                o = o + p[w] * v_s[R + r - 2 * w, rows, :]
            if odd:
                ow[rows, :] = _pack(q_s[r - 1, rows, :], o)
            else:
                q_s[r, rows, :] = o

    def prep_c(r0):
        src, dst = _ds(r0, D // G, 16), _ds(r0 // 2, D // G // 2, 8)
        for c in range(4):
            sl = slice(c * 128, min(D, (c + 1) * 128))
            xr, xi = cre[src, sl].astype(F32), cim[src, sl].astype(F32)
            cr, ci = co_re[:, sl], co_im[:, sl]
            yr, yi = xr * cr - xi * ci, -(xr * ci + xi * cr)
            if c < 3:
                cst[dst, c * 256:c * 256 + 128] = _words(yr)
                cst[dst, c * 256 + 128:c * 256 + 256] = _words(yi)
            else:
                cst[dst, 768:896] = _words(jnp.concatenate([yr, yi], axis=1))

    for cp in c_cp:
        cp.wait()

    for r in range(0, R, 2):
        pacer.pace([partial(qkv_part, r + 1, k) for k in (1, 2)], 2 * DH + 1)
        attend(r, False)
        shift_kv(r + 1)
        if r % 4 == 2:
            prep_c(r // 4 * (D // G))

    def y_copy(i):
        rows = _ds(i * TP, TP)
        return copy(ob.at[rows, pl.ds(512, 384)], out_hbm.at[0, rows, pl.ds(512, 384)], sem_out.at[i])

    def a_copy(i):
        rows = _ds(i * TP, TP)
        return copy(ob.at[rows, pl.ds(0, 512)], out_hbm.at[0, rows, pl.ds(0, 512)], sem_out.at[NP + i])

    def y_piece(i):
        rows = _ds(i * TP, TP)
        sub = _ds((i % (TG // TP)) * TP, TP)
        hh = jnp.concatenate([h_s[k * G + i // (TG // TP), sub, :] for k in range(7)], axis=1)
        res = lax.dot_general(_bf16(cst[...]), hh, NT, preferred_element_type=F32)
        y = res + xbt[0:D, rows] * dcol[0:D, :]
        ylow[i] = y[0:64]
        for n in range(3):
            ob[rows, 512 + n * 128:640 + n * 128] = y[64 + n * 128:192 + n * 128].T
        y_copy(i).start()
        return res

    qkv_part(1, 0)
    for i in range(R // 2):
        nxt = [partial(qkv_part, 2 * i + 3, 0)] if i < R // 2 - 1 else []
        ys = [partial(y_piece, k) for k in range(NY * i // 8, NY * (i + 1) // 8)]
        pacer.pace(nxt + ys, 2 * DH + 4)
        attend(2 * i + 1, True)
        for c in range(4):
            o_s[c * NP:(c + 1) * NP, i * 8:(i + 1) * 8, :] = (
                ow[c * 128:(c + 1) * 128, :].T.reshape(NP, 8, 128))
        pacer.finish()

    def a_piece(i):
        rows = _ds(i * TP, TP)
        oo = jnp.concatenate([
            _bf16(jnp.concatenate(
                [o_s[c * NP + i, pl.ds(j, R // 2, stride=8), :]
                 for j in range(TP // R)], axis=0))
            for c in range(4)], axis=1)
        a = lax.dot_general(_bf16(wot[0:D // 2, :]), oo, NT, preferred_element_type=F32)
        for n in range(3):
            ob[rows, n * 128:(n + 1) * 128] = a[n * 128:(n + 1) * 128].T
        ob[rows, 384:512] = jnp.concatenate([a[384:D], ylow[i]], axis=0).T
        a_copy(i).start()

    def phase4(g, carry):
        for k in range(1):
            y_piece(NY + g * 1 + k)
        for k in range(4):
            a_piece(g * 4 + k)
        return carry

    lax.fori_loop(0, 4, phase4, 0)
    for i in range(NP):
        y_copy(i).wait()
        a_copy(i).wait()


@jax.jit
def pallas_concat_heads__sliding_local_dilated__ssm_conv_s5__prompt_kernel(
    A_x, A_wqkv, A_wo, B_x, B_Lambda_re, B_Lambda_im, B_B_re, B_B_im, B_C_re, B_C_im,
    B_log_dt, B_Dskip,
):
    hbm = pl.BlockSpec(memory_space=pl.ANY)
    vm = pltpu.VMEM
    dma = pltpu.SemaphoreType.DMA
    scratch = [vm((D,), BF16)] * 4 + [
        vm((512, S), BF16), vm((512, S), BF16),
        vm((4 * S + 16, 128), BF16), vm((4 * S + 16, 128), BF16),
        vm((S // 2, 512), U32), vm((S // 2, 512), U32),
        vm((2 * D, D), BF16),
        vm((S, 2 * D), F32),
        vm((D, 3 * D), BF16),
        vm((4 * 1408, 128), BF16),
        vm((3 * D // 2, 512), U32),
        vm((R, D, 128), F32),
        vm((2 * R, D, 128), F32), vm((2 * R, D, 128), F32),
        vm((7 * G, TG + 16, 128), BF16),
        vm((4 * NP, TP // 2 + 8, 128), U32),
        vm((D, D), BF16), vm((D, D), BF16),
        vm((D // 2, 2 * D), U32),
        vm((D, D), BF16), vm((4, D + 32, 128), BF16),
        vm((256, 128), U32), vm((256, 512), U32),
        vm((512, 128), U32),
        vm((512, 128), F32),
        vm((NP, 64, 128), F32),
        vm((G * JG, 1024), F32),
        vm((S, 2 * D), F32),
        dma((G,)), dma((7,)), dma((6,)), dma((2 * NP,)),
    ]
    return pl.pallas_call(
        _kernel,
        out_shape=jax.ShapeDtypeStruct((1, S, 2 * D), F32),
        in_specs=[hbm] * 12,
        out_specs=hbm,
        scratch_shapes=scratch,
        compiler_params=pltpu.CompilerParams(
            vmem_limit_bytes=100 * 1024 * 1024,
            flags={"XLA_TPU_EVENLY_DISTRIBUTE_CRITICAL_NODES": True}),
    )(jnp.swapaxes(A_x, 1, 2), A_wqkv, A_wo, jnp.swapaxes(B_x, 1, 2), B_Lambda_re, B_Lambda_im,
      B_B_re, B_B_im, B_C_re, B_C_im, B_log_dt, B_Dskip)
```

```python
from functools import partial
from itertools import chain

import jax
import jax.numpy as jnp
from jax import lax
import jax.experimental.pallas as pl
import jax.experimental.pallas.tpu as pltpu

S = 2048
D = 448
H = 16
DH = 28
W = 8
R = 16
G = 4
TG = S // G
JG = TG // R
TP = 128
NP = S // TP
NY = 12

F32 = jnp.float32
BF16 = jnp.bfloat16
U32 = jnp.uint32
NT = (((1,), (1,)), ((), ()))


def _unpack(w):
    lo = pltpu.bitcast(w.astype(jnp.uint16), U32)
    hi = pltpu.bitcast((w >> 16).astype(jnp.uint16), U32)
    return lo, hi


def _pack(even, odd):
    return pltpu.bitcast(pltpu.pack_elementwise([even, odd], packed_dtype=BF16), U32)


def _words(x):
    return pltpu.bitcast(x.astype(BF16), U32)


def _bf16(w, cols=None):
    x = pltpu.bitcast(w, BF16)
    return x if cols is None else x[:, :cols]


def _ds(start, size, align=None):
    return pl.ds(pl.multiple_of(start, align or size), size)


def _step(lam, h, b):
    lr, li = lam
    return (lr * h[0] - li * h[1] + b[0], lr * h[1] + li * h[0] + b[1])


def _lam_tiles(re, im, lane):
    out = [(re[:, c * 128:(c + 1) * 128], im[:, c * 128:(c + 1) * 128]) for c in range(3)]
    z = jnp.zeros((1, 64), F32)
    r3 = jnp.concatenate([re[:, 384:], z], axis=1)
    i3 = jnp.concatenate([im[:, 384:], z], axis=1)
    out.append((jnp.where(lane < 64, r3, pltpu.roll(r3, 64, 1)),
                jnp.where(lane < 64, i3, -pltpu.roll(i3, 64, 1))))
    return out


class _Pacer:
    def __init__(self):
        self.zero = lax.broadcasted_iota(U32, (8, 128), 1) >> 16

    def pace(self, matmuls, steps):
        self.queue = list(matmuls)
        self.per = -(-steps // len(matmuls))
        self.pos = 0

    def gate(self, *xs):
        i = self.pos % self.per
        if i == 0 and not self.queue:
            return xs if len(xs) > 1 else xs[0]
        if i == 0:
            self.res = self.queue.pop(0)()
        self.pos += 1
        k = (self.res.shape[0] // 8 * i) // self.per * 8
        tok = pltpu.bitcast(self.res[k:k + 8, 0:128], U32) & self.zero
        out = []
        for x in xs:
            u = pltpu.bitcast(x, U32)
            u = u | jnp.tile(tok, (u.shape[0] // 8, u.shape[1] // 128))
            out.append(pltpu.bitcast(u, x.dtype))
        return out if len(out) > 1 else out[0]

    def finish(self):
        while self.queue:
            self.queue.pop(0)()
        self.pos = 0


def _run(*tasks):
    for _ in chain(*tasks):
        pass


def _loop(body, init, unroll=2):
    def outer(t, carry):
        for u in range(unroll):
            carry = body(t * unroll + u, carry)
        return carry
    return lax.fori_loop(0, G // unroll, outer, init)


def _kernel(xa_hbm, wqkv_hbm, wo_hbm, xb_hbm, lre_hbm, lim_hbm, bre_hbm, bim_hbm,
            cre_hbm, cim_hbm, ldt_hbm, dsk_hbm, out_hbm,
            lre, lim, ldt, dsk, xat, xbt, xan, xbn, xap, xbp, bst, bu, wraw, wtn, wt,
            q_s, k_s, v_s, h_s, o_s, cre, cim, cst, woraw, won, wop, wot, ow, dcol, ylow, fin, ob,
            sem_xb, sem_b, sem_in, sem_out):
    copy = pltpu.make_async_copy
    xb_cp = [copy(xb_hbm.at[0, :, pl.ds(g * TG, TG)], xbt.at[pl.ds(0, D), pl.ds(g * TG, TG)],
                  sem_xb.at[g]) for g in range(G)]
    b_cp = []
    for c in range(3):
        b_cp.append([copy(bre_hbm.at[pl.ds(c * 128, 128)], bst.at[pl.ds(c * 256, 128)], sem_b.at[2 * c])])
        b_cp.append([copy(bim_hbm.at[pl.ds(c * 128, 128)], bst.at[pl.ds(c * 256 + 128, 128)],
                          sem_b.at[2 * c + 1])])
    b_cp.append([copy(bre_hbm.at[pl.ds(384, 64)], bst.at[pl.ds(768, 64)], sem_b.at[6]),
                 copy(bim_hbm.at[pl.ds(384, 64)], bst.at[pl.ds(832, 64)], sem_b.at[6])])
    p_cp = [copy(src, dst, sem_in.at[5]) for src, dst in
            ((lre_hbm, lre), (lim_hbm, lim), (ldt_hbm, ldt), (dsk_hbm, dsk))]
    w_cp = copy(wqkv_hbm, wraw, sem_in.at[0])
    xa_cp = [copy(xa_hbm.at[0, pl.ds(lo, n)], xat.at[pl.ds(lo, n)], sem_in.at[i])
             for lo, n, i in ((0, 128, 1), (128, D - 128, 6))]
    c_cp = [copy(cre_hbm, cre, sem_in.at[2]), copy(cim_hbm, cim, sem_in.at[3])]
    wo_cp = [copy(wo_hbm.at[:, pl.ds(c * 128, 128)], won.at[c, pl.ds(0, D)], sem_in.at[4]) for c in range(3)]
    wo_cp.append(copy(wo_hbm, woraw, sem_in.at[4]))

    for cp in [xb_cp[0]] + sum(b_cp, []) + p_cp:
        cp.start()

    xat[D:512, :] = jnp.zeros((512 - D, S), BF16)
    xbt[D:512, :] = jnp.zeros((512 - D, S), BF16)
    ow[D:512, :] = jnp.zeros((512 - D, 128), U32)
    xan[4 * S:, :] = jnp.zeros((16, 128), BF16)
    xbn[4 * S:, :] = jnp.zeros((16, 128), BF16)
    won[:, D:, :] = jnp.zeros((4, 32, 128), BF16)
    o_s[:, TP // 2:, :] = jnp.zeros((4 * NP, 8, 128), U32)
    pacer = _Pacer()
    gate = pacer.gate

    def transpose_x(xt_ref, xn_ref, c, g):
        for t in range(g * TG, (g + 1) * TG, 128):
            xn_ref[pl.ds(c * S + t, 128), :] = gate(xt_ref[c * 128:(c + 1) * 128, t:t + 128]).T
            yield

    def gather_x(xn_ref, xp_ref, c, row0, rhos, nj, g8=gate):
        xu = xn_ref.bitcast(U32)
        for rho in rhos:
            lo, hi = _unpack(g8(xu[pl.ds(c * (S // 2) + row0 + rho, nj, stride=R // 2), :]))
            dst = row0 + rho * nj
            xp_ref[dst:dst + nj // 2, c * 128:(c + 1) * 128] = lo
            xp_ref[dst + nj // 2:dst + nj, c * 128:(c + 1) * 128] = hi
            yield

    def w_transpose(n):
        cols = min(128, 3 * D - n * 128)
        for c in range(4):
            rows = min(128, D - c * 128)
            v = wraw[c * 128:c * 128 + rows, n * 128:n * 128 + cols]
            if rows < 128:
                v = jnp.concatenate([v, jnp.zeros((128 - rows, cols), BF16)], axis=0)
            if cols < 128:
                v = jnp.concatenate([v, jnp.zeros((128, 128 - cols), BF16)], axis=1)
            wtn[pl.ds(c * 1408 + n * 128, 128), :] = gate(v).T
            yield

    def w_gather(part, c):
        wu = wtn.bitcast(U32)
        for dp in range(DH // 2):
            lo, hi = _unpack(gate(wu[pl.ds(c * 704 + part * (D // 2) + dp, H, stride=DH // 2), :]))
            base = part * (D // 2) + dp * H
            wt[base:base + H // 2, c * 128:(c + 1) * 128] = lo
            wt[base + H // 2:base + H, c * 128:(c + 1) * 128] = hi
            yield

    def bu_piece(g, n):
        res = lax.dot_general(_bf16(xbp[g * TG // 2:(g + 1) * TG // 2, :], D),
                              bst[n * 128:(n + 1) * 128, :], NT, preferred_element_type=F32)
        bu[g * TG:(g + 1) * TG, n * 128:(n + 1) * 128] = res
        return res

    def prep_xb(g):
        for c in range(4):
            yield from transpose_x(xbt, xbn, c, g)
            yield from gather_x(xbn, xbp, c, g * (TG // 2), range(R // 2), JG)

    def prep_xa(cs):
        for c in cs:
            for g in range(G):
                yield from transpose_x(xat, xan, c, g)
            yield from gather_x(xan, xap, c, 0, range(R // 2), 128)

    xb_cp[0].wait()
    for cp in [xb_cp[1], w_cp, xb_cp[2]]:
        cp.start()
    for c in range(4):
        xbn[pl.ds(c * S, TG), :] = xbt[c * 128:(c + 1) * 128, 0:TG].T
        _run(gather_x(xbn, xbp, c, 0, range(R // 2), JG, lambda v: v))

    def load_bu(g, c, r):
        v = [bu[_ds(g * TG + r * JG, JG), c * 256 + k * 128:c * 256 + (k + 1) * 128]
             for k in range(2 if c < 3 else 1)]
        return v if c < 3 else (v[0], pltpu.roll(v[0], 64, 1))

    def local_scan(g):
        for c in range(4):
            f = gate(*load_bu(g, c, 0))
            for r in range(1, R):
                f = _step(lam1[c], f, gate(*load_bu(g, c, r)))
                yield
            for k in range(2):
                fin[g * JG:(g + 1) * JG, (2 * c + k) * 128:(2 * c + k + 1) * 128] = f[k]

    def bu_chunk(g, steps):
        pacer.pace([partial(bu_piece, g, n) for n in range(7)], steps)

    for cp in b_cp[0] + b_cp[1]:
        cp.wait()
    bu_chunk(0, 70)
    for _ in range(20):
        gate(pacer.zero)
    for cp in sum(b_cp[2:], []):
        cp.wait()
    xb_cp[1].wait()
    _run(prep_xb(1))
    for cp in p_cp:
        cp.wait()
    lane = lax.broadcasted_iota(jnp.int32, (1, 128), 1)
    a_re = lre[...].astype(F32).reshape(1, D)
    a_im = lim[...].astype(F32).reshape(1, D)
    dt = jnp.exp(ldt[...].astype(F32).reshape(1, D)).astype(BF16).astype(F32)
    mag = jnp.exp(dt * a_re)
    l_re = mag * jnp.cos(dt * a_im)
    l_im = mag * jnp.sin(dt * a_im)
    den = a_re * a_re + a_im * a_im
    n_re = l_re - 1.0
    co_re = 2.0 * (n_re * a_re + l_im * a_im) / den
    co_im = 2.0 * (l_im * a_re - n_re * a_im) / den
    lam1 = _lam_tiles(l_re, l_im, lane)
    p_re, p_im = l_re, l_im
    for _ in range(4):
        p_re, p_im = p_re * p_re - p_im * p_im, 2.0 * p_re * p_im
    lam_pows = []
    for _ in range(5):
        lam_pows.append(_lam_tiles(p_re, p_im, lane))
        p_re, p_im = p_re * p_re - p_im * p_im, 2.0 * p_re * p_im
    drow = jnp.concatenate([dsk[...].astype(F32).reshape(1, D), jnp.zeros((1, 64), F32)], axis=1)
    dcol[...] = jnp.broadcast_to(drow, (128, 512)).T

    pacer.finish()

    for cp in (xb_cp[3], xa_cp[0]):
        cp.start()
    bu_chunk(1, 28 + 48 + 12 + 56 + 64)
    w_cp.wait()
    xb_cp[2].wait()
    _run(chain(*[w_transpose(n) for n in range(10)], prep_xb(2),
               *[w_gather(0, c) for c in range(4)]), local_scan(0))
    pacer.finish()

    xa_cp[1].start()
    bu_chunk(2, 4 + 48 + 112 + 24 + 64)
    xa_cp[0].wait()
    xb_cp[3].wait()
    _run(chain(w_transpose(10), prep_xb(3), *[w_gather(p, c) for p in (1, 2) for c in range(4)],
               prep_xa([0])), local_scan(1))
    pacer.finish()

    for cp in wo_cp + c_cp:
        cp.start()
    xa_cp[1].wait()
    bu_chunk(3, 78 + 64)
    _run(prep_xa([1, 2, 3]), local_scan(2))
    pacer.finish()
    _run(local_scan(3))
    for cp in wo_cp:
        cp.wait()
    won[3, 0:D, :] = jnp.concatenate([woraw[:, 384:D], jnp.zeros((D, 64), BF16)], axis=1)

    row = lax.broadcasted_iota(jnp.int32, (JG, 128), 0)
    hu = h_s.bitcast(U32)

    def scan_chunk(g, c, prev):
        nparts = 2 if c < 3 else 1
        load = partial(load_bu, g, c)
        f = [fin[_ds(g * JG, JG), (2 * c + k) * 128:(2 * c + k + 1) * 128] for k in range(2)]
        s = tuple(pltpu.roll(jnp.where(row == JG - 1, p, x), 1, 0) for p, x in zip(prev, f))
        for m in range(5):
            sh = tuple(jnp.where(row >= 2 ** m, pltpu.roll(x, 2 ** m, 0), 0.0) for x in s)
            s = _step(lam_pows[m][c], sh, s)
        for rho in range(R // 2):
            e = _step(lam1[c], s, gate(*load(2 * rho)))
            s = _step(lam1[c], e, load(2 * rho + 1))
            for k in range(nparts):
                hu[(2 * c + k) * G + g, pl.ds(rho, JG, stride=R // 2), :] = _pack(e[k], s[k])
        return s

    def qkv_part(r, part):
        dst, i = ((q_s, r), (k_s, R + r), (v_s, R + r))[part]
        res = lax.dot_general(_bf16(wt[part * D // 2:(part + 1) * D // 2, :], D),
                              _bf16(xap[_ds(r * 64, 64), :], D), NT, preferred_element_type=F32)
        dst[i] = res
        return res

    def shift_kv(r):
        k_s[r] = pltpu.roll(k_s[R + r], 1, 1)
        v_s[r] = pltpu.roll(v_s[R + r], 1, 1)

    def prep_wo(c):
        wu = won.bitcast(U32)
        for dp in range(DH // 2):
            lo, hi = _unpack(wu[c, pl.ds(dp, H, stride=DH // 2), :])
            wop[dp * H:dp * H + H // 2, :] = lo
            wop[dp * H + H // 2:(dp + 1) * H, :] = hi
        wop[D // 2:256, :] = jnp.zeros((256 - D // 2, 128), U32)
        wot[_ds(c * 64, 64), :] = pltpu.bitcast(_bf16(wop[...]).T, U32)

    def phase2a(g, prev):
        last = []
        for i in range(2):
            r = 4 * g + 2 * i
            pacer.pace([partial(qkv_part, r, k) for k in (1, 2, 0)], 18)
            last.append(scan_chunk(g, 2 * i, prev[2 * i]))
            last.append(scan_chunk(g, 2 * i + 1, prev[2 * i + 1]))
            pacer.finish()
            shift_kv(r)
        prep_wo(g)
        return tuple(last)

    zero = jnp.zeros((JG, 128), F32)
    _loop(phase2a, ((zero, zero),) * 4)

    lane_h = lax.broadcasted_iota(jnp.int32, (H, 128), 1)
    scale = DH ** -0.5

    def attend(r, odd):
        acc = [None] * W
        for d in range(DH):
            rows = slice(d * H, (d + 1) * H)
            qd = gate(q_s[r, rows, :])
            for w in range(W):
                t = qd * k_s[R + r - 2 * w, rows, :]
                acc[w] = t if d == 0 else acc[w] + t
        lg = []
        for w in range(W):
            first = jnp.where(r < 2 * w, 1, 0)
            lg.append(jnp.where(lane_h < first, -1e9, acc[w] * scale))
        m = lg[0]
        for w in range(1, W):
            m = jnp.maximum(m, lg[w])
        e = [jnp.exp(x - m) for x in lg]
        tot = e[0]
        for w in range(1, W):
            tot = tot + e[w]
        inv = 1.0 / tot
        p = [x * inv for x in e]
        for d in range(DH):
            rows = slice(d * H, (d + 1) * H)
            o = gate(p[0] * v_s[R + r, rows, :])
            for w in range(1, W):
                o = o + p[w] * v_s[R + r - 2 * w, rows, :]
            if odd:
                ow[rows, :] = _pack(q_s[r - 1, rows, :], o)
            else:
                q_s[r, rows, :] = o

    def prep_c(r0):
        src, dst = _ds(r0, D // G, 16), _ds(r0 // 2, D // G // 2, 8)
        for c in range(4):
            sl = slice(c * 128, min(D, (c + 1) * 128))
            xr, xi = cre[src, sl].astype(F32), cim[src, sl].astype(F32)
            cr, ci = co_re[:, sl], co_im[:, sl]
            yr, yi = xr * cr - xi * ci, -(xr * ci + xi * cr)
            if c < 3:
                cst[dst, c * 256:c * 256 + 128] = _words(yr)
                cst[dst, c * 256 + 128:c * 256 + 256] = _words(yi)
            else:
                cst[dst, 768:896] = _words(jnp.concatenate([yr, yi], axis=1))

    for cp in c_cp:
        cp.wait()

    for r in range(0, R, 2):
        pacer.pace([partial(qkv_part, r + 1, k) for k in (1, 2)], 2 * DH + 1)
        attend(r, False)
        shift_kv(r + 1)
        if r % 4 == 2:
            prep_c(r // 4 * (D // G))

    def y_copy(i):
        rows = _ds(i * TP, TP)
        return copy(ob.at[rows, pl.ds(512, 384)], out_hbm.at[0, rows, pl.ds(512, 384)], sem_out.at[i])

    def a_copy(i):
        rows = _ds(i * TP, TP)
        return copy(ob.at[rows, pl.ds(0, 512)], out_hbm.at[0, rows, pl.ds(0, 512)], sem_out.at[NP + i])

    def y_piece(i):
        rows = _ds(i * TP, TP)
        sub = _ds((i % (TG // TP)) * TP, TP)
        hh = jnp.concatenate([h_s[k * G + i // (TG // TP), sub, :] for k in range(7)], axis=1)
        res = lax.dot_general(_bf16(cst[...]), hh, NT, preferred_element_type=F32)
        y = res + xbt[0:D, rows] * dcol[0:D, :]
        ylow[i] = y[0:64]
        for n in range(3):
            ob[rows, 512 + n * 128:640 + n * 128] = y[64 + n * 128:192 + n * 128].T
        y_copy(i).start()
        return res

    qkv_part(1, 0)
    for i in range(R // 2):
        nxt = [partial(qkv_part, 2 * i + 3, 0)] if i < R // 2 - 1 else []
        ys = [partial(y_piece, k) for k in range(NY * i // 8, NY * (i + 1) // 8)]
        pacer.pace(nxt + ys, 2 * DH + 4)
        attend(2 * i + 1, True)
        for c in range(4):
            o_s[c * NP:(c + 1) * NP, i * 8:(i + 1) * 8, :] = (
                ow[c * 128:(c + 1) * 128, :].T.reshape(NP, 8, 128))
        pacer.finish()

    def a_piece(i):
        rows = _ds(i * TP, TP)
        oo = jnp.concatenate([
            _bf16(jnp.concatenate(
                [o_s[c * NP + i, pl.ds(j, R // 2, stride=8), :]
                 for j in range(TP // R)], axis=0))
            for c in range(4)], axis=1)
        a = lax.dot_general(_bf16(wot[0:D // 2, :]), oo, NT, preferred_element_type=F32)
        for n in range(3):
            ob[rows, n * 128:(n + 1) * 128] = a[n * 128:(n + 1) * 128].T
        ob[rows, 384:512] = jnp.concatenate([a[384:D], ylow[i]], axis=0).T
        a_copy(i).start(priority=1)

    def phase4(g, carry):
        for k in range(4):
            if k == 3:
                y_piece(NY + g)
            a_piece(4 * g + k)
        return carry

    lax.fori_loop(0, 4, phase4, 0)
    for i in range(NP):
        y_copy(i).wait()
        a_copy(i).wait()


@jax.jit
def pallas_concat_heads__sliding_local_dilated__ssm_conv_s5__prompt_kernel(
    A_x, A_wqkv, A_wo, B_x, B_Lambda_re, B_Lambda_im, B_B_re, B_B_im, B_C_re, B_C_im,
    B_log_dt, B_Dskip,
):
    hbm = pl.BlockSpec(memory_space=pl.ANY)
    vm = pltpu.VMEM
    dma = pltpu.SemaphoreType.DMA
    scratch = [vm((D,), BF16)] * 4 + [
        vm((512, S), BF16), vm((512, S), BF16),
        vm((4 * S + 16, 128), BF16), vm((4 * S + 16, 128), BF16),
        vm((S // 2, 512), U32), vm((S // 2, 512), U32),
        vm((2 * D, D), BF16),
        vm((S, 2 * D), F32),
        vm((D, 3 * D), BF16),
        vm((4 * 1408, 128), BF16),
        vm((3 * D // 2, 512), U32),
        vm((R, D, 128), F32),
        vm((2 * R, D, 128), F32), vm((2 * R, D, 128), F32),
        vm((7 * G, TG + 16, 128), BF16),
        vm((4 * NP, TP // 2 + 8, 128), U32),
        vm((D, D), BF16), vm((D, D), BF16),
        vm((D // 2, 2 * D), U32),
        vm((D, D), BF16), vm((4, D + 32, 128), BF16),
        vm((256, 128), U32), vm((256, 512), U32),
        vm((512, 128), U32),
        vm((512, 128), F32),
        vm((NP, 64, 128), F32),
        vm((G * JG, 1024), F32),
        vm((S, 2 * D), F32),
        dma((G,)), dma((7,)), dma((7,)), dma((2 * NP,)),
    ]
    return pl.pallas_call(
        _kernel,
        out_shape=jax.ShapeDtypeStruct((1, S, 2 * D), F32),
        in_specs=[hbm] * 12,
        out_specs=hbm,
        scratch_shapes=scratch,
        compiler_params=pltpu.CompilerParams(
            vmem_limit_bytes=100 * 1024 * 1024,
            flags={"XLA_TPU_EVENLY_DISTRIBUTE_CRITICAL_NODES": True}),
    )(jnp.swapaxes(A_x, 1, 2), A_wqkv, A_wo, jnp.swapaxes(B_x, 1, 2), B_Lambda_re, B_Lambda_im,
      B_B_re, B_B_im, B_C_re, B_C_im, B_log_dt, B_Dskip)
```

```python
from functools import partial
from itertools import chain

import jax
import jax.numpy as jnp
from jax import lax
import jax.experimental.pallas as pl
import jax.experimental.pallas.tpu as pltpu

S = 2048
D = 448
H = 16
DH = 28
W = 8
R = 16
G = 4
TG = S // G
JG = TG // R
TP = 128
NP = S // TP
NY = 12

F32 = jnp.float32
BF16 = jnp.bfloat16
U32 = jnp.uint32
NT = (((1,), (1,)), ((), ()))


def _unpack(w):
    lo = pltpu.bitcast(w.astype(jnp.uint16), U32)
    hi = pltpu.bitcast((w >> 16).astype(jnp.uint16), U32)
    return lo, hi


def _pack(even, odd):
    return pltpu.bitcast(pltpu.pack_elementwise([even, odd], packed_dtype=BF16), U32)


def _words(x):
    return pltpu.bitcast(x.astype(BF16), U32)


def _bf16(w, cols=None):
    x = pltpu.bitcast(w, BF16)
    return x if cols is None else x[:, :cols]


def _ds(start, size, align=None):
    return pl.ds(pl.multiple_of(start, align or size), size)


def _step(lam, h, b):
    lr, li = lam
    return (lr * h[0] - li * h[1] + b[0], lr * h[1] + li * h[0] + b[1])


def _lam_tiles(re, im, lane):
    out = [(re[:, c * 128:(c + 1) * 128], im[:, c * 128:(c + 1) * 128]) for c in range(3)]
    z = jnp.zeros((1, 64), F32)
    r3 = jnp.concatenate([re[:, 384:], z], axis=1)
    i3 = jnp.concatenate([im[:, 384:], z], axis=1)
    out.append((jnp.where(lane < 64, r3, pltpu.roll(r3, 64, 1)),
                jnp.where(lane < 64, i3, -pltpu.roll(i3, 64, 1))))
    return out


class _Pacer:
    def __init__(self):
        self.zero = lax.broadcasted_iota(U32, (8, 128), 1) >> 16

    def pace(self, matmuls, steps):
        self.queue = list(matmuls)
        self.per = -(-steps // len(matmuls))
        self.pos = 0

    def gate(self, *xs):
        i = self.pos % self.per
        if i == 0 and not self.queue:
            return xs if len(xs) > 1 else xs[0]
        if i == 0:
            self.res = self.queue.pop(0)()
        self.pos += 1
        k = (self.res.shape[0] // 8 * i) // self.per * 8
        tok = pltpu.bitcast(self.res[k:k + 8, 0:128], U32) & self.zero
        out = []
        for x in xs:
            u = pltpu.bitcast(x, U32)
            u = u | jnp.tile(tok, (u.shape[0] // 8, u.shape[1] // 128))
            out.append(pltpu.bitcast(u, x.dtype))
        return out if len(out) > 1 else out[0]

    def finish(self):
        while self.queue:
            self.queue.pop(0)()
        self.pos = 0


def _run(*tasks):
    for _ in chain(*tasks):
        pass


def _loop(body, init, unroll=2):
    def outer(t, carry):
        for u in range(unroll):
            carry = body(t * unroll + u, carry)
        return carry
    return lax.fori_loop(0, G // unroll, outer, init)


def _kernel(xa_hbm, wqkv_hbm, wo_hbm, xb_hbm, lre_hbm, lim_hbm, bre_hbm, bim_hbm,
            cre_hbm, cim_hbm, ldt_hbm, dsk_hbm, out_hbm,
            lre, lim, ldt, dsk, xat, xbt, xan, xbn, xap, xbp, bst, bu, wraw, wtn, wt,
            q_s, k_s, v_s, h_s, o_s, cre, cim, cst, woraw, won, wop, wot, ow, dcol, ylow, fin, ob,
            sem_xb, sem_b, sem_in, sem_out):
    copy = pltpu.make_async_copy
    xb_cp = [copy(xb_hbm.at[0, :, pl.ds(g * TG, TG)], xbt.at[pl.ds(0, D), pl.ds(g * TG, TG)],
                  sem_xb.at[g]) for g in range(G)]
    b_cp = []
    for c in range(3):
        b_cp.append([copy(bre_hbm.at[pl.ds(c * 128, 128)], bst.at[pl.ds(c * 256, 128)], sem_b.at[2 * c])])
        b_cp.append([copy(bim_hbm.at[pl.ds(c * 128, 128)], bst.at[pl.ds(c * 256 + 128, 128)],
                          sem_b.at[2 * c + 1])])
    b_cp.append([copy(bre_hbm.at[pl.ds(384, 64)], bst.at[pl.ds(768, 64)], sem_b.at[6]),
                 copy(bim_hbm.at[pl.ds(384, 64)], bst.at[pl.ds(832, 64)], sem_b.at[6])])
    p_cp = [copy(src, dst, sem_in.at[5]) for src, dst in
            ((lre_hbm, lre), (lim_hbm, lim), (ldt_hbm, ldt), (dsk_hbm, dsk))]
    w_cp = copy(wqkv_hbm, wraw, sem_in.at[0])
    xa_cp = [copy(xa_hbm.at[0, pl.ds(lo, n)], xat.at[pl.ds(lo, n)], sem_in.at[i])
             for lo, n, i in ((0, 128, 1), (128, D - 128, 6))]
    c_cp = [copy(cre_hbm, cre, sem_in.at[2]), copy(cim_hbm, cim, sem_in.at[3])]
    wo_cp = [copy(wo_hbm.at[:, pl.ds(c * 128, 128)], won.at[c, pl.ds(0, D)], sem_in.at[4]) for c in range(3)]
    wo_cp.append(copy(wo_hbm, woraw, sem_in.at[4]))

    for cp in [xb_cp[0]] + sum(b_cp, []) + p_cp:
        cp.start()

    xat[D:512, :] = jnp.zeros((512 - D, S), BF16)
    xbt[D:512, :] = jnp.zeros((512 - D, S), BF16)
    ow[D:512, :] = jnp.zeros((512 - D, 128), U32)
    xan[4 * S:, :] = jnp.zeros((16, 128), BF16)
    xbn[4 * S:, :] = jnp.zeros((16, 128), BF16)
    won[:, D:, :] = jnp.zeros((4, 32, 128), BF16)
    o_s[:, TP // 2:, :] = jnp.zeros((4 * NP, 8, 128), U32)
    pacer = _Pacer()
    gate = pacer.gate

    def transpose_x(xt_ref, xn_ref, c, g):
        for t in range(g * TG, (g + 1) * TG, 128):
            xn_ref[pl.ds(c * S + t, 128), :] = gate(xt_ref[c * 128:(c + 1) * 128, t:t + 128]).T
            yield

    def gather_x(xn_ref, xp_ref, c, row0, rhos, nj, g8=gate):
        xu = xn_ref.bitcast(U32)
        for rho in rhos:
            lo, hi = _unpack(g8(xu[pl.ds(c * (S // 2) + row0 + rho, nj, stride=R // 2), :]))
            dst = row0 + rho * nj
            xp_ref[dst:dst + nj // 2, c * 128:(c + 1) * 128] = lo
            xp_ref[dst + nj // 2:dst + nj, c * 128:(c + 1) * 128] = hi
            yield

    def w_transpose(n):
        cols = min(128, 3 * D - n * 128)
        for c in range(4):
            rows = min(128, D - c * 128)
            v = wraw[c * 128:c * 128 + rows, n * 128:n * 128 + cols]
            if rows < 128:
                v = jnp.concatenate([v, jnp.zeros((128 - rows, cols), BF16)], axis=0)
            if cols < 128:
                v = jnp.concatenate([v, jnp.zeros((128, 128 - cols), BF16)], axis=1)
            wtn[pl.ds(c * 1408 + n * 128, 128), :] = gate(v).T
            yield

    def w_gather(part, c):
        wu = wtn.bitcast(U32)
        for dp in range(DH // 2):
            lo, hi = _unpack(gate(wu[pl.ds(c * 704 + part * (D // 2) + dp, H, stride=DH // 2), :]))
            base = part * (D // 2) + dp * H
            wt[base:base + H // 2, c * 128:(c + 1) * 128] = lo
            wt[base + H // 2:base + H, c * 128:(c + 1) * 128] = hi
            yield

    def bu_piece(g, n):
        res = lax.dot_general(_bf16(xbp[g * TG // 2:(g + 1) * TG // 2, :], D),
                              bst[n * 128:(n + 1) * 128, :], NT, preferred_element_type=F32)
        bu[g * TG:(g + 1) * TG, n * 128:(n + 1) * 128] = res
        return res

    def prep_xb(g):
        for c in range(4):
            yield from transpose_x(xbt, xbn, c, g)
            yield from gather_x(xbn, xbp, c, g * (TG // 2), range(R // 2), JG)

    def prep_xa(cs):
        for c in cs:
            for g in range(G):
                yield from transpose_x(xat, xan, c, g)
            yield from gather_x(xan, xap, c, 0, range(R // 2), 128)

    xb_cp[0].wait()
    for cp in [xb_cp[1], w_cp, xb_cp[2]]:
        cp.start()
    for c in range(4):
        xbn[pl.ds(c * S, TG), :] = xbt[c * 128:(c + 1) * 128, 0:TG].T
        _run(gather_x(xbn, xbp, c, 0, range(R // 2), JG, lambda v: v))

    def load_bu(g, c, r):
        v = [bu[_ds(g * TG + r * JG, JG), c * 256 + k * 128:c * 256 + (k + 1) * 128]
             for k in range(2 if c < 3 else 1)]
        return v if c < 3 else (v[0], pltpu.roll(v[0], 64, 1))

    def local_scan(g):
        for c in range(4):
            f = gate(*load_bu(g, c, 0))
            for r in range(1, R):
                f = _step(lam1[c], f, gate(*load_bu(g, c, r)))
                yield
            for k in range(2):
                fin[g * JG:(g + 1) * JG, (2 * c + k) * 128:(2 * c + k + 1) * 128] = f[k]

    def bu_chunk(g, steps):
        pacer.pace([partial(bu_piece, g, n) for n in range(7)], steps)

    for cp in b_cp[0] + b_cp[1]:
        cp.wait()
    bu_chunk(0, 70)
    for _ in range(20):
        gate(pacer.zero)
    for cp in sum(b_cp[2:], []):
        cp.wait()
    xb_cp[1].wait()
    _run(prep_xb(1))
    for cp in p_cp:
        cp.wait()
    lane = lax.broadcasted_iota(jnp.int32, (1, 128), 1)
    a_re = lre[...].astype(F32).reshape(1, D)
    a_im = lim[...].astype(F32).reshape(1, D)
    dt = jnp.exp(ldt[...].astype(F32).reshape(1, D)).astype(BF16).astype(F32)
    mag = jnp.exp(dt * a_re)
    l_re = mag * jnp.cos(dt * a_im)
    l_im = mag * jnp.sin(dt * a_im)
    big = jnp.maximum(jnp.abs(a_re), jnp.abs(a_im))
    u_re, u_im = a_re / big, a_im / big
    den = (u_re * u_re + u_im * u_im) * big
    n_re = l_re - 1.0
    co_re = 2.0 * (n_re * u_re + l_im * u_im) / den
    co_im = 2.0 * (l_im * u_re - n_re * u_im) / den
    lam1 = _lam_tiles(l_re, l_im, lane)
    p_re, p_im = l_re, l_im
    for _ in range(4):
        p_re, p_im = p_re * p_re - p_im * p_im, 2.0 * p_re * p_im
    lam_pows = []
    for _ in range(5):
        lam_pows.append(_lam_tiles(p_re, p_im, lane))
        p_re, p_im = p_re * p_re - p_im * p_im, 2.0 * p_re * p_im
    drow = jnp.concatenate([dsk[...].astype(F32).reshape(1, D), jnp.zeros((1, 64), F32)], axis=1)
    dcol[...] = jnp.broadcast_to(drow, (128, 512)).T

    pacer.finish()

    for cp in (xb_cp[3], xa_cp[0]):
        cp.start()
    bu_chunk(1, 28 + 48 + 12 + 56 + 64)
    w_cp.wait()
    xb_cp[2].wait()
    _run(chain(*[w_transpose(n) for n in range(10)], prep_xb(2),
               *[w_gather(0, c) for c in range(4)]), local_scan(0))
    pacer.finish()

    xa_cp[1].start()
    bu_chunk(2, 4 + 48 + 112 + 24 + 64)
    xa_cp[0].wait()
    xb_cp[3].wait()
    _run(chain(w_transpose(10), prep_xb(3), *[w_gather(p, c) for p in (1, 2) for c in range(4)],
               prep_xa([0])), local_scan(1))
    pacer.finish()

    for cp in wo_cp + c_cp:
        cp.start()
    xa_cp[1].wait()
    bu_chunk(3, 78 + 64)
    _run(prep_xa([1, 2, 3]), local_scan(2))
    pacer.finish()
    _run(local_scan(3))
    for cp in wo_cp:
        cp.wait()
    won[3, 0:D, :] = jnp.concatenate([woraw[:, 384:D], jnp.zeros((D, 64), BF16)], axis=1)

    row = lax.broadcasted_iota(jnp.int32, (JG, 128), 0)
    hu = h_s.bitcast(U32)

    def scan_chunk(g, c, prev):
        nparts = 2 if c < 3 else 1
        load = partial(load_bu, g, c)
        f = [fin[_ds(g * JG, JG), (2 * c + k) * 128:(2 * c + k + 1) * 128] for k in range(2)]
        s = tuple(pltpu.roll(jnp.where(row == JG - 1, p, x), 1, 0) for p, x in zip(prev, f))
        for m in range(5):
            sh = tuple(jnp.where(row >= 2 ** m, pltpu.roll(x, 2 ** m, 0), 0.0) for x in s)
            s = _step(lam_pows[m][c], sh, s)
        for rho in range(R // 2):
            e = _step(lam1[c], s, gate(*load(2 * rho)))
            s = _step(lam1[c], e, load(2 * rho + 1))
            for k in range(nparts):
                hu[(2 * c + k) * G + g, pl.ds(rho, JG, stride=R // 2), :] = _pack(e[k], s[k])
        return s

    def qkv_part(r, part):
        dst, i = ((q_s, r), (k_s, R + r), (v_s, R + r))[part]
        res = lax.dot_general(_bf16(wt[part * D // 2:(part + 1) * D // 2, :], D),
                              _bf16(xap[_ds(r * 64, 64), :], D), NT, preferred_element_type=F32)
        dst[i] = res
        return res

    def shift_kv(r):
        k_s[r] = pltpu.roll(k_s[R + r], 1, 1)
        v_s[r] = pltpu.roll(v_s[R + r], 1, 1)

    def prep_wo(c):
        wu = won.bitcast(U32)
        for dp in range(DH // 2):
            lo, hi = _unpack(wu[c, pl.ds(dp, H, stride=DH // 2), :])
            wop[dp * H:dp * H + H // 2, :] = lo
            wop[dp * H + H // 2:(dp + 1) * H, :] = hi
        wop[D // 2:256, :] = jnp.zeros((256 - D // 2, 128), U32)
        wot[_ds(c * 64, 64), :] = pltpu.bitcast(_bf16(wop[...]).T, U32)

    def phase2a(g, prev):
        last = []
        for i in range(2):
            r = 4 * g + 2 * i
            pacer.pace([partial(qkv_part, r, k) for k in (1, 2, 0)], 18)
            last.append(scan_chunk(g, 2 * i, prev[2 * i]))
            last.append(scan_chunk(g, 2 * i + 1, prev[2 * i + 1]))
            pacer.finish()
            shift_kv(r)
        prep_wo(g)
        return tuple(last)

    zero = jnp.zeros((JG, 128), F32)
    _loop(phase2a, ((zero, zero),) * 4)

    lane_h = lax.broadcasted_iota(jnp.int32, (H, 128), 1)
    scale = DH ** -0.5

    def attend(r, odd):
        acc = [None] * W
        for d in range(DH):
            rows = slice(d * H, (d + 1) * H)
            qd = gate(q_s[r, rows, :])
            for w in range(W):
                t = qd * k_s[R + r - 2 * w, rows, :]
                acc[w] = t if d == 0 else acc[w] + t
        lg = []
        for w in range(W):
            first = jnp.where(r < 2 * w, 1, 0)
            lg.append(jnp.where(lane_h < first, -1e9, acc[w] * scale))
        m = lg[0]
        for w in range(1, W):
            m = jnp.maximum(m, lg[w])
        e = [jnp.exp(x - m) for x in lg]
        tot = e[0]
        for w in range(1, W):
            tot = tot + e[w]
        inv = 1.0 / tot
        p = [x * inv for x in e]
        for d in range(DH):
            rows = slice(d * H, (d + 1) * H)
            o = gate(p[0] * v_s[R + r, rows, :])
            for w in range(1, W):
                o = o + p[w] * v_s[R + r - 2 * w, rows, :]
            if odd:
                ow[rows, :] = _pack(q_s[r - 1, rows, :], o)
            else:
                q_s[r, rows, :] = o

    def prep_c(r0):
        src, dst = _ds(r0, D // G, 16), _ds(r0 // 2, D // G // 2, 8)
        for c in range(4):
            sl = slice(c * 128, min(D, (c + 1) * 128))
            xr, xi = cre[src, sl].astype(F32), cim[src, sl].astype(F32)
            cr, ci = co_re[:, sl], co_im[:, sl]
            yr, yi = xr * cr - xi * ci, -(xr * ci + xi * cr)
            if c < 3:
                cst[dst, c * 256:c * 256 + 128] = _words(yr)
                cst[dst, c * 256 + 128:c * 256 + 256] = _words(yi)
            else:
                cst[dst, 768:896] = _words(jnp.concatenate([yr, yi], axis=1))

    for cp in c_cp:
        cp.wait()

    for r in range(0, R, 2):
        pacer.pace([partial(qkv_part, r + 1, k) for k in (1, 2)], 2 * DH + 1)
        attend(r, False)
        shift_kv(r + 1)
        if r % 4 == 2:
            prep_c(r // 4 * (D // G))

    def y_copy(i):
        rows = _ds(i * TP, TP)
        return copy(ob.at[rows, pl.ds(512, 384)], out_hbm.at[0, rows, pl.ds(512, 384)], sem_out.at[i])

    def a_copy(i):
        rows = _ds(i * TP, TP)
        return copy(ob.at[rows, pl.ds(0, 512)], out_hbm.at[0, rows, pl.ds(0, 512)], sem_out.at[NP + i])

    def y_piece(i):
        rows = _ds(i * TP, TP)
        sub = _ds((i % (TG // TP)) * TP, TP)
        hh = jnp.concatenate([h_s[k * G + i // (TG // TP), sub, :] for k in range(7)], axis=1)
        res = lax.dot_general(_bf16(cst[...]), hh, NT, preferred_element_type=F32)
        y = res + xbt[0:D, rows] * dcol[0:D, :]
        ylow[i] = y[0:64]
        for n in range(3):
            ob[rows, 512 + n * 128:640 + n * 128] = y[64 + n * 128:192 + n * 128].T
        y_copy(i).start()
        return res

    qkv_part(1, 0)
    for i in range(R // 2):
        nxt = [partial(qkv_part, 2 * i + 3, 0)] if i < R // 2 - 1 else []
        ys = [partial(y_piece, k) for k in range(NY * i // 8, NY * (i + 1) // 8)]
        pacer.pace(nxt + ys, 2 * DH + 4)
        attend(2 * i + 1, True)
        for c in range(4):
            o_s[c * NP:(c + 1) * NP, i * 8:(i + 1) * 8, :] = (
                ow[c * 128:(c + 1) * 128, :].T.reshape(NP, 8, 128))
        pacer.finish()

    def a_piece(i):
        rows = _ds(i * TP, TP)
        oo = jnp.concatenate([
            _bf16(jnp.concatenate(
                [o_s[c * NP + i, pl.ds(j, R // 2, stride=8), :]
                 for j in range(TP // R)], axis=0))
            for c in range(4)], axis=1)
        a = lax.dot_general(_bf16(wot[0:D // 2, :]), oo, NT, preferred_element_type=F32)
        for n in range(3):
            ob[rows, n * 128:(n + 1) * 128] = a[n * 128:(n + 1) * 128].T
        ob[rows, 384:512] = jnp.concatenate([a[384:D], ylow[i]], axis=0).T
        a_copy(i).start(priority=1)

    def phase4(g, carry):
        for k in range(4):
            if k == 3:
                y_piece(NY + g)
            a_piece(4 * g + k)
        return carry

    lax.fori_loop(0, 4, phase4, 0)
    for i in range(NP):
        y_copy(i).wait()
        a_copy(i).wait()


@jax.jit
def pallas_concat_heads__sliding_local_dilated__ssm_conv_s5__prompt_kernel(
    A_x, A_wqkv, A_wo, B_x, B_Lambda_re, B_Lambda_im, B_B_re, B_B_im, B_C_re, B_C_im,
    B_log_dt, B_Dskip,
):
    hbm = pl.BlockSpec(memory_space=pl.ANY)
    vm = pltpu.VMEM
    dma = pltpu.SemaphoreType.DMA
    scratch = [vm((D,), BF16)] * 4 + [
        vm((512, S), BF16), vm((512, S), BF16),
        vm((4 * S + 16, 128), BF16), vm((4 * S + 16, 128), BF16),
        vm((S // 2, 512), U32), vm((S // 2, 512), U32),
        vm((2 * D, D), BF16),
        vm((S, 2 * D), F32),
        vm((D, 3 * D), BF16),
        vm((4 * 1408, 128), BF16),
        vm((3 * D // 2, 512), U32),
        vm((R, D, 128), F32),
        vm((2 * R, D, 128), F32), vm((2 * R, D, 128), F32),
        vm((7 * G, TG + 16, 128), BF16),
        vm((4 * NP, TP // 2 + 8, 128), U32),
        vm((D, D), BF16), vm((D, D), BF16),
        vm((D // 2, 2 * D), U32),
        vm((D, D), BF16), vm((4, D + 32, 128), BF16),
        vm((256, 128), U32), vm((256, 512), U32),
        vm((512, 128), U32),
        vm((512, 128), F32),
        vm((NP, 64, 128), F32),
        vm((G * JG, 1024), F32),
        vm((S, 2 * D), F32),
        dma((G,)), dma((7,)), dma((7,)), dma((2 * NP,)),
    ]
    return pl.pallas_call(
        _kernel,
        out_shape=jax.ShapeDtypeStruct((1, S, 2 * D), F32),
        in_specs=[hbm] * 12,
        out_specs=hbm,
        scratch_shapes=scratch,
        compiler_params=pltpu.CompilerParams(
            vmem_limit_bytes=100 * 1024 * 1024,
            flags={"XLA_TPU_EVENLY_DISTRIBUTE_CRITICAL_NODES": True}),
    )(jnp.swapaxes(A_x, 1, 2), A_wqkv, A_wo, jnp.swapaxes(B_x, 1, 2), B_Lambda_re, B_Lambda_im,
      B_B_re, B_B_im, B_C_re, B_C_im, B_log_dt, B_Dskip)
```

```python
from functools import partial
from itertools import chain, islice

import jax
import jax.numpy as jnp
from jax import lax
import jax.experimental.pallas as pl
import jax.experimental.pallas.tpu as pltpu

S = 2048
D = 448
H = 16
DH = 28
W = 8
R = 16
G = 4
TG = S // G
JG = TG // R
TP = 128
NP = S // TP
NY = 12

F32 = jnp.float32
BF16 = jnp.bfloat16
U32 = jnp.uint32
NT = (((1,), (1,)), ((), ()))


def _unpack(w):
    lo = pltpu.bitcast(w.astype(jnp.uint16), U32)
    hi = pltpu.bitcast((w >> 16).astype(jnp.uint16), U32)
    return lo, hi


def _pack(even, odd):
    return pltpu.bitcast(pltpu.pack_elementwise([even, odd], packed_dtype=BF16), U32)


def _words(x):
    return pltpu.bitcast(x.astype(BF16), U32)


def _bf16(w, cols=None):
    x = pltpu.bitcast(w, BF16)
    return x if cols is None else x[:, :cols]


def _ds(start, size, align=None):
    return pl.ds(pl.multiple_of(start, align or size), size)


def _step(lam, h, b):
    lr, li = lam
    return (lr * h[0] - li * h[1] + b[0], lr * h[1] + li * h[0] + b[1])


def _lam_tiles(re, im, lane):
    out = [(re[:, c * 128:(c + 1) * 128], im[:, c * 128:(c + 1) * 128]) for c in range(3)]
    z = jnp.zeros((1, 64), F32)
    r3 = jnp.concatenate([re[:, 384:], z], axis=1)
    i3 = jnp.concatenate([im[:, 384:], z], axis=1)
    out.append((jnp.where(lane < 64, r3, pltpu.roll(r3, 64, 1)),
                jnp.where(lane < 64, i3, -pltpu.roll(i3, 64, 1))))
    return out


class _Pacer:
    def __init__(self):
        self.zero = lax.broadcasted_iota(U32, (8, 128), 1) >> 16

    def pace(self, matmuls, steps):
        self.queue = list(matmuls)
        self.per = -(-steps // len(matmuls))
        self.pos = 0

    def gate(self, *xs):
        i = self.pos % self.per
        if i == 0 and not self.queue:
            return xs if len(xs) > 1 else xs[0]
        if i == 0:
            self.res = self.queue.pop(0)()
        self.pos += 1
        k = (self.res.shape[0] // 8 * i) // self.per * 8
        tok = pltpu.bitcast(self.res[k:k + 8, 0:128], U32) & self.zero
        out = []
        for x in xs:
            u = pltpu.bitcast(x, U32)
            u = u | jnp.tile(tok, (u.shape[0] // 8, u.shape[1] // 128))
            out.append(pltpu.bitcast(u, x.dtype))
        return out if len(out) > 1 else out[0]

    def finish(self):
        while self.queue:
            self.queue.pop(0)()
        self.pos = 0


def _run(*tasks):
    for _ in chain(*tasks):
        pass


def _loop(body, init, unroll=2):
    def outer(t, carry):
        for u in range(unroll):
            carry = body(t * unroll + u, carry)
        return carry
    return lax.fori_loop(0, G // unroll, outer, init)


def _kernel(xa_hbm, wqkv_hbm, wo_hbm, xb_hbm, lre_hbm, lim_hbm, bre_hbm, bim_hbm,
            cre_hbm, cim_hbm, ldt_hbm, dsk_hbm, out_hbm,
            lre, lim, ldt, dsk, xat, xbt, xan, xbn, xap, xbp, bst, bu, wraw, wtn, wt,
            q_s, k_s, v_s, h_s, o_s, cre, cim, cst, woraw, won, wop, wot, ow, dcol, ylow, fin, ob,
            sem_xb, sem_b, sem_in, sem_out):
    copy = pltpu.make_async_copy
    xb_cp = [copy(xb_hbm.at[0, :, pl.ds(g * TG, TG)], xbt.at[pl.ds(0, D), pl.ds(g * TG, TG)],
                  sem_xb.at[g]) for g in range(G)]
    b_cp = []
    for c in range(3):
        b_cp.append([copy(bre_hbm.at[pl.ds(c * 128, 128)], bst.at[pl.ds(c * 256, 128)], sem_b.at[2 * c])])
        b_cp.append([copy(bim_hbm.at[pl.ds(c * 128, 128)], bst.at[pl.ds(c * 256 + 128, 128)],
                          sem_b.at[2 * c + 1])])
    b_cp.append([copy(bre_hbm.at[pl.ds(384, 64)], bst.at[pl.ds(768, 64)], sem_b.at[6]),
                 copy(bim_hbm.at[pl.ds(384, 64)], bst.at[pl.ds(832, 64)], sem_b.at[6])])
    p_cp = [copy(src, dst, sem_in.at[5]) for src, dst in
            ((lre_hbm, lre), (lim_hbm, lim), (ldt_hbm, ldt), (dsk_hbm, dsk))]
    w_cp = copy(wqkv_hbm, wraw, sem_in.at[0])
    xa_cp = [copy(xa_hbm.at[0, pl.ds(lo, n)], xat.at[pl.ds(lo, n)], sem_in.at[i])
             for lo, n, i in ((0, 128, 1), (128, D - 128, 6))]
    c_cp = [copy(cre_hbm, cre, sem_in.at[2]), copy(cim_hbm, cim, sem_in.at[3])]
    wo_cp = [copy(wo_hbm.at[:, pl.ds(c * 128, 128)], won.at[c, pl.ds(0, D)], sem_in.at[4]) for c in range(3)]
    wo_cp.append(copy(wo_hbm, woraw, sem_in.at[4]))

    for cp in [xb_cp[0]] + b_cp[6] + sum(b_cp[:6], []) + p_cp:
        cp.start()

    xat[D:512, :] = jnp.zeros((512 - D, S), BF16)
    xbt[D:512, :] = jnp.zeros((512 - D, S), BF16)
    ow[D:512, :] = jnp.zeros((512 - D, 128), U32)
    xan[4 * S:, :] = jnp.zeros((16, 128), BF16)
    xbn[4 * S:, :] = jnp.zeros((16, 128), BF16)
    won[:, D:, :] = jnp.zeros((4, 32, 128), BF16)
    o_s[:, TP // 2:, :] = jnp.zeros((4 * NP, 8, 128), U32)
    pacer = _Pacer()
    gate = pacer.gate

    def transpose_x(xt_ref, xn_ref, c, g):
        for t in range(g * TG, (g + 1) * TG, 128):
            xn_ref[pl.ds(c * S + t, 128), :] = gate(xt_ref[c * 128:(c + 1) * 128, t:t + 128]).T
            yield

    def gather_x(xn_ref, xp_ref, c, row0, rhos, nj, g8=gate):
        xu = xn_ref.bitcast(U32)
        for rho in rhos:
            lo, hi = _unpack(g8(xu[pl.ds(c * (S // 2) + row0 + rho, nj, stride=R // 2), :]))
            dst = row0 + rho * nj
            xp_ref[dst:dst + nj // 2, c * 128:(c + 1) * 128] = lo
            xp_ref[dst + nj // 2:dst + nj, c * 128:(c + 1) * 128] = hi
            yield

    def w_transpose(n):
        cols = min(128, 3 * D - n * 128)
        for c in range(4):
            rows = min(128, D - c * 128)
            v = wraw[c * 128:c * 128 + rows, n * 128:n * 128 + cols]
            if rows < 128:
                v = jnp.concatenate([v, jnp.zeros((128 - rows, cols), BF16)], axis=0)
            if cols < 128:
                v = jnp.concatenate([v, jnp.zeros((128, 128 - cols), BF16)], axis=1)
            wtn[pl.ds(c * 1408 + n * 128, 128), :] = gate(v).T
            yield

    def w_gather(part, c):
        wu = wtn.bitcast(U32)
        for dp in range(DH // 2):
            lo, hi = _unpack(gate(wu[pl.ds(c * 704 + part * (D // 2) + dp, H, stride=DH // 2), :]))
            base = part * (D // 2) + dp * H
            wt[base:base + H // 2, c * 128:(c + 1) * 128] = lo
            wt[base + H // 2:base + H, c * 128:(c + 1) * 128] = hi
            yield

    def bu_piece(g, n):
        res = lax.dot_general(_bf16(xbp[g * TG // 2:(g + 1) * TG // 2, :], D),
                              bst[n * 128:(n + 1) * 128, :], NT, preferred_element_type=F32)
        bu[g * TG:(g + 1) * TG, n * 128:(n + 1) * 128] = res
        return res

    def prep_xb(g):
        for c in range(4):
            yield from transpose_x(xbt, xbn, c, g)
            yield from gather_x(xbn, xbp, c, g * (TG // 2), range(R // 2), JG)

    def prep_xa(cs):
        for c in cs:
            for g in range(G):
                yield from transpose_x(xat, xan, c, g)
            yield from gather_x(xan, xap, c, 0, range(R // 2), 128)

    xb_cp[0].wait()
    for cp in [xb_cp[1], w_cp, xb_cp[2]]:
        cp.start()
    for c in range(4):
        xbn[pl.ds(c * S, TG), :] = xbt[c * 128:(c + 1) * 128, 0:TG].T
        _run(gather_x(xbn, xbp, c, 0, range(R // 2), JG, lambda v: v))

    def load_bu(g, c, r):
        v = [bu[_ds(g * TG + r * JG, JG), c * 256 + k * 128:c * 256 + (k + 1) * 128]
             for k in range(2 if c < 3 else 1)]
        return v if c < 3 else (v[0], pltpu.roll(v[0], 64, 1))

    def local_scan(g, cs=range(4)):
        for c in cs:
            f = gate(*load_bu(g, c, 0))
            for r in range(1, R):
                f = _step(lam1[c], f, gate(*load_bu(g, c, r)))
                yield
            for k in range(2):
                fin[g * JG:(g + 1) * JG, (2 * c + k) * 128:(2 * c + k + 1) * 128] = f[k]

    def bu_chunk(g, steps):
        pacer.pace([partial(bu_piece, g, n) for n in (6, 0, 1, 2, 3, 4, 5)], steps)

    for cp in b_cp[6] + b_cp[0]:
        cp.wait()
    bu_chunk(0, 70)
    for _ in range(20):
        gate(pacer.zero)
    for cp in sum(b_cp[1:6], []):
        cp.wait()
    xb_cp[1].wait()
    steps = prep_xb(1)
    _run(islice(steps, 30))
    for cp in p_cp:
        cp.wait()
    lane = lax.broadcasted_iota(jnp.int32, (1, 128), 1)
    a_re = lre[...].astype(F32).reshape(1, D)
    a_im = lim[...].astype(F32).reshape(1, D)
    dt = jnp.exp(ldt[...].astype(F32).reshape(1, D)).astype(BF16).astype(F32)
    mag = jnp.exp(dt * a_re)
    l_re = mag * jnp.cos(dt * a_im)
    l_im = mag * jnp.sin(dt * a_im)
    big = jnp.maximum(jnp.abs(a_re), jnp.abs(a_im))
    u_re, u_im = a_re / big, a_im / big
    den = (u_re * u_re + u_im * u_im) * big
    n_re = l_re - 1.0
    co_re = 2.0 * (n_re * u_re + l_im * u_im) / den
    co_im = 2.0 * (l_im * u_re - n_re * u_im) / den
    lam1 = _lam_tiles(l_re, l_im, lane)
    p_re, p_im = l_re, l_im
    for _ in range(4):
        p_re, p_im = p_re * p_re - p_im * p_im, 2.0 * p_re * p_im
    lam_pows = []
    for _ in range(5):
        lam_pows.append(_lam_tiles(p_re, p_im, lane))
        p_re, p_im = p_re * p_re - p_im * p_im, 2.0 * p_re * p_im
    drow = jnp.concatenate([dsk[...].astype(F32).reshape(1, D), jnp.zeros((1, 64), F32)], axis=1)
    dcol[...] = jnp.broadcast_to(drow, (128, 512)).T
    for v in (p_re, co_re, co_im):
        pacer.zero &= pltpu.bitcast(jnp.broadcast_to(v[:, 0:128], (8, 128)), U32)
    _run(steps)

    pacer.finish()

    for cp in (xb_cp[3], xa_cp[0]):
        cp.start()
    bu_chunk(1, 28 + 48 + 12 + 56 + 64)
    w_cp.wait()
    xb_cp[2].wait()
    _run(chain(*[w_transpose(n) for n in range(10)], prep_xb(2),
               *[w_gather(0, c) for c in range(4)]), local_scan(0))
    pacer.finish()

    xa_cp[1].start()
    bu_chunk(2, 4 + 48 + 112 + 24 + 64)
    xa_cp[0].wait()
    xb_cp[3].wait()
    _run(chain(w_transpose(10), prep_xb(3), *[w_gather(p, c) for p in (1, 2) for c in range(4)],
               prep_xa([0])), local_scan(1))
    pacer.finish()

    for cp in wo_cp + c_cp:
        cp.start()
    xa_cp[1].wait()
    bu_chunk(3, 184)
    _run(local_scan(2), local_scan(3, [3]), prep_xa([1]), local_scan(3, [0]), prep_xa([2]),
         local_scan(3, [1]), prep_xa([3]))
    pacer.finish()
    _run(local_scan(3, [2]))
    for cp in wo_cp:
        cp.wait()
    won[3, 0:D, :] = jnp.concatenate([woraw[:, 384:D], jnp.zeros((D, 64), BF16)], axis=1)

    row = lax.broadcasted_iota(jnp.int32, (JG, 128), 0)
    hu = h_s.bitcast(U32)

    def scan_chunk(g, c, prev):
        nparts = 2 if c < 3 else 1
        load = partial(load_bu, g, c)
        f = [fin[_ds(g * JG, JG), (2 * c + k) * 128:(2 * c + k + 1) * 128] for k in range(2)]
        s = tuple(pltpu.roll(jnp.where(row == JG - 1, p, x), 1, 0) for p, x in zip(prev, f))
        for m in range(5):
            sh = tuple(jnp.where(row >= 2 ** m, pltpu.roll(x, 2 ** m, 0), 0.0) for x in s)
            s = _step(lam_pows[m][c], sh, s)
        for rho in range(R // 2):
            e = _step(lam1[c], s, gate(*load(2 * rho)))
            s = _step(lam1[c], e, load(2 * rho + 1))
            for k in range(nparts):
                hu[(2 * c + k) * G + g, pl.ds(rho, JG, stride=R // 2), :] = _pack(e[k], s[k])
        return s

    def qkv_part(r, part):
        dst, i = ((q_s, r), (k_s, R + r), (v_s, R + r))[part]
        res = lax.dot_general(_bf16(wt[part * D // 2:(part + 1) * D // 2, :], D),
                              _bf16(xap[_ds(r * 64, 64), :], D), NT, preferred_element_type=F32)
        dst[i] = res
        return res

    def shift_kv(r):
        k_s[r] = pltpu.roll(k_s[R + r], 1, 1)
        v_s[r] = pltpu.roll(v_s[R + r], 1, 1)

    def prep_wo(c):
        wu = won.bitcast(U32)
        for dp in range(DH // 2):
            lo, hi = _unpack(wu[c, pl.ds(dp, H, stride=DH // 2), :])
            wop[dp * H:dp * H + H // 2, :] = lo
            wop[dp * H + H // 2:(dp + 1) * H, :] = hi
        wop[D // 2:256, :] = jnp.zeros((256 - D // 2, 128), U32)
        wot[_ds(c * 64, 64), :] = pltpu.bitcast(_bf16(wop[...]).T, U32)

    def phase2a(g, prev):
        last = []
        for i in range(2):
            r = 4 * g + 2 * i
            pacer.pace([partial(qkv_part, r, k) for k in (1, 2, 0)], 18)
            last.append(scan_chunk(g, 2 * i, prev[2 * i]))
            last.append(scan_chunk(g, 2 * i + 1, prev[2 * i + 1]))
            pacer.finish()
            shift_kv(r)
        prep_wo(g)
        return tuple(last)

    zero = jnp.zeros((JG, 128), F32)
    _loop(phase2a, ((zero, zero),) * 4)

    lane_h = lax.broadcasted_iota(jnp.int32, (H, 128), 1)
    scale = DH ** -0.5

    def attend(r, odd):
        acc = [None] * W
        for d in range(DH):
            rows = slice(d * H, (d + 1) * H)
            qd = gate(q_s[r, rows, :])
            for w in range(W):
                t = qd * k_s[R + r - 2 * w, rows, :]
                acc[w] = t if d == 0 else acc[w] + t
        lg = []
        for w in range(W):
            first = jnp.where(r < 2 * w, 1, 0)
            lg.append(jnp.where(lane_h < first, -1e9, acc[w] * scale))
        m = lg[0]
        for w in range(1, W):
            m = jnp.maximum(m, lg[w])
        e = [jnp.exp(x - m) for x in lg]
        tot = e[0]
        for w in range(1, W):
            tot = tot + e[w]
        inv = 1.0 / tot
        p = [x * inv for x in e]
        for d in range(DH):
            rows = slice(d * H, (d + 1) * H)
            o = gate(p[0] * v_s[R + r, rows, :])
            for w in range(1, W):
                o = o + p[w] * v_s[R + r - 2 * w, rows, :]
            if odd:
                ow[rows, :] = _pack(q_s[r - 1, rows, :], o)
            else:
                q_s[r, rows, :] = o

    def prep_c(r0):
        src, dst = _ds(r0, D // G, 16), _ds(r0 // 2, D // G // 2, 8)
        for c in range(4):
            sl = slice(c * 128, min(D, (c + 1) * 128))
            xr, xi = cre[src, sl].astype(F32), cim[src, sl].astype(F32)
            cr, ci = co_re[:, sl], co_im[:, sl]
            yr, yi = xr * cr - xi * ci, -(xr * ci + xi * cr)
            if c < 3:
                cst[dst, c * 256:c * 256 + 128] = _words(yr)
                cst[dst, c * 256 + 128:c * 256 + 256] = _words(yi)
            else:
                cst[dst, 768:896] = _words(jnp.concatenate([yr, yi], axis=1))

    for cp in c_cp:
        cp.wait()

    for r in range(0, R, 2):
        pacer.pace([partial(qkv_part, r + 1, k) for k in (1, 2)], 2 * DH + 1)
        attend(r, False)
        shift_kv(r + 1)
        if r % 4 == 2:
            prep_c(r // 4 * (D // G))

    def y_copy(i):
        rows = _ds(i * TP, TP)
        return copy(ob.at[rows, pl.ds(512, 384)], out_hbm.at[0, rows, pl.ds(512, 384)], sem_out.at[i])

    def a_copy(i):
        rows = _ds(i * TP, TP)
        return copy(ob.at[rows, pl.ds(0, 512)], out_hbm.at[0, rows, pl.ds(0, 512)], sem_out.at[NP + i])

    def y_piece(i):
        rows = _ds(i * TP, TP)
        sub = _ds((i % (TG // TP)) * TP, TP)
        hh = jnp.concatenate([h_s[k * G + i // (TG // TP), sub, :] for k in range(7)], axis=1)
        res = lax.dot_general(_bf16(cst[...]), hh, NT, preferred_element_type=F32)
        y = res + xbt[0:D, rows] * dcol[0:D, :]
        ylow[i] = y[0:64]
        for n in range(3):
            ob[rows, 512 + n * 128:640 + n * 128] = y[64 + n * 128:192 + n * 128].T
        y_copy(i).start()
        return res

    qkv_part(1, 0)
    for i in range(R // 2):
        nxt = [partial(qkv_part, 2 * i + 3, 0)] if i < R // 2 - 1 else []
        ys = [partial(y_piece, k) for k in range(NY * i // 8, NY * (i + 1) // 8)]
        pacer.pace(nxt + ys, 2 * DH + 4)
        attend(2 * i + 1, True)
        for c in range(4):
            o_s[c * NP:(c + 1) * NP, i * 8:(i + 1) * 8, :] = (
                ow[c * 128:(c + 1) * 128, :].T.reshape(NP, 8, 128))
        pacer.finish()

    def a_piece(i):
        rows = _ds(i * TP, TP)
        oo = jnp.concatenate([
            _bf16(jnp.concatenate(
                [o_s[c * NP + i, pl.ds(j, R // 2, stride=8), :]
                 for j in range(TP // R)], axis=0))
            for c in range(4)], axis=1)
        a = lax.dot_general(_bf16(wot[0:D // 2, :]), oo, NT, preferred_element_type=F32)
        for n in range(3):
            ob[rows, n * 128:(n + 1) * 128] = a[n * 128:(n + 1) * 128].T
        ob[rows, 384:512] = jnp.concatenate([a[384:D], ylow[i]], axis=0).T
        a_copy(i).start(priority=1)

    def phase4(g, carry):
        for k in range(4):
            if k == 3:
                y_piece(NY + g)
            a_piece(4 * g + k)
        return carry

    lax.fori_loop(0, 4, phase4, 0)
    for i in range(NP):
        y_copy(i).wait()
        a_copy(i).wait()


@jax.jit
def pallas_concat_heads__sliding_local_dilated__ssm_conv_s5__prompt_kernel(
    A_x, A_wqkv, A_wo, B_x, B_Lambda_re, B_Lambda_im, B_B_re, B_B_im, B_C_re, B_C_im,
    B_log_dt, B_Dskip,
):
    hbm = pl.BlockSpec(memory_space=pl.ANY)
    vm = pltpu.VMEM
    dma = pltpu.SemaphoreType.DMA
    scratch = [vm((D,), BF16)] * 4 + [
        vm((512, S), BF16), vm((512, S), BF16),
        vm((4 * S + 16, 128), BF16), vm((4 * S + 16, 128), BF16),
        vm((S // 2, 512), U32), vm((S // 2, 512), U32),
        vm((2 * D, D), BF16),
        vm((S, 2 * D), F32),
        vm((D, 3 * D), BF16),
        vm((4 * 1408, 128), BF16),
        vm((3 * D // 2, 512), U32),
        vm((R, D, 128), F32),
        vm((2 * R, D, 128), F32), vm((2 * R, D, 128), F32),
        vm((7 * G, TG + 16, 128), BF16),
        vm((4 * NP, TP // 2 + 8, 128), U32),
        vm((D, D), BF16), vm((D, D), BF16),
        vm((D // 2, 2 * D), U32),
        vm((D, D), BF16), vm((4, D + 32, 128), BF16),
        vm((256, 128), U32), vm((256, 512), U32),
        vm((512, 128), U32),
        vm((512, 128), F32),
        vm((NP, 64, 128), F32),
        vm((G * JG, 1024), F32),
        vm((S, 2 * D), F32),
        dma((G,)), dma((7,)), dma((7,)), dma((2 * NP,)),
    ]
    return pl.pallas_call(
        _kernel,
        out_shape=jax.ShapeDtypeStruct((1, S, 2 * D), F32),
        in_specs=[hbm] * 12,
        out_specs=hbm,
        scratch_shapes=scratch,
        compiler_params=pltpu.CompilerParams(
            vmem_limit_bytes=100 * 1024 * 1024,
            flags={"XLA_TPU_EVENLY_DISTRIBUTE_CRITICAL_NODES": True}),
    )(jnp.swapaxes(A_x, 1, 2), A_wqkv, A_wo, jnp.swapaxes(B_x, 1, 2), B_Lambda_re, B_Lambda_im,
      B_B_re, B_B_im, B_C_re, B_C_im, B_log_dt, B_Dskip)
```

```python
from functools import partial
from itertools import chain, islice

import jax
import jax.numpy as jnp
from jax import lax
import jax.experimental.pallas as pl
import jax.experimental.pallas.tpu as pltpu

S = 2048
D = 448
H = 16
DH = 28
W = 8
R = 16
G = 4
TG = S // G
JG = TG // R
TP = 128
NP = S // TP
NY = 12

F32 = jnp.float32
BF16 = jnp.bfloat16
U32 = jnp.uint32
NT = (((1,), (1,)), ((), ()))


def _unpack(w):
    lo = pltpu.bitcast(w.astype(jnp.uint16), U32)
    hi = pltpu.bitcast((w >> 16).astype(jnp.uint16), U32)
    return lo, hi


def _pack(even, odd):
    return pltpu.bitcast(pltpu.pack_elementwise([even, odd], packed_dtype=BF16), U32)


def _words(x):
    return pltpu.bitcast(x.astype(BF16), U32)


def _bf16(w, cols=None):
    x = pltpu.bitcast(w, BF16)
    return x if cols is None else x[:, :cols]


def _ds(start, size, align=None):
    return pl.ds(pl.multiple_of(start, align or size), size)


def _step(lam, h, b):
    lr, li = lam
    return (lr * h[0] - li * h[1] + b[0], lr * h[1] + li * h[0] + b[1])


def _lam_tiles(re, im, lane):
    out = [(re[:, c * 128:(c + 1) * 128], im[:, c * 128:(c + 1) * 128]) for c in range(3)]
    z = jnp.zeros((1, 64), F32)
    r3 = jnp.concatenate([re[:, 384:], z], axis=1)
    i3 = jnp.concatenate([im[:, 384:], z], axis=1)
    out.append((jnp.where(lane < 64, r3, pltpu.roll(r3, 64, 1)),
                jnp.where(lane < 64, i3, -pltpu.roll(i3, 64, 1))))
    return out


class _Pacer:
    def __init__(self):
        self.zero = lax.broadcasted_iota(U32, (8, 128), 1) >> 16

    def pace(self, matmuls, steps):
        self.queue = list(matmuls)
        self.per = -(-steps // len(matmuls))
        self.pos = 0

    def gate(self, *xs):
        i = self.pos % self.per
        if i == 0 and not self.queue:
            return xs if len(xs) > 1 else xs[0]
        if i == 0:
            self.res = self.queue.pop(0)()
        self.pos += 1
        k = (self.res.shape[0] // 8 * i) // self.per * 8
        tok = pltpu.bitcast(self.res[k:k + 8, 0:128], U32) & self.zero
        out = []
        for x in xs:
            u = pltpu.bitcast(x, U32)
            u = u | jnp.tile(tok, (u.shape[0] // 8, u.shape[1] // 128))
            out.append(pltpu.bitcast(u, x.dtype))
        return out if len(out) > 1 else out[0]

    def finish(self):
        while self.queue:
            self.queue.pop(0)()
        self.pos = 0


def _run(*tasks):
    for _ in chain(*tasks):
        pass


def _loop(body, init, unroll=2):
    def outer(t, carry):
        for u in range(unroll):
            carry = body(t * unroll + u, carry)
        return carry
    return lax.fori_loop(0, G // unroll, outer, init)


def _kernel(xa_hbm, wqkv_hbm, wo_hbm, xb_hbm, lre_hbm, lim_hbm, bre_hbm, bim_hbm,
            cre_hbm, cim_hbm, ldt_hbm, dsk_hbm, out_hbm,
            lre, lim, ldt, dsk, xat, xbt, xan, xbn, xap, xbp, bst, bu, wraw, wtn, wt,
            q_s, k_s, v_s, h_s, o_s, cre, cim, cst, woraw, won, wop, wot, ow, dcol, ylow, fin, ob,
            sem_x0, sem_xb, sem_b, sem_in, sem_out):
    copy = pltpu.make_async_copy
    xb_cp = [copy(xb_hbm.at[0, :, pl.ds(g * TG, TG)], xbt.at[pl.ds(0, D), pl.ds(g * TG, TG)],
                  sem_xb.at[g]) if g else None for g in range(G)]
    x0_cp = [copy(xb_hbm.at[0, pl.ds(c * 128, min(128, D - c * 128)), pl.ds(0, TG)],
                  xbt.at[pl.ds(c * 128, min(128, D - c * 128)), pl.ds(0, TG)], sem_x0.at[c])
             for c in range(4)]
    b_cp = []
    for c in range(3):
        b_cp.append([copy(bre_hbm.at[pl.ds(c * 128, 128)], bst.at[pl.ds(c * 256, 128)], sem_b.at[2 * c])])
        b_cp.append([copy(bim_hbm.at[pl.ds(c * 128, 128)], bst.at[pl.ds(c * 256 + 128, 128)],
                          sem_b.at[2 * c + 1])])
    b_cp.append([copy(bre_hbm.at[pl.ds(384, 64)], bst.at[pl.ds(768, 64)], sem_b.at[6]),
                 copy(bim_hbm.at[pl.ds(384, 64)], bst.at[pl.ds(832, 64)], sem_b.at[6])])
    p_cp = [copy(src, dst, sem_in.at[5]) for src, dst in
            ((lre_hbm, lre), (lim_hbm, lim), (ldt_hbm, ldt), (dsk_hbm, dsk))]
    w_cp = copy(wqkv_hbm, wraw, sem_in.at[0])
    xa_cp = copy(xa_hbm.at[0], xat.at[pl.ds(0, D)], sem_in.at[1])
    c_cp = [copy(cre_hbm, cre, sem_in.at[2]), copy(cim_hbm, cim, sem_in.at[3])]
    wo_cp = [copy(wo_hbm.at[:, pl.ds(c * 128, 128)], won.at[c, pl.ds(0, D)], sem_in.at[4]) for c in range(3)]
    wo_cp.append(copy(wo_hbm, woraw, sem_in.at[4]))

    for cp in x0_cp + b_cp[6] + sum(b_cp[:6], []) + p_cp:
        cp.start()

    xat[D:512, :] = jnp.zeros((512 - D, S), BF16)
    xbt[D:512, :] = jnp.zeros((512 - D, S), BF16)
    ow[D:512, :] = jnp.zeros((512 - D, 128), U32)
    xan[4 * S:, :] = jnp.zeros((16, 128), BF16)
    xbn[4 * S:, :] = jnp.zeros((16, 128), BF16)
    won[:, D:, :] = jnp.zeros((4, 32, 128), BF16)
    o_s[:, TP // 2:, :] = jnp.zeros((4 * NP, 8, 128), U32)
    pacer = _Pacer()
    gate = pacer.gate

    def transpose_x(xt_ref, xn_ref, c, g):
        for t in range(g * TG, (g + 1) * TG, 128):
            xn_ref[pl.ds(c * S + t, 128), :] = gate(xt_ref[c * 128:(c + 1) * 128, t:t + 128]).T
            yield

    def gather_x(xn_ref, xp_ref, c, row0, rhos, nj, g8=gate):
        xu = xn_ref.bitcast(U32)
        for rho in rhos:
            lo, hi = _unpack(g8(xu[pl.ds(c * (S // 2) + row0 + rho, nj, stride=R // 2), :]))
            dst = row0 + rho * nj
            xp_ref[dst:dst + nj // 2, c * 128:(c + 1) * 128] = lo
            xp_ref[dst + nj // 2:dst + nj, c * 128:(c + 1) * 128] = hi
            yield

    def w_transpose(n):
        cols = min(128, 3 * D - n * 128)
        for c in range(4):
            rows = min(128, D - c * 128)
            v = wraw[c * 128:c * 128 + rows, n * 128:n * 128 + cols]
            if rows < 128:
                v = jnp.concatenate([v, jnp.zeros((128 - rows, cols), BF16)], axis=0)
            if cols < 128:
                v = jnp.concatenate([v, jnp.zeros((128, 128 - cols), BF16)], axis=1)
            wtn[pl.ds(c * 1408 + n * 128, 128), :] = gate(v).T
            yield

    def w_gather(part, c):
        wu = wtn.bitcast(U32)
        for dp in range(DH // 2):
            lo, hi = _unpack(gate(wu[pl.ds(c * 704 + part * (D // 2) + dp, H, stride=DH // 2), :]))
            base = part * (D // 2) + dp * H
            wt[base:base + H // 2, c * 128:(c + 1) * 128] = lo
            wt[base + H // 2:base + H, c * 128:(c + 1) * 128] = hi
            yield

    def bu_piece(g, n):
        res = lax.dot_general(_bf16(xbp[g * TG // 2:(g + 1) * TG // 2, :], D),
                              bst[n * 128:(n + 1) * 128, :], NT, preferred_element_type=F32)
        bu[g * TG:(g + 1) * TG, n * 128:(n + 1) * 128] = res
        return res

    def prep_xb(g):
        for c in range(4):
            yield from transpose_x(xbt, xbn, c, g)
            yield from gather_x(xbn, xbp, c, g * (TG // 2), range(R // 2), JG)

    def prep_xa(cs):
        for c in cs:
            for g in range(G):
                yield from transpose_x(xat, xan, c, g)
            yield from gather_x(xan, xap, c, 0, range(R // 2), 128)

    for c in range(4):
        x0_cp[c].wait()
        if c == 3:
            for cp in [xb_cp[1], w_cp, xb_cp[2]]:
                cp.start()
        xbn[pl.ds(c * S, TG), :] = xbt[c * 128:(c + 1) * 128, 0:TG].T
        _run(gather_x(xbn, xbp, c, 0, range(R // 2), JG, lambda v: v))

    def load_bu(g, c, r):
        v = [bu[_ds(g * TG + r * JG, JG), c * 256 + k * 128:c * 256 + (k + 1) * 128]
             for k in range(2 if c < 3 else 1)]
        return v if c < 3 else (v[0], pltpu.roll(v[0], 64, 1))

    def local_scan(g, cs=range(4)):
        for c in cs:
            f = gate(*load_bu(g, c, 0))
            for r in range(1, R):
                f = _step(lam1[c], f, gate(*load_bu(g, c, r)))
                yield
            for k in range(2):
                fin[g * JG:(g + 1) * JG, (2 * c + k) * 128:(2 * c + k + 1) * 128] = f[k]

    def bu_chunk(g, steps):
        pacer.pace([partial(bu_piece, g, n) for n in (6, 0, 1, 2, 3, 4, 5)], steps)

    for cp in b_cp[6] + b_cp[0]:
        cp.wait()
    bu_chunk(0, 70)
    for _ in range(20):
        gate(pacer.zero)
    for cp in sum(b_cp[1:6], []):
        cp.wait()
    xb_cp[1].wait()
    steps = prep_xb(1)
    _run(islice(steps, 30))
    for cp in p_cp:
        cp.wait()
    lane = lax.broadcasted_iota(jnp.int32, (1, 128), 1)
    a_re = lre[...].astype(F32).reshape(1, D)
    a_im = lim[...].astype(F32).reshape(1, D)
    dt = jnp.exp(ldt[...].astype(F32).reshape(1, D)).astype(BF16).astype(F32)
    mag = jnp.exp(dt * a_re)
    l_re = mag * jnp.cos(dt * a_im)
    l_im = mag * jnp.sin(dt * a_im)
    big = jnp.maximum(jnp.abs(a_re), jnp.abs(a_im))
    u_re, u_im = a_re / big, a_im / big
    den = (u_re * u_re + u_im * u_im) * big
    n_re = l_re - 1.0
    co_re = 2.0 * (n_re * u_re + l_im * u_im) / den
    co_im = 2.0 * (l_im * u_re - n_re * u_im) / den
    lam1 = _lam_tiles(l_re, l_im, lane)
    p_re, p_im = l_re, l_im
    for _ in range(4):
        p_re, p_im = p_re * p_re - p_im * p_im, 2.0 * p_re * p_im
    lam_pows = []
    for _ in range(5):
        lam_pows.append(_lam_tiles(p_re, p_im, lane))
        p_re, p_im = p_re * p_re - p_im * p_im, 2.0 * p_re * p_im
    drow = jnp.concatenate([dsk[...].astype(F32).reshape(1, D), jnp.zeros((1, 64), F32)], axis=1)
    dcol[...] = jnp.broadcast_to(drow, (128, 512)).T
    for v in (p_re, co_re, co_im):
        pacer.zero &= pltpu.bitcast(jnp.broadcast_to(v[:, 0:128], (8, 128)), U32)
    _run(steps)
    pacer.finish()

    for cp in (xb_cp[3], xa_cp):
        cp.start()
    bu_chunk(1, 28 + 48 + 12 + 56 + 64)
    w_cp.wait()
    xb_cp[2].wait()
    _run(*[w_transpose(n) for n in range(10)], prep_xb(2),
         *[w_gather(0, c) for c in range(4)], local_scan(0))
    pacer.finish()

    bu_chunk(2, 4 + 48 + 112 + 24 + 64)
    _run(w_transpose(10), *[w_gather(p, c) for p in (1, 2) for c in range(4)], local_scan(1, [0]))
    xa_cp.wait()
    xb_cp[3].wait()
    _run(prep_xb(3), local_scan(1, [1, 2, 3]), prep_xa([0]))
    pacer.finish()

    for cp in wo_cp + c_cp:
        cp.start()
    bu_chunk(3, 184)
    _run(local_scan(2), local_scan(3, [3]), prep_xa([1]), local_scan(3, [0]), prep_xa([2]),
         local_scan(3, [1]), prep_xa([3]))
    pacer.finish()
    _run(local_scan(3, [2]))
    for cp in wo_cp:
        cp.wait()
    won[3, 0:D, :] = jnp.concatenate([woraw[:, 384:D], jnp.zeros((D, 64), BF16)], axis=1)

    row = lax.broadcasted_iota(jnp.int32, (JG, 128), 0)
    hu = h_s.bitcast(U32)

    def scan_chunk(g, c, prev):
        nparts = 2 if c < 3 else 1
        load = partial(load_bu, g, c)
        f = [fin[_ds(g * JG, JG), (2 * c + k) * 128:(2 * c + k + 1) * 128] for k in range(2)]
        s = tuple(pltpu.roll(jnp.where(row == JG - 1, p, x), 1, 0) for p, x in zip(prev, f))
        for m in range(5):
            sh = tuple(jnp.where(row >= 2 ** m, pltpu.roll(x, 2 ** m, 0), 0.0) for x in s)
            s = _step(lam_pows[m][c], sh, s)
        for rho in range(R // 2):
            e = _step(lam1[c], s, gate(*load(2 * rho)))
            s = _step(lam1[c], e, load(2 * rho + 1))
            for k in range(nparts):
                hu[(2 * c + k) * G + g, pl.ds(rho, JG, stride=R // 2), :] = _pack(e[k], s[k])
        return s

    def qkv_part(r, part):
        dst, i = ((q_s, r), (k_s, R + r), (v_s, R + r))[part]
        res = lax.dot_general(_bf16(wt[part * D // 2:(part + 1) * D // 2, :], D),
                              _bf16(xap[_ds(r * 64, 64), :], D), NT, preferred_element_type=F32)
        dst[i] = res
        return res

    def shift_kv(r):
        k_s[r] = pltpu.roll(k_s[R + r], 1, 1)
        v_s[r] = jnp.where(lane == 0, v_s[R], pltpu.roll(v_s[R + r], 1, 1))

    def prep_wo(c):
        wu = won.bitcast(U32)
        for dp in range(DH // 2):
            lo, hi = _unpack(wu[c, pl.ds(dp, H, stride=DH // 2), :])
            wop[dp * H:dp * H + H // 2, :] = lo
            wop[dp * H + H // 2:(dp + 1) * H, :] = hi
        wop[D // 2:256, :] = jnp.zeros((256 - D // 2, 128), U32)
        wot[_ds(c * 64, 64), :] = pltpu.bitcast(_bf16(wop[...]).T, U32)

    def phase2a(g, prev):
        last = []
        for i in range(2):
            r = 4 * g + 2 * i
            pacer.pace([partial(qkv_part, r, k) for k in (1, 2, 0)], 18)
            last.append(scan_chunk(g, 2 * i, prev[2 * i]))
            last.append(scan_chunk(g, 2 * i + 1, prev[2 * i + 1]))
            pacer.finish()
            shift_kv(r)
        prep_wo(g)
        return tuple(last)

    zero = jnp.zeros((JG, 128), F32)
    _loop(phase2a, ((zero, zero),) * 4)

    lane_h = lax.broadcasted_iota(jnp.int32, (H, 128), 1)
    scale = DH ** -0.5

    def attend(r, odd):
        acc = [None] * W
        for d in range(DH):
            rows = slice(d * H, (d + 1) * H)
            qd = gate(q_s[r, rows, :])
            for w in range(W):
                t = qd * k_s[R + r - 2 * w, rows, :]
                acc[w] = t if d == 0 else acc[w] + t
        lg = []
        for w in range(W):
            first = jnp.where(r < 2 * w, 1, 0)
            lg.append(jnp.where(lane_h < first, -1e9, acc[w] * scale))
        m = lg[0]
        for w in range(1, W):
            m = jnp.maximum(m, lg[w])
        e = [jnp.exp(x - m) for x in lg]
        tot = e[0]
        for w in range(1, W):
            tot = tot + e[w]
        inv = 1.0 / tot
        p = [x * inv for x in e]
        for d in range(DH):
            rows = slice(d * H, (d + 1) * H)
            o = gate(p[0] * v_s[R + r, rows, :])
            for w in range(1, W):
                o = o + p[w] * v_s[R + r - 2 * w, rows, :]
            if odd:
                ow[rows, :] = _pack(q_s[r - 1, rows, :], o)
            else:
                q_s[r, rows, :] = o

    def prep_c(r0):
        src, dst = _ds(r0, D // G, 16), _ds(r0 // 2, D // G // 2, 8)
        for c in range(4):
            sl = slice(c * 128, min(D, (c + 1) * 128))
            xr, xi = cre[src, sl].astype(F32), cim[src, sl].astype(F32)
            cr, ci = co_re[:, sl], co_im[:, sl]
            yr, yi = xr * cr - xi * ci, -(xr * ci + xi * cr)
            if c < 3:
                cst[dst, c * 256:c * 256 + 128] = _words(yr)
                cst[dst, c * 256 + 128:c * 256 + 256] = _words(yi)
            else:
                cst[dst, 768:896] = _words(jnp.concatenate([yr, yi], axis=1))

    for cp in c_cp:
        cp.wait()

    for r in range(0, R, 2):
        pacer.pace([partial(qkv_part, r + 1, k) for k in (1, 2)], 2 * DH + 1)
        attend(r, False)
        shift_kv(r + 1)
        if r % 4 == 2:
            prep_c(r // 4 * (D // G))

    def y_copy(i):
        rows = _ds(i * TP, TP)
        return copy(ob.at[rows, pl.ds(512, 384)], out_hbm.at[0, rows, pl.ds(512, 384)], sem_out.at[i])

    def a_copy(i):
        rows = _ds(i * TP, TP)
        return copy(ob.at[rows, pl.ds(0, 512)], out_hbm.at[0, rows, pl.ds(0, 512)], sem_out.at[NP + i])

    def y_piece(i):
        rows = _ds(i * TP, TP)
        sub = _ds((i % (TG // TP)) * TP, TP)
        hh = jnp.concatenate([h_s[k * G + i // (TG // TP), sub, :] for k in range(7)], axis=1)
        res = lax.dot_general(_bf16(cst[...]), hh, NT, preferred_element_type=F32)
        y = res + xbt[0:D, rows] * dcol[0:D, :]
        ylow[i] = y[0:64]
        for n in range(3):
            ob[rows, 512 + n * 128:640 + n * 128] = y[64 + n * 128:192 + n * 128].T
        y_copy(i).start()
        return res

    qkv_part(1, 0)
    for i in range(R // 2):
        nxt = [partial(qkv_part, 2 * i + 3, 0)] if i < R // 2 - 1 else []
        ys = [partial(y_piece, k) for k in range(NY * i // 8, NY * (i + 1) // 8)]
        pacer.pace(nxt + ys, 2 * DH + 4)
        attend(2 * i + 1, True)
        for c in range(4):
            o_s[c * NP:(c + 1) * NP, i * 8:(i + 1) * 8, :] = (
                ow[c * 128:(c + 1) * 128, :].T.reshape(NP, 8, 128))
        pacer.finish()

    def a_piece(i):
        rows = _ds(i * TP, TP)
        oo = jnp.concatenate([
            _bf16(jnp.concatenate(
                [o_s[c * NP + i, pl.ds(j, R // 2, stride=8), :]
                 for j in range(TP // R)], axis=0))
            for c in range(4)], axis=1)
        a = lax.dot_general(_bf16(wot[0:D // 2, :]), oo, NT, preferred_element_type=F32)
        for n in range(3):
            ob[rows, n * 128:(n + 1) * 128] = a[n * 128:(n + 1) * 128].T
        ob[rows, 384:512] = jnp.concatenate([a[384:D], ylow[i]], axis=0).T
        a_copy(i).start(priority=1)

    def phase4(g, carry):
        for k in range(4):
            if k == 3:
                y_piece(NY + g)
            a_piece(4 * g + k)
        return carry

    lax.fori_loop(0, 4, phase4, 0)
    for i in range(NP):
        y_copy(i).wait()
        a_copy(i).wait()


@jax.jit
def pallas_concat_heads__sliding_local_dilated__ssm_conv_s5__prompt_kernel(
    A_x, A_wqkv, A_wo, B_x, B_Lambda_re, B_Lambda_im, B_B_re, B_B_im, B_C_re, B_C_im,
    B_log_dt, B_Dskip,
):
    hbm = pl.BlockSpec(memory_space=pl.ANY)
    vm = pltpu.VMEM
    dma = pltpu.SemaphoreType.DMA
    scratch = [vm((D,), BF16)] * 4 + [
        vm((512, S), BF16), vm((512, S), BF16),
        vm((4 * S + 16, 128), BF16),
        vm((4 * S + 16, 128), BF16),
        vm((S // 2, 512), U32), vm((S // 2, 512), U32),
        vm((2 * D, D), BF16),
        vm((S, 2 * D), F32),
        vm((D, 3 * D), BF16),
        vm((4 * 1408, 128), BF16),
        vm((3 * D // 2, 512), U32),
        vm((R, D, 128), F32),
        vm((2 * R, D, 128), F32), vm((2 * R, D, 128), F32),
        vm((7 * G, TG + 16, 128), BF16),
        vm((4 * NP, TP // 2 + 8, 128), U32),
        vm((D, D), BF16), vm((D, D), BF16),
        vm((D // 2, 2 * D), U32),
        vm((D, D), BF16), vm((4, D + 32, 128), BF16),
        vm((256, 128), U32), vm((256, 512), U32),
        vm((512, 128), U32),
        vm((512, 128), F32),
        vm((NP, 64, 128), F32),
        vm((G * JG, 1024), F32),
        vm((S, 2 * D), F32),
        dma((4,)), dma((G,)), dma((7,)), dma((6,)), dma((2 * NP,)),
    ]
    return pl.pallas_call(
        _kernel,
        out_shape=jax.ShapeDtypeStruct((1, S, 2 * D), F32),
        in_specs=[hbm] * 12,
        out_specs=hbm,
        scratch_shapes=scratch,
        compiler_params=pltpu.CompilerParams(
            vmem_limit_bytes=100 * 1024 * 1024,
            flags={"XLA_TPU_EVENLY_DISTRIBUTE_CRITICAL_NODES": True}),
    )(jnp.swapaxes(A_x, 1, 2), A_wqkv, A_wo, jnp.swapaxes(B_x, 1, 2), B_Lambda_re, B_Lambda_im,
      B_B_re, B_B_im, B_C_re, B_C_im, B_log_dt, B_Dskip)
```
